```python
import os as _os
_os.environ.setdefault("JAX_PLATFORMS", "cpu")
import jax
import jax.numpy as jnp

def _softmax(x, axis=-1):
    return jax.nn.softmax(x, axis=axis)
def _gelu(x):
    return jax.nn.gelu(x, approximate=True)
def _silu(x):
    return jax.nn.silu(x)
def _sigmoid(x):
    return jax.nn.sigmoid(x)
def _layernorm(x, axis=-1, eps=1e-5):
    m = jnp.mean(x, axis=axis, keepdims=True)
    v = jnp.var(x, axis=axis, keepdims=True)
    return (x - m) / jnp.sqrt(v + eps)
def _scatter_add(tgt, idx, src, axis=0):
    return tgt.at[idx].add(src)
def _segment_sum(src, seg, n):
    return jax.ops.segment_sum(src, seg, n)
class _Rng:
    def __init__(self, key):
        self._k = key
    def _next(self):
        self._k, sub = jax.random.split(self._k)
        return sub
    def normal(self, shape):
        return jax.random.normal(self._next(), shape, dtype=jnp.bfloat16)
    def randint(self, lo, hi, shape):
        return jax.random.randint(self._next(), shape, lo, hi, dtype=jnp.int32)
    def uniform(self, shape, lo=0.0, hi=1.0):
        return jax.random.uniform(self._next(), shape, jnp.bfloat16, lo, hi)
    def permutation(self, n):
        return jax.random.permutation(self._next(), n)


kernel_name = 'gated_mix__ssm_conv_h3__mha_block__prompt'

def setup_inputs():
    _rng = _Rng(jax.random.key(int.from_bytes(__import__("os").urandom(4), "little")))
    _w = (lambda a: (lambda t: t.astype(jnp.bfloat16) if jnp.issubdtype(t.dtype, jnp.floating) else t)(jnp.asarray(a)))
    def _A_setup():
        B, S, D = 1, 2048, 640
        ks = 4
        return {
            "q": _w((lambda *s: _rng.normal(s) * 0.05)(B, S, D)),
            "k": _w((lambda *s: _rng.normal(s) * 0.4)(B, S, D)),
            "v": _w((lambda *s: _rng.normal(s) * 0.4)(B, S, D)),
            "shift_k": _w((lambda *s: _rng.normal(s) * 0.4)(D, ks) * 0.5),
            "ssm_k": _w((lambda *s: _rng.normal(s) * 0.4)(D, S) * (1.0 / S ** 0.5)),
            "ssm_D": _w((lambda *s: _rng.normal(s) * 0.4)(D)),
        }
    _A_in = _A_setup()

    def _B_setup():
        B, S, D, H = 1, 2048, 640, 32
        return {
            "x": _w((lambda *s: _rng.normal(s) * 0.05)(B, S, D)),
            "wqkv": _w((lambda *s: _rng.normal(s) * 0.4)(D, 3 * D)),
            "wo": _w((lambda *s: _rng.normal(s) * 0.05)(D, D)),
        }
    _B_in = _B_setup()

    return {
        "A_q": _A_in["q"],
        "A_k": _A_in["k"],
        "A_v": _A_in["v"],
        "A_shift_k": _A_in["shift_k"],
        "A_ssm_k": _A_in["ssm_k"],
        "A_ssm_D": _A_in["ssm_D"],
        "B_x": _B_in["x"],
        "B_wqkv": _B_in["wqkv"],
        "B_wo": _B_in["wo"],
        "gate_w": _w((lambda *s: _rng.normal(s) * 0.05)(640) * 16.0),
    }

def reference(A_q, A_k, A_v, A_shift_k, A_ssm_k, A_ssm_D, B_x, B_wqkv, B_wo, gate_w):
    def _A_ref(q, k, v, shift_k, ssm_k, ssm_D):
        B, S, D = q.shape
        ks = shift_k.shape[-1]
        k_pad = jnp.pad(k, ((0, 0), (ks - 1, 0), (0, 0)))
        k_shift = jnp.zeros_like(k)
        for t in range(ks):
            k_shift = k_shift + k_pad[:, t:t + S, :] * shift_k[:, ks - 1 - t][None, None, :]
        kv = k_shift * v
        L = 2 * S
        kv_pad = jnp.pad(kv, ((0, 0), (0, S), (0, 0)))
        kf_pad = jnp.pad(ssm_k, ((0, 0), (0, S)))
        kv_f = (lambda x, axes=(-2,-1): jnp.fft.rfft2(x.astype(jnp.float32), axes=axes))(kv_pad[:, None, :, :], axes=(1, 2))
        kf_f = (lambda x, axes=(-2,-1): jnp.fft.rfft2(x.astype(jnp.float32), axes=axes))(kf_pad[:, None, :], axes=(1, 2))
        kf_f = (lambda x, *d: x.transpose(*d))(kf_f, 1, 2, 0)
        y_f = kv_f * kf_f[None, :, :, :]
        y = (lambda x, s, axes=(-2,-1): jnp.fft.irfft2(x, s=s, axes=axes).astype(jnp.bfloat16))(y_f, (1, L), axes=(1, 2))[:, 0, :S, :]
        y = y + kv * ssm_D[None, None, :]
        return q * y

    def _B_ref(x, wqkv, wo):
        B, S, D = x.shape
        H = 32
        Dh = D // H
        qkv = (lambda x, *d: x.transpose(*d))((x @ wqkv).reshape(B, S, 3, H, Dh), 2, 0, 3, 1, 4)
        q, k, v = qkv[0], qkv[1], qkv[2]
        scores = jnp.einsum("bhqd,bhkd->bhqk", q, k) * (Dh ** -0.5)
        p = _softmax(scores, axis=-1)
        o = jnp.einsum("bhqk,bhkd->bhqd", p, v)
        return (lambda x, *d: x.transpose(*d))(o, 0, 2, 1, 3).reshape(B, S, D) @ wo

    x = A_q
    g = _sigmoid((x * gate_w).sum(-1, keepdims=True))
    a = _A_ref(x, A_k, A_v, A_shift_k, A_ssm_k, A_ssm_D)
    b = _B_ref(x, B_wqkv, B_wo)
    return g * a + (1 - g) * b
```

```python
import math

import jax
import jax.numpy as jnp
import numpy as np
import jax.experimental.pallas as pl
import jax.experimental.pallas.tpu as pltpu

S = 2048
D = 640
H = 32
DH = 20
KS = 4
NCH = D // 128
NBUF = 2 * NCH - 1
BLK = 128
NB = S // BLK
CK = 128
SB = 512
RB = 256
F32 = jnp.float32
BF16 = jnp.bfloat16
U32 = jnp.uint32
NT = (((1,), (1,)), ((), ()))


def _dft_consts():
    f = np.concatenate([np.arange(0, BLK, 2), np.arange(1, BLK, 2)]).astype(np.float64)
    n = np.arange(BLK, dtype=np.float64)
    ang = 2.0 * np.pi * (f[:, None] + 0.5) * n[None, :] / (2 * BLK)
    fwd = np.concatenate([np.cos(ang), -np.sin(ang)], axis=0)
    inv = fwd.T / BLK
    return fwd, inv


def _kernel(x_hbm, k_hbm, v_hbm, shk_ref, h_hbm, ssd_ref, w_hbm, wo_hbm, gw_ref,
            fwd_ref, inv_ref, out_hbm,
            x_v, k_v, v_v, h_v, w_v, wo_v, wt_s, k9, q9, vt_s, ot_s,
            kf_s, kv_s, uf_s, hf_s, zf_s, s2, m2, out_v, sems):
    cp_w = pltpu.make_async_copy(w_hbm, w_v, sems.at[0])
    cp_x = pltpu.make_async_copy(x_hbm.at[0], x_v, sems.at[1])
    cp_k = pltpu.make_async_copy(k_hbm.at[0], k_v, sems.at[2])
    cp_v = pltpu.make_async_copy(v_hbm.at[0], v_v, sems.at[3])
    cp_h = pltpu.make_async_copy(h_hbm, h_v, sems.at[4])
    cp_wo = pltpu.make_async_copy(wo_hbm, wo_v, sems.at[5])
    for cp in (cp_w, cp_x, cp_k, cp_v, cp_h, cp_wo):
        cp.start()

    cp_w.wait()
    wt_s[0:D, :] = w_v[:, 0:D].astype(F32).T.astype(BF16)
    wt_s[D:2 * D, :] = w_v[:, 2 * D:3 * D].astype(F32).T.astype(BF16)
    cp_x.wait()

    qscale = (DH ** -0.5) * math.log2(math.e)

    def proj(rb, carry):
        r0 = pl.multiple_of(rb * RB, RB)
        xb = x_v[pl.ds(r0, RB), :]
        kk = jnp.dot(xb, w_v[:, D:2 * D], preferred_element_type=F32)
        kp = pltpu.bitcast(kk.astype(BF16), U32)
        lane = jax.lax.broadcasted_iota(jnp.int32, (RB // 2, 128), 1)
        h0 = pl.multiple_of(rb * (RB // 2), RB // 2)
        for c in range(NCH):
            k9[c, pl.ds(h0, RB // 2), :] = kp[:, c * 128:(c + 1) * 128]
        for c in range(NCH - 1):
            k9[NCH + c, pl.ds(h0, RB // 2), :] = jnp.where(
                lane >= 64, kp[:, c * 128:(c + 1) * 128], kp[:, (c + 1) * 128:(c + 2) * 128])
        qt = jax.lax.dot_general(wt_s[0:D, :], xb, NT, preferred_element_type=F32)
        qp = pltpu.bitcast((qt * qscale).astype(BF16), U32)
        for c in range(NCH):
            q9[c, :, pl.ds(r0, RB)] = qp[c * 64:(c + 1) * 64, :]
        for c in range(NCH - 1):
            q9[NCH + c, 0:32, pl.ds(r0, RB)] = qp[(c + 1) * 64:(c + 1) * 64 + 32, :]
            q9[NCH + c, 32:64, pl.ds(r0, RB)] = qp[c * 64 + 32:(c + 1) * 64, :]
        vt = jax.lax.dot_general(wt_s[D:2 * D, :], xb, NT, preferred_element_type=F32)
        vt = vt.astype(BF16).astype(F32).reshape(H // 2, 2 * DH, RB)
        row = jax.lax.broadcasted_iota(jnp.int32, (H // 2, 24, RB), 1)
        vt_s[0, :, :, pl.ds(r0, RB)] = jnp.where(row < DH, vt[:, 0:24, :], 1.0)
        vt_s[1, :, :, pl.ds(r0, RB)] = jnp.where(row >= 4, vt[:, 16:40, :], 1.0)
        return carry

    jax.lax.fori_loop(0, S // RB, proj, 0)

    eye = (jax.lax.broadcasted_iota(jnp.int32, (8, KS), 0)
           == jax.lax.broadcasted_iota(jnp.int32, (8, KS), 1)).astype(BF16)
    shk = jax.lax.dot_general(eye, shk_ref[...], NT, preferred_element_type=F32)
    cp_k.wait()
    cp_v.wait()
    cp_h.wait()
    kf_s[0:8, :] = jnp.zeros((8, D), F32)

    def conv_fwd(i, carry):
        r0 = pl.multiple_of(i * BLK, BLK)
        kf_s[8:8 + BLK, :] = k_v[pl.ds(r0, BLK), :].astype(F32)
        ksh = kf_s[8:8 + BLK, :] * shk[0:1, :]
        for j in range(1, KS):
            ksh = ksh + kf_s[8 - j:8 - j + BLK, :] * shk[j:j + 1, :]
        kf_s[0:8, :] = kf_s[BLK:BLK + 8, :]
        kv = (ksh * v_v[pl.ds(r0, BLK), :].astype(F32)).astype(BF16)
        kv_s[pl.ds(r0, BLK), :] = kv.astype(F32)
        uf_s[i] = jnp.dot(fwd_ref[...], kv, preferred_element_type=F32)
        hf_s[i] = jax.lax.dot_general(fwd_ref[...], h_v[:, pl.ds(r0, BLK)], NT,
                                      preferred_element_type=F32)
        return carry

    jax.lax.fori_loop(0, NB, conv_fwd, 0)

    def fold(t, carry):
        r = NB - 1 - t
        hb = BLK // 2
        hf_s[r, 0:hb, :] = hf_s[r, 0:hb, :] - hf_s[r - 1, BLK:BLK + hb, :]
        hf_s[r, hb:BLK, :] = hf_s[r, hb:BLK, :] + hf_s[r - 1, BLK + hb:2 * BLK, :]
        hf_s[r, BLK:BLK + hb, :] = hf_s[r, BLK:BLK + hb, :] + hf_s[r - 1, 0:hb, :]
        hf_s[r, BLK + hb:2 * BLK, :] = hf_s[r, BLK + hb:2 * BLK, :] - hf_s[r - 1, hb:BLK, :]
        return carry

    jax.lax.fori_loop(0, NB - 1, fold, 0)

    def freq_mac(g, lo, hi):
        r_re = pl.multiple_of(g * 8, 8)
        r_im = pl.multiple_of(g * 8 + BLK, 8)
        for c in range(lo, hi):
            cols = slice(c * 128, (c + 1) * 128)
            ur = [uf_s[m, pl.ds(r_re, 8), cols] for m in range(NB)]
            ui = [uf_s[m, pl.ds(r_im, 8), cols] for m in range(NB)]
            hr = [hf_s[m, pl.ds(r_re, 8), cols] for m in range(NB)]
            hi_ = [hf_s[m, pl.ds(r_im, 8), cols] for m in range(NB)]
            for i in range(NB):
                zr = None
                zi = None
                for m in range(i + 1):
                    tr = ur[m] * hr[i - m] - ui[m] * hi_[i - m]
                    ti = ur[m] * hi_[i - m] + ui[m] * hr[i - m]
                    zr = tr if zr is None else zr + tr
                    zi = ti if zi is None else zi + ti
                zf_s[i, pl.ds(r_re, 8), cols] = zr
                zf_s[i, pl.ds(r_im, 8), cols] = zi

    def stage(h_qk, h_pv, par_pv, wbuf, rbuf):
        if h_qk is not None:
            f0 = h_qk * DH
            c0 = f0 // 128
            b = jnp.where((f0 % 128) + DH > 128, c0 + NCH, c0)
            row = jax.lax.broadcasted_iota(jnp.int32, (64, SB), 0)
            mask = ((row - h_qk * (DH // 2)) & 63) < (DH // 2)
        if h_pv is not None:
            j = h_pv // 2
        for sb in range(S // SB):
            cols = slice(sb * SB, (sb + 1) * SB)
            if h_qk is not None:
                qt = pltpu.bitcast(jnp.where(mask, q9[b, :, cols], jnp.uint32(0)), BF16)
                mx = None
            if h_pv is not None:
                m = m2[rbuf, 0:1, cols]
                acc = None
            for c in range(S // CK):
                if h_qk is not None:
                    kc = pltpu.bitcast(k9[b, c * CK // 2:(c + 1) * CK // 2, :], BF16)
                    s = jnp.dot(kc, qt, preferred_element_type=F32)
                    s2[wbuf, c * CK:(c + 1) * CK, cols] = s
                    cm = jnp.max(s.reshape(CK // 8, 8, SB), axis=0)
                    mx = cm if mx is None else jnp.maximum(mx, cm)
                if h_pv is not None:
                    p = jnp.exp2(s2[rbuf, c * CK:(c + 1) * CK, cols] - m)
                    r = jnp.dot(vt_s[par_pv, j, :, c * CK:(c + 1) * CK], p,
                                preferred_element_type=F32)
                    acc = r if acc is None else acc + r
            if h_qk is not None:
                m2[wbuf, :, cols] = jnp.broadcast_to(
                    jnp.max(mx, axis=0, keepdims=True), (8, SB))
            if h_pv is not None:
                if par_pv == 0:
                    ot_s[j, 0:DH, cols] = acc[0:DH] * pl.reciprocal(acc[DH:DH + 1, :])
                else:
                    ot_s[j, DH:2 * DH, cols] = acc[4:24] * pl.reciprocal(acc[0:1, :])

    stage(0, None, None, 0, None)
    freq_mac(0, 0, 3)

    def body(h, carry):
        @pl.when(h % 2 == 0)
        def _():
            stage(h + 1, h, 0, 1, 0)
            freq_mac(h // 2, 3, 5)

        @pl.when(h % 2 == 1)
        def _():
            stage(h + 1, h, 1, 0, 1)
            freq_mac((h + 1) // 2, 0, 3)
        return carry

    jax.lax.fori_loop(0, H - 1, body, 0)
    stage(None, H - 1, 1, None, 1)

    cp_wo.wait()
    gw = gw_ref[...].astype(F32).reshape(1, D)
    ssd = ssd_ref[...].astype(F32).reshape(1, D)

    def out_copy(i):
        r0 = pl.multiple_of(i * BLK, BLK)
        return pltpu.make_async_copy(out_v.at[pl.ds(r0, BLK), :],
                                     out_hbm.at[0, pl.ds(r0, BLK), :], sems.at[6])

    def final(i, carry):
        r0 = pl.multiple_of(i * BLK, BLK)
        y = jnp.dot(inv_ref[...], zf_s[i], preferred_element_type=F32)
        o = ot_s[:, :, pl.ds(r0, BLK)].reshape(D, BLK).T.astype(BF16)
        bb = jnp.dot(o, wo_v[...], preferred_element_type=F32)
        x = x_v[pl.ds(r0, BLK), :].astype(F32)
        g = jax.nn.sigmoid(jnp.sum(x * gw, axis=-1, keepdims=True))
        a = x * (y + kv_s[pl.ds(r0, BLK), :] * ssd)
        out_v[pl.ds(r0, BLK), :] = (g * a + (1.0 - g) * bb).astype(BF16)
        out_copy(i).start()
        return carry

    jax.lax.fori_loop(0, NB, final, 0)
    pltpu.make_async_copy(out_v, out_hbm.at[0], sems.at[6]).wait()


@jax.jit
def pallas_gated_mix__ssm_conv_h3__mha_block__prompt_kernel(
    A_q: jax.Array,
    A_k: jax.Array,
    A_v: jax.Array,
    A_shift_k: jax.Array,
    A_ssm_k: jax.Array,
    A_ssm_D: jax.Array,
    B_x: jax.Array,
    B_wqkv: jax.Array,
    B_wo: jax.Array,
    gate_w: jax.Array,
):
    fwd, inv = _dft_consts()
    fwd = jnp.asarray(fwd, dtype=BF16)
    inv = jnp.asarray(inv, dtype=BF16).astype(F32)
    hbm = pl.BlockSpec(memory_space=pl.ANY)
    vmem = pl.BlockSpec(memory_space=pltpu.VMEM)
    scratch = [
        pltpu.VMEM((S, D), BF16),
        pltpu.VMEM((S, D), BF16),
        pltpu.VMEM((S, D), BF16),
        pltpu.VMEM((D, S), BF16),
        pltpu.VMEM((D, 3 * D), BF16),
        pltpu.VMEM((D, D), BF16),
        pltpu.VMEM((2 * D, D), BF16),
        pltpu.VMEM((NBUF, S // 2, 128), U32),
        pltpu.VMEM((NBUF, 64, S), U32),
        pltpu.VMEM((2, H // 2, 24, S), F32),
        pltpu.VMEM((H // 2, 2 * DH, S), F32),
        pltpu.VMEM((BLK + 8, D), F32),
        pltpu.VMEM((S, D), F32),
        pltpu.VMEM((NB, 2 * BLK, D), F32),
        pltpu.VMEM((NB, 2 * BLK, D), F32),
        pltpu.VMEM((NB, 2 * BLK, D), F32),
        pltpu.VMEM((2, S, S), F32),
        pltpu.VMEM((2, 8, S), F32),
        pltpu.VMEM((S, D), BF16),
        pltpu.SemaphoreType.DMA((7,)),
    ]
    return pl.pallas_call(
        _kernel,
        out_shape=jax.ShapeDtypeStruct((1, S, D), BF16),
        in_specs=[hbm, hbm, hbm, vmem, hbm, vmem, hbm, hbm, vmem, vmem, vmem],
        out_specs=hbm,
        scratch_shapes=scratch,
        compiler_params=pltpu.CompilerParams(vmem_limit_bytes=120 * 1024 * 1024),
    )(A_q, A_k, A_v, A_shift_k, A_ssm_k, A_ssm_D, B_wqkv, B_wo, gate_w, fwd, inv)
```

```python
import math
import os

import jax
import jax.numpy as jnp
import numpy as np
import jax.experimental.pallas as pl
import jax.experimental.pallas.tpu as pltpu

S = 2048
D = 640
H = 32
DH = 20
KS = 4
NCH = D // 128
NBUF = 2 * NCH - 1
BLK = 128
NB = S // BLK
NG = BLK // 8
CK = int(os.environ.get('KCK', 128))
SB = 512
NC = S // CK
NSB = S // SB
NU = NC * NSB
RB = 256
NRB = S // RB
CQ = 512
NCQ = S // CQ
FB = 256
R = int(os.environ.get("KR", 256))
PK = int(os.environ.get("KPK", 16))
PQ = int(os.environ.get("KPQ", 256))
AE = int(os.environ.get("KAE", 5))
DEFM = int(os.environ.get("KDEFM", 1))
ACH = int(os.environ.get("KACH", 1))
FT0 = float(os.environ.get("KFT0", 0))
FT1 = float(os.environ.get("KFT1", 0.008))
PT1 = float(os.environ.get("KPT1", 0.04))
VT1 = float(os.environ.get("KVT1", 0))
FE = int(os.environ.get("KFE", 2))
SCOPES = int(os.environ.get("KSCOPES", 0))
SM = S - R
SQ = 256
FL = int(os.environ.get('KFL', 2))
SCORE_BOUND = 80.0
FORCE_SLOW = int(os.environ.get('KSLOW', 0))
RTIE = int(os.environ.get('KRTIE', 1))
NPEEL = int(os.environ.get('KNPEEL', 3))
NOMAX = int(os.environ.get('KNOMAX', 0))
QORD = os.environ.get('KQORD', 'hikqavb')
QB = int(os.environ.get('KQB', 512))
F32 = jnp.float32
BF16 = jnp.bfloat16
U32 = jnp.uint32
I32 = jnp.int32
NT = (((1,), (1,)), ((), ()))

SEM_WK, SEM_WQ, SEM_WV, SEM_WO, SEM_OUT = 0, 1, 2, 3, 4
SEM_GW, SEM_SHK, SEM_SSD, SEM_FWD, SEM_INV = 5, 6, 7, 8, 9
SEM_X = 10
SEM_K = SEM_X + NRB
SEM_V = SEM_K + NCQ
SEM_H = SEM_V + NCQ
NSEM = SEM_H + NCQ


class _Null:
    def __enter__(self):
        return self

    def __exit__(self, *a):
        return False


def scope(name):
    return jax.named_scope(name) if SCOPES else _Null()


def _dft_consts():
    f = np.concatenate([np.arange(0, BLK, 2), np.arange(1, BLK, 2)]).astype(np.float64)
    n = np.arange(BLK, dtype=np.float64)
    ang = 2.0 * np.pi * (f[:, None] + 0.5) * n[None, :] / (2 * BLK)
    re = np.cos(ang).reshape(NG, 8, BLK)
    im = -np.sin(ang).reshape(NG, 8, BLK)
    fwd = np.concatenate([re, im], axis=1).reshape(2 * BLK, BLK)
    inv = fwd.T / BLK
    return fwd, inv


def _kernel(x_hbm, k_hbm, v_hbm, shk_hbm, h_hbm, ssd_hbm, w_hbm, wo_hbm, gw_hbm,
            fwd_hbm, inv_hbm, out_hbm,
            x_v, k_v, wo_v, kp_s, qh_s, vt_s, kv_s, g_s, uf_s, hf_s,
            kfp, kb_s, qf_s, qb_s, bd_s, inv_ref, sems):
    out_v = k_v
    cp_wo = pltpu.make_async_copy(wo_hbm, wo_v, sems.at[SEM_WO])
    cp_inv = pltpu.make_async_copy(inv_hbm, inv_ref, sems.at[SEM_INV])

    def build_kb(j, par, d, anchor=None):
        t = jnp.full((8, 128), par * DH + d, I32)
        if anchor is not None:
            t = anchor(t) & 127
        idx = jnp.concatenate([t] * (R // 8), axis=0)
        kb_s[par, d] = jnp.take_along_axis(kfp[j], idx, axis=1, mode="promise_in_bounds")

    def pre_phase(v_v, h_v, w_v, wt_s, kf_s, hp_s, kn_s, fwd_ref, shk_ref, ssd_ref, gw_ref):

        def w_copy(part, sem):
            return pltpu.make_async_copy(w_hbm.at[:, part * D:(part + 1) * D],
                                         w_v.at[:, part * D:(part + 1) * D], sems.at[sem])

        def x_copy(i):
            r0 = pl.multiple_of(i * RB, RB)
            return pltpu.make_async_copy(x_hbm.at[0, pl.ds(r0, RB), :],
                                         x_v.at[pl.ds(r0, RB), :], sems.at[SEM_X + i])

        def kvh_copies(i):
            r0 = pl.multiple_of(i * CQ, CQ)
            return (
                pltpu.make_async_copy(k_hbm.at[0, pl.ds(r0, CQ), :],
                                      k_v.at[pl.ds(r0, CQ), :], sems.at[SEM_K + i]),
                pltpu.make_async_copy(v_hbm.at[0, pl.ds(r0, CQ), :],
                                      v_v.at[pl.ds(r0, CQ), :], sems.at[SEM_V + i]),
                pltpu.make_async_copy(h_hbm.at[:, pl.ds(r0, CQ)],
                                      h_v.at[:, pl.ds(r0, CQ)], sems.at[SEM_H + i]),
            )


        cp_gw = pltpu.make_async_copy(gw_hbm, gw_ref, sems.at[SEM_GW])
        cp_small = (
            pltpu.make_async_copy(shk_hbm, shk_ref, sems.at[SEM_SHK]),
            pltpu.make_async_copy(ssd_hbm, ssd_ref, sems.at[SEM_SSD]),
            pltpu.make_async_copy(fwd_hbm, fwd_ref, sems.at[SEM_FWD]),
        )
        w_copy(1, SEM_WK).start()
        x_copy(0).start()
        cp_gw.start()
        for i in range(1, NRB):
            x_copy(i).start()
        for cp in cp_small:
            cp.start()
        w_copy(0, SEM_WQ).start()
        w_copy(2, SEM_WV).start()
        for i in range(NCQ):
            for cp in kvh_copies(i):
                cp.start()
        cp_wo.start()
        cp_inv.start()

        kf_s[:, 0:8, :] = jnp.zeros((NCH, 8, 128), F32)
        hp_s[...] = jnp.zeros((2 * BLK, D), F32)
        bd_s[...] = jnp.zeros((4, 8, 128), F32)

        def track(i, val):
            a = jnp.abs(val)
            a = jnp.max(a.reshape(a.shape[0] // 8, 8, a.shape[1]), axis=0)
            m = bd_s[i]
            for c in range(a.shape[1] // 128):
                m = jnp.maximum(m, a[:, c * 128:(c + 1) * 128])
            bd_s[i] = m

        def split_pairs(val):
            lane = jax.lax.broadcasted_iota(I32, (val.shape[0], 128), 1)
            parts = [val[:, c * 128:(c + 1) * 128] for c in range(NCH)]
            out = []
            for j in range(H // 2):
                c, sh = divmod(2 * DH * j, 128)
                src = parts[c]
                if sh + 2 * DH > 128:
                    src = jnp.where(lane >= 64, src, parts[c + 1])
                out.append(pltpu.roll(src, 128 - sh, 1) if sh else src)
            return out

        def kproj(rb, keep_f32=False):
            r0 = pl.multiple_of(rb * RB, RB)
            xb = x_v[pl.ds(r0, RB), :]
            kk = jnp.dot(xb, w_v[:, D:2 * D], preferred_element_type=F32)
            track(0, kk)
            kb16 = kk.astype(BF16)
            kp = pltpu.bitcast(kb16, U32)
            h0 = pl.multiple_of(rb * (RB // 2), RB // 2)
            kn_s[pl.ds(h0, RB // 2), :] = kp
            if keep_f32:
                lo = max(SM, rb * RB)
                if lo < (rb + 1) * RB:
                    for j, part in enumerate(split_pairs(kp[(lo - rb * RB) // 2:, :])):
                        kfp[j, lo - SM:(rb + 1) * RB - SM, :] = pltpu.bitcast(part, BF16).astype(F32)
            gw = gw_ref[...].astype(F32).reshape(1, D)
            g = jax.nn.sigmoid(jnp.sum(xb.astype(F32) * gw, axis=-1, keepdims=True))
            g_s[pl.ds(r0, RB), :] = jnp.broadcast_to(g, (RB, 128))

        with scope("s_wait_wk"):
            w_copy(1, SEM_WK).wait()
            cp_gw.wait()

        def kproj_loop(rb, carry):
            x_copy(rb).wait()
            kproj(rb)
            return carry

        with scope("s_kloop"):
            jax.lax.fori_loop(0, NRB - NPEEL, kproj_loop, 0)
        with scope("s_kpeel"):
            for i in range(NRB - NPEEL, NRB):
                x_copy(i).wait()
            w_copy(0, SEM_WQ).wait()
            w_copy(2, SEM_WV).wait()
            for cp in cp_small:
                cp.wait()
            kproj(NRB - 1, keep_f32=True)
            wt_s[0:D, :] = w_v[:, 0:D].astype(F32).T.astype(BF16)
            wt_s[D:2 * D, :] = w_v[:, 2 * D:3 * D].astype(F32).T.astype(BF16)
            for i in range(NRB - 2, NRB - NPEEL - 1, -1):
                kproj(i, keep_f32=True)
            for d in range(DH):
                build_kb(0, 0, d)

        qscale = (DH ** -0.5) * math.log2(math.e)

        def fold(cur, prev):
            cur = cur.reshape(NG, 16, D)
            prev = prev.reshape(NG, 16, D)
            hg = NG // 2
            lo = jnp.concatenate([cur[:hg, 0:8] - prev[:hg, 8:16], cur[:hg, 8:16] + prev[:hg, 0:8]], axis=1)
            hi = jnp.concatenate([cur[hg:, 0:8] + prev[hg:, 8:16], cur[hg:, 8:16] - prev[hg:, 0:8]], axis=1)
            return jnp.concatenate([lo, hi], axis=0)

        def qvproj(rb, carry):
            if QB < CQ:
                @pl.when(rb % (CQ // QB) == 0)
                def _():
                    for cp in kvh_copies(rb // (CQ // QB)):
                        cp.wait()
            else:
                for cp in kvh_copies(rb):
                    cp.wait()

            ssd = ssd_ref[...].astype(F32).reshape(1, D)
            shk = shk_ref[...].astype(F32)
            r0 = pl.multiple_of(rb * QB, QB)
            nsub = QB // RB
            nblk = RB // BLK

            def q_part(rs):
                xb = x_v[pl.ds(rs, RB), :]
                qt = jax.lax.dot_general(wt_s[0:D, :], xb, NT, preferred_element_type=F32)
                qt = qt * qscale
                track(1, qt)
                qb16 = qt.astype(BF16)
                qf = qb16.astype(F32).reshape(H // 2, 2 * DH, RB)
                row = jax.lax.broadcasted_iota(I32, (H // 2, 24, RB), 1)
                zpad = jnp.zeros((H // 2, 8, RB), F32)
                for par, win in ((0, jnp.where(row < DH, qf[:, 0:24], 0.0)),
                                 (1, jnp.where(row >= 4, qf[:, 16:40], 0.0))):
                    win = jnp.concatenate([win, zpad], axis=1).reshape(H // 2 * 32, RB).astype(BF16)
                    qh_s[par, :, :, pl.ds(rs, RB)] = pltpu.bitcast(win, U32).reshape(H // 2, 16, RB)
                qf_s[:, :, pl.ds(rs, RB)] = qf
                for d in range(DH):
                    qb_s[0, d, :, pl.ds(rs, RB)] = jnp.broadcast_to(qf[0, d:d + 1, :], (8, RB))

            def v_part(rs):
                xb = x_v[pl.ds(rs, RB), :]
                vt = jax.lax.dot_general(wt_s[D:2 * D, :], xb, NT, preferred_element_type=F32)
                track(2, vt)
                vt = vt.astype(BF16).astype(F32).reshape(H // 2, 2 * DH, RB)
                row = jax.lax.broadcasted_iota(I32, (H // 2, 24, RB), 1)
                vt_s[0, :, :, pl.ds(rs, RB)] = jnp.where(row < DH, vt[:, 0:24, :], 1.0)
                vt_s[1, :, :, pl.ds(rs, RB)] = jnp.where(row >= 4, vt[:, 16:40, :], 1.0)

            def k_split(rs):
                h0 = pl.multiple_of(rs // 2, RB // 2)
                for j, part in enumerate(split_pairs(kn_s[pl.ds(h0, RB // 2), :])):
                    kp_s[j, pl.ds(h0, RB // 2), :] = part

            def u_part(u):
                ru = pl.multiple_of(r0 + u * BLK, BLK)
                parts = []
                for c in range(NCH):
                    cols = slice(c * 128, (c + 1) * 128)
                    base = 8 + u * BLK
                    ksh = kf_s[c, base:base + BLK, :] * shk[0:1, cols]
                    for j in range(1, KS):
                        ksh = ksh + kf_s[c, base - j:base - j + BLK, :] * shk[j:j + 1, cols]
                    parts.append(ksh)
                ksh = jnp.concatenate(parts, axis=1)
                kv = (ksh * v_v[pl.ds(ru, BLK), :].astype(F32)).astype(BF16)
                kv_s[pl.ds(ru, BLK), :] = kv.astype(F32) * ssd
                uf_s[:, rb * (QB // BLK) + u] = jnp.dot(
                    fwd_ref[...], kv, preferred_element_type=F32).reshape(NG, 16, D)

            def h_part(u, prev):
                ru = pl.multiple_of(r0 + u * BLK, BLK)
                raw = jax.lax.dot_general(fwd_ref[...], h_v[:, pl.ds(ru, BLK)], NT,
                                          preferred_element_type=F32)
                hf_s[:, rb * (QB // BLK) + u] = fold(raw, prev)
                return raw

            kin = k_v[pl.ds(r0, QB), :].astype(F32)
            for c in range(NCH):
                kf_s[c, 8:8 + QB, :] = kin[:, c * 128:(c + 1) * 128]
            prev = hp_s[...]
            for sub in range(nsub):
                rs = pl.multiple_of(r0 + sub * RB, RB)
                for op in QORD:
                    if op == "q":
                        q_part(rs)
                    elif op == "v":
                        v_part(rs)
                    elif op == "a":
                        u_part(sub * nblk)
                    elif op == "b":
                        u_part(sub * nblk + 1)
                    elif op == "k":
                        k_split(rs)
                    elif op == "h":
                        prev = h_part(sub * nblk, prev)
                    elif op == "i":
                        prev = h_part(sub * nblk + 1, prev)
                        if sub == nsub - 1:
                            hp_s[...] = prev
            kf_s[:, 0:8, :] = kf_s[:, QB:QB + 8, :]
            return carry

        with scope("s_qv"):
            jax.lax.fori_loop(0, S // QB, qvproj, 0)

    pl.run_scoped(
        pre_phase,
        pltpu.VMEM((S, D), BF16),
        pltpu.VMEM((D, S), BF16),
        pltpu.VMEM((D, 3 * D), BF16),
        pltpu.VMEM((2 * D, D), BF16),
        pltpu.VMEM((NCH, QB + 32, 128), F32),
        pltpu.VMEM((2 * BLK, D), F32),
        pltpu.VMEM((S // 2, D), U32),
        pltpu.VMEM((2 * BLK, BLK), BF16),
        pltpu.VMEM((KS, D), BF16),
        pltpu.VMEM((D,), BF16),
        pltpu.VMEM((D,), BF16),
    )

    def post_phase(s2, m2, zf_s, ot_s):
        def freq_steps(g, chunks):
            steps = []
            for c in chunks:
                cols = slice(c * 128, (c + 1) * 128) if isinstance(c, int) else c
                for i in range(NB):
                    st = {}
                    for m0 in range(0, i + 1, FE):
                        ms = list(range(m0, min(i + 1, m0 + FE)))

                        def step(anchor, i=i, cols=cols, ms=ms, st=st):
                            for m in ms:
                                ur = uf_s[g, m, 0:8, cols]
                                ui = uf_s[g, m, 8:16, cols]
                                hr = hf_s[g, i - m, 0:8, cols]
                                hi = hf_s[g, i - m, 8:16, cols]
                                if m == ms[0]:
                                    ur = anchor(ur)
                                tr = ur * hr - ui * hi
                                ti = ur * hi + ui * hr
                                st["r"] = tr if m == 0 else st["r"] + tr
                                st["i"] = ti if m == 0 else st["i"] + ti
                            if ms[-1] == i:
                                zf_s[g, i, 0:8, cols] = st["r"]
                                zf_s[g, i, 8:16, cols] = st["i"]
                        steps.append((len(ms), step))
            return steps

        def timeline(steps, t0, t1):
            total = sum(w for w, _ in steps)
            out = {}
            acc = 0
            for w, p in steps:
                tau = t0 + (t1 - t0) * acc / total
                out.setdefault(int(tau), []).append((tau - int(tau), p))
                acc += w
            return out

        bounds = [min(SM, ((SM * c // NC) + 15) // 16 * 16) for c in range(NC + 1)]

        def stage(h_qk, par_qk, h_pv, live=None, fpieces=None, extra=None):
            par_pv = 1 - par_qk
            wbuf, rbuf = par_qk, par_pv

            def tie_to(tie):
                def anchor(v):
                    t = tie if tie.dtype == v.dtype else pltpu.bitcast(tie, v.dtype)
                    if v.shape[0] > 8:
                        t = jnp.concatenate([t] * (v.shape[0] // 8), axis=0)
                    if v.shape[1] > 128:
                        t = jnp.concatenate([t] * (v.shape[1] // 128), axis=1)
                    return jnp.where(live, v, t)
                return anchor

            if h_qk is not None:
                jq = h_qk >> 1
                j_nx = jnp.minimum(h_qk + 1, H - 1) >> 1
                ftl = timeline(fpieces, FT0 * NU, NU * (1 - FT1))

                def prep_q(anchor, t):
                    tc = slice(t * 128, (t + 1) * 128)
                    blk = anchor(qf_s[j_nx, par_pv * 16:par_pv * 16 + 24, tc])
                    for d in range(DH):
                        rr = par_pv * 4 + d
                        qb_s[par_pv, d, :, tc] = jnp.broadcast_to(blk[rr:rr + 1, :], (8, 128))

                psteps = []
                for i in range(DH):
                    psteps.append((1, lambda anchor, i=i: build_kb(j_nx, par_pv, i, anchor)))
                    if i < S // 128:
                        psteps.append((1, lambda anchor, i=i: prep_q(anchor, i)))
                ptl = timeline(psteps, 0, NU * (1 - PT1))
            if h_pv is not None:
                j = h_pv >> 1
            for sb in range(NSB):
                cols = slice(sb * SB, (sb + 1) * SB)
                if h_qk is not None:
                    vsteps = []
                    for kg in range(R // PK):
                        for qq in range(SB // PQ):
                            st = {}
                            for d0 in range(0, DH, AE):
                                def step(anchor, kg=kg, qq=qq, d0=d0, st=st):
                                    q0 = sb * SB + qq * PQ
                                    for d in range(d0, min(DH, d0 + AE)):
                                        kb = kb_s[par_qk, d, kg * PK:(kg + 1) * PK, :]
                                        if d == d0:
                                            kb = anchor(kb)
                                        qr = qb_s[par_qk, d, :, q0:q0 + PQ]
                                        t = (jnp.concatenate([kb] * (PQ // 128), axis=1)
                                             * jnp.concatenate([qr] * (PK // 8), axis=0))
                                        st["a"] = t if d == 0 else st["a"] + t
                                    if d0 + AE >= DH:
                                        s2[wbuf, SM + kg * PK:SM + (kg + 1) * PK,
                                           q0:q0 + PQ] = jnp.exp2(st["a"])
                                vsteps.append((1, step))
                    vtl = timeline(vsteps, 0, NC - VT1)
                acc = None
                for c in range(NC):
                    u = sb * NC + c
                    if h_qk is not None:
                        r0, r1 = bounds[c], bounds[c + 1]
                        kc = pltpu.bitcast(kp_s[jq, r0 // 2:r1 // 2, :], BF16)
                        qt = qh_s[par_qk, jq, :, cols]
                        if par_qk == 1:
                            qt = jnp.concatenate([jnp.zeros((8, SB), U32), qt], axis=0)
                        qt = pltpu.bitcast(qt, BF16)
                        s = jnp.dot(kc[:, 0:qt.shape[0]], qt, preferred_element_type=F32)
                        s2[wbuf, r0:r1, cols] = jnp.exp2(s)
                    if h_pv is not None:
                        r = jnp.dot(vt_s[par_pv, j, :, c * CK:(c + 1) * CK],
                                    s2[rbuf, c * CK:(c + 1) * CK, cols],
                                    preferred_element_type=F32)
                        if acc is None and h_qk is not None:
                            z = tie_to(s[0:8, 0:128])(jnp.zeros((8, 128), F32))
                            z = jnp.concatenate([z] * 3, axis=0)
                            acc = jnp.concatenate([z] * (SB // 128), axis=1)
                        acc = r if acc is None else acc + r
                    if h_qk is not None:
                        ties = s
                        if h_pv is not None and u < NU - 1:
                            ties = jnp.concatenate([s, r], axis=0)
                        ng = ties.shape[0] // 8
                        for col, tl in ((0, vtl.get(c, [])), (1, ptl.get(u, [])), (2, ftl.get(u, []))):
                            for frac, p in tl:
                                gi = min(ng - 1, int(frac * ng))
                                p(tie_to(ties[gi * 8:(gi + 1) * 8, col * 128:(col + 1) * 128]))
                    if extra is not None:
                        extra(u)
                if h_pv is not None:
                    ot_s[par_pv, j, :, cols] = acc

        def inv_block(i):
            rows = pl.ds(i * BLK, BLK) if isinstance(i, int) else pl.ds(pl.multiple_of(i * BLK, BLK), BLK)
            y = jnp.dot(inv_ref[...], zf_s[:, i].reshape(2 * BLK, D), preferred_element_type=F32)
            g = g_s[rows, :]
            gx = x_v[rows, :].astype(F32) * jnp.concatenate([g] * NCH, axis=1)
            kv_s[rows, :] = gx * (y + kv_s[rows, :])

        def fast_path():
            def body(t, carry):
                live = t >= 0

                @pl.when(t == 0)
                def _():
                    with scope("s_stage0"):
                        stage(t, 0, None, live, freq_steps(t >> 1, (0, 1, 2)))

                @pl.when((t & 1) == 1)
                def _():
                    with scope("s_odd"):
                        stage(t, 1, t - 1, live, freq_steps(t >> 1, (3, 4)))

                @pl.when(jnp.logical_and((t & 1) == 0, t > 0))
                def _():
                    with scope("s_even"):
                        stage(t, 0, t - 1, live, freq_steps(t >> 1, (0, 1, 2)))
                return carry

            jax.lax.fori_loop(0, H, body, 0)

            def extra(u):
                if u % (NU // NB) == 0:
                    inv_block(u // (NU // NB))

            with scope("s_epi"):
                stage(None, 0, H - 1, extra=extra)

        def slow_path():
            nq = S // SQ

            def block(it_qk, it_pv, wbuf):
                rbuf = 1 - wbuf
                h = it_qk // nq
                c0 = pl.multiple_of((it_qk % nq) * SQ, SQ)
                q32 = qh_s[h & 1, h >> 1, :, pl.ds(c0, SQ)]
                z = jnp.zeros((8, SQ), U32)
                qt = pltpu.bitcast(jnp.where((h & 1) == 1, jnp.concatenate([z, q32], axis=0),
                                             jnp.concatenate([q32, z], axis=0)), BF16)
                if it_pv is not None:
                    hp = it_pv // nq
                    m = jnp.max(m2[rbuf], axis=0, keepdims=True)
                mx = None
                acc = None
                for c in range(S // SQ):
                    rows = slice(c * SQ, (c + 1) * SQ)
                    kc = pltpu.bitcast(kp_s[h >> 1, c * SQ // 2:(c + 1) * SQ // 2, :], BF16)
                    s = jnp.dot(kc[:, 0:48], qt, preferred_element_type=F32)
                    s2[wbuf, rows, 0:SQ] = s
                    cm = jnp.max(s.reshape(SQ // 8, 8, SQ), axis=0)
                    mx = cm if mx is None else jnp.maximum(mx, cm)
                    if it_pv is not None:
                        p = jnp.exp2(s2[rbuf, rows, 0:SQ] - m)
                        r = jnp.dot(vt_s[hp & 1, hp >> 1, :, rows], p, preferred_element_type=F32)
                        acc = r if acc is None else acc + r
                m2[wbuf] = mx
                if it_pv is not None:
                    cp = pl.multiple_of((it_pv % nq) * SQ, SQ)
                    ot_s[hp & 1, hp >> 1, :, pl.ds(cp, SQ)] = acc

            block(jnp.int32(0), None, 0)

            def body(it, carry):
                nxt = jnp.minimum(it + 1, H * nq - 1)

                @pl.when((it & 1) == 0)
                def _():
                    block(nxt, it, 1)

                @pl.when((it & 1) == 1)
                def _():
                    block(nxt, it, 0)
                return carry

            jax.lax.fori_loop(0, H * nq, body, 0)

            def fbody(i, carry):
                cols = pl.ds(pl.multiple_of((i % NCH) * 128, 128), 128)
                for _, p in freq_steps(i // NCH, (cols,)):
                    p(lambda v: v)
                return carry

            jax.lax.fori_loop(0, NG * NCH, fbody, 0)

            def ibody(i, carry):
                inv_block(i)
                return carry

            jax.lax.fori_loop(0, NB, ibody, 0)

        cp_inv.wait()
        kmax = jnp.max(bd_s[0])
        qmax = jnp.max(bd_s[1])
        vmax = jnp.max(bd_s[2])
        safe = jnp.logical_and(
            kmax * qmax * (1.02 * DH) <= SCORE_BOUND,
            jnp.logical_and(vmax <= 2.0 ** 30, vmax >= 2.0 ** -20))
        if FORCE_SLOW:
            safe = jnp.logical_and(safe, kmax < 0)

        @pl.when(safe)
        def _():
            fast_path()

        @pl.when(jnp.logical_not(safe))
        def _():
            slow_path()

        cp_wo.wait()
        def final(it, carry):
            for i in range(S // FB // FL):
                r0 = pl.multiple_of(it * (S // FL) + i * FB, FB)
                rows = pl.ds(r0, FB)
                oe = ot_s[0, :, :, rows]
                oo = ot_s[1, :, :, rows]
                oe = oe * pl.reciprocal(oe[:, DH:DH + 1, :])
                oo = oo * pl.reciprocal(oo[:, 0:1, :])
                row = jax.lax.broadcasted_iota(I32, (H // 2, 8, FB), 1)
                o = jnp.concatenate(
                    [oe[:, 0:16], jnp.where(row < 4, oe[:, 16:24], oo[:, 0:8]), oo[:, 8:24]], axis=1)
                o = o.reshape(D, FB).T.astype(BF16)
                bb = jnp.dot(o, wo_v[...], preferred_element_type=F32)
                g1 = 1.0 - g_s[rows, :]
                out_v[rows, :] = (kv_s[rows, :]
                                  + jnp.concatenate([g1] * NCH, axis=1) * bb).astype(BF16)
                pltpu.make_async_copy(out_v.at[rows, :], out_hbm.at[0, rows, :],
                                      sems.at[SEM_OUT]).start()
            return carry

        with scope("s_final"):
            jax.lax.fori_loop(0, FL, final, 0)
        with scope("s_outwait"):
            pltpu.make_async_copy(out_v, out_hbm.at[0], sems.at[SEM_OUT]).wait()

    pl.run_scoped(
        post_phase,
        pltpu.VMEM((2, S, S), F32),
        pltpu.VMEM((2, 8, SQ), F32),
        pltpu.VMEM((NG, NB, 16, D), F32),
        pltpu.VMEM((2, H // 2, 24, S), F32),
    )


@jax.jit
def pallas_gated_mix__ssm_conv_h3__mha_block__prompt_kernel(
    A_q: jax.Array,
    A_k: jax.Array,
    A_v: jax.Array,
    A_shift_k: jax.Array,
    A_ssm_k: jax.Array,
    A_ssm_D: jax.Array,
    B_x: jax.Array,
    B_wqkv: jax.Array,
    B_wo: jax.Array,
    gate_w: jax.Array,
):
    fwd, inv = _dft_consts()
    fwd = jnp.asarray(fwd, dtype=BF16)
    inv = jnp.asarray(inv, dtype=BF16).astype(F32)
    hbm = pl.BlockSpec(memory_space=pl.ANY)
    scratch = [
        pltpu.VMEM((S, D), BF16),
        pltpu.VMEM((S, D), BF16),
        pltpu.VMEM((D, D), BF16),
        pltpu.VMEM((H // 2, S // 2, 128), U32),
        pltpu.VMEM((2, H // 2, 16, S), U32),
        pltpu.VMEM((2, H // 2, 24, S), F32),
        pltpu.VMEM((S, D), F32),
        pltpu.VMEM((S, 128), F32),
        pltpu.VMEM((NG, NB, 16, D), F32),
        pltpu.VMEM((NG, NB, 16, D), F32),
        pltpu.VMEM((H // 2, R, 128), F32),
        pltpu.VMEM((2, DH, R, 128), F32),
        pltpu.VMEM((H // 2, 2 * DH, S), F32),
        pltpu.VMEM((2, DH, 8, S), F32),
        pltpu.VMEM((4, 8, 128), F32),
        pltpu.VMEM((BLK, 2 * BLK), F32),
        pltpu.SemaphoreType.DMA((NSEM,)),
    ]
    return pl.pallas_call(
        _kernel,
        out_shape=jax.ShapeDtypeStruct((1, S, D), BF16),
        in_specs=[hbm] * 11,
        out_specs=hbm,
        scratch_shapes=scratch,
        compiler_params=pltpu.CompilerParams(vmem_limit_bytes=127 * 1024 * 1024),
    )(A_q, A_k, A_v, A_shift_k.T, A_ssm_k, A_ssm_D, B_wqkv, B_wo, gate_w, fwd, inv)
```

```python
import math

import jax
import jax.numpy as jnp
import numpy as np
import jax.experimental.pallas as pl
import jax.experimental.pallas.tpu as pltpu

S = 2048
D = 640
H = 32
DH = 20
KS = 4
NCH = D // 128
BLK = 128
NB = S // BLK
NG = BLK // 8
CK = 128
SB = 512
NC = S // CK
NSB = S // SB
NU = NC * NSB
RB = 256
NRB = S // RB
NPEEL = 3
QB = 512
NQB = S // QB
FB = 128
R = 256
SM = S - R
PK, PQ = 16, 256
AE = 5
FE = 2
SQ = 256
SCORE_BOUND = 80.0
F32 = jnp.float32
BF16 = jnp.bfloat16
U32 = jnp.uint32
I32 = jnp.int32
NT = (((1,), (1,)), ((), ()))

SEM_WK, SEM_WQ, SEM_WV, SEM_WO, SEM_OUT = 0, 1, 2, 3, 4
SEM_GW, SEM_SHK, SEM_SSD, SEM_FWD, SEM_INV = 5, 6, 7, 8, 9
SEM_X = 10
SEM_K = SEM_X + NRB
SEM_V = SEM_K + NQB
SEM_H = SEM_V + NQB
NSEM = SEM_H + NQB


def _dft_consts():
    f = np.concatenate([np.arange(0, BLK, 2), np.arange(1, BLK, 2)]).astype(np.float64)
    n = np.arange(BLK, dtype=np.float64)
    ang = 2.0 * np.pi * (f[:, None] + 0.5) * n[None, :] / (2 * BLK)
    re = np.cos(ang).reshape(NG, 8, BLK)
    im = -np.sin(ang).reshape(NG, 8, BLK)
    fwd = np.concatenate([re, im], axis=1).reshape(2 * BLK, BLK)
    inv = fwd.T / BLK
    return fwd, inv


def _timeline(steps, t0, t1):
    total = sum(w for w, _ in steps)
    out = {}
    acc = 0
    for w, p in steps:
        tau = t0 + (t1 - t0) * acc / total
        out.setdefault(int(tau), []).append((tau - int(tau), p))
        acc += w
    return out


def _kernel(x_hbm, k_hbm, v_hbm, shk_hbm, h_hbm, ssd_hbm, w_hbm, wo_hbm, gw_hbm,
            fwd_hbm, inv_hbm, out_hbm,
            x_v, k_v, wo_v, kp_s, qh_s, vt_s, kv_s, g_s, uf_s, hf_s,
            kfp, kb_s, qf_s, qb_s, bd_s, inv_ref, sems):
    out_v = k_v
    cp_wo = pltpu.make_async_copy(wo_hbm, wo_v, sems.at[SEM_WO])
    cp_inv = pltpu.make_async_copy(inv_hbm, inv_ref, sems.at[SEM_INV])

    def build_kb(j, par, d, anchor=None):
        t = jnp.full((8, 128), par * DH + d, I32)
        if anchor is not None:
            t = anchor(t) & 127
        idx = jnp.concatenate([t] * (R // 8), axis=0)
        kb_s[par, d] = jnp.take_along_axis(kfp[j], idx, axis=1, mode="promise_in_bounds")

    def pre_phase(v_v, h_v, w_v, wt_s, kf_s, hp_s, kn_s, fwd_ref, shk_ref, ssd_ref, gw_ref):
        def w_copy(part, sem):
            return pltpu.make_async_copy(w_hbm.at[:, part * D:(part + 1) * D],
                                         w_v.at[:, part * D:(part + 1) * D], sems.at[sem])

        def x_copy(i):
            r0 = pl.multiple_of(i * RB, RB)
            return pltpu.make_async_copy(x_hbm.at[0, pl.ds(r0, RB), :],
                                         x_v.at[pl.ds(r0, RB), :], sems.at[SEM_X + i])

        def kvh_copies(i):
            r0 = pl.multiple_of(i * QB, QB)
            return (
                pltpu.make_async_copy(k_hbm.at[0, pl.ds(r0, QB), :],
                                      k_v.at[pl.ds(r0, QB), :], sems.at[SEM_K + i]),
                pltpu.make_async_copy(v_hbm.at[0, pl.ds(r0, QB), :],
                                      v_v.at[pl.ds(r0, QB), :], sems.at[SEM_V + i]),
                pltpu.make_async_copy(h_hbm.at[:, pl.ds(r0, QB)],
                                      h_v.at[:, pl.ds(r0, QB)], sems.at[SEM_H + i]),
            )

        cp_gw = pltpu.make_async_copy(gw_hbm, gw_ref, sems.at[SEM_GW])
        cp_small = (
            pltpu.make_async_copy(shk_hbm, shk_ref, sems.at[SEM_SHK]),
            pltpu.make_async_copy(ssd_hbm, ssd_ref, sems.at[SEM_SSD]),
            pltpu.make_async_copy(fwd_hbm, fwd_ref, sems.at[SEM_FWD]),
        )
        x_copy(0).start()
        w_copy(1, SEM_WK).start()
        cp_gw.start()
        for i in range(1, NRB):
            x_copy(i).start()
        for cp in cp_small:
            cp.start()
        w_copy(0, SEM_WQ).start()
        w_copy(2, SEM_WV).start()
        for i in range(NQB):
            for cp in kvh_copies(i):
                cp.start()
        cp_wo.start()
        cp_inv.start()

        kf_s[0:8, :] = jnp.zeros((8, D), F32)
        hp_s[...] = jnp.zeros((2 * BLK, D), F32)
        bd_s[...] = jnp.zeros((4, 8, 128), F32)

        def track(i, val):
            a = jnp.abs(val)
            a = jnp.max(a.reshape(a.shape[0] // 8, 8, a.shape[1]), axis=0)
            m = bd_s[i]
            for c in range(a.shape[1] // 128):
                m = jnp.maximum(m, a[:, c * 128:(c + 1) * 128])
            bd_s[i] = m

        def split_pairs(val):
            lane = jax.lax.broadcasted_iota(I32, (val.shape[0], 128), 1)
            parts = [val[:, c * 128:(c + 1) * 128] for c in range(NCH)]
            out = []
            for j in range(H // 2):
                c, sh = divmod(2 * DH * j, 128)
                src = parts[c]
                if sh + 2 * DH > 128:
                    src = jnp.where(lane >= 64, src, parts[c + 1])
                out.append(pltpu.roll(src, 128 - sh, 1) if sh else src)
            return out

        def kproj(rb):
            r0 = pl.multiple_of(rb * RB, RB)
            xb = x_v[pl.ds(r0, RB), :]
            kk = jnp.dot(xb, w_v[:, D:2 * D], preferred_element_type=F32)
            track(0, kk)
            kp = pltpu.bitcast(kk.astype(BF16), U32)
            h0 = pl.multiple_of(rb * (RB // 2), RB // 2)
            kn_s[pl.ds(h0, RB // 2), :] = kp
            if isinstance(rb, int) and (rb + 1) * RB > SM:
                lo = max(SM, rb * RB)
                for j, part in enumerate(split_pairs(kp[(lo - rb * RB) // 2:, :])):
                    kfp[j, lo - SM:(rb + 1) * RB - SM, :] = pltpu.bitcast(part, BF16).astype(F32)
            gw = gw_ref[...].astype(F32).reshape(1, D)
            g = jax.nn.sigmoid(jnp.sum(xb.astype(F32) * gw, axis=-1, keepdims=True))
            g_s[pl.ds(r0, RB), :] = jnp.broadcast_to(g, (RB, 128))

        w_copy(1, SEM_WK).wait()
        cp_gw.wait()

        def kproj_loop(rb, carry):
            x_copy(rb).wait()
            kproj(rb)
            return carry

        jax.lax.fori_loop(0, NRB - NPEEL, kproj_loop, 0)
        for i in range(NRB - NPEEL, NRB):
            x_copy(i).wait()
        w_copy(0, SEM_WQ).wait()
        w_copy(2, SEM_WV).wait()
        for cp in cp_small:
            cp.wait()
        kproj(NRB - 1)
        wt_s[0:D, :] = w_v[:, 0:D].astype(F32).T.astype(BF16)
        wt_s[D:2 * D, :] = w_v[:, 2 * D:3 * D].astype(F32).T.astype(BF16)
        for i in range(NRB - 2, NRB - NPEEL - 1, -1):
            kproj(i)
        for d in range(DH):
            build_kb(0, 0, d)

        qscale = (DH ** -0.5) * math.log2(math.e)

        def fold(cur, prev):
            cur = cur.reshape(NG, 16, D)
            prev = prev.reshape(NG, 16, D)
            hg = NG // 2
            lo = jnp.concatenate(
                [cur[:hg, 0:8] - prev[:hg, 8:16], cur[:hg, 8:16] + prev[:hg, 0:8]], axis=1)
            hi = jnp.concatenate(
                [cur[hg:, 0:8] + prev[hg:, 8:16], cur[hg:, 8:16] - prev[hg:, 0:8]], axis=1)
            return jnp.concatenate([lo, hi], axis=0)

        def qvproj(rb, carry):
            for cp in kvh_copies(rb):
                cp.wait()
            ssd = ssd_ref[...].astype(F32).reshape(1, D)
            shk = shk_ref[...].astype(F32)
            r0 = pl.multiple_of(rb * QB, QB)

            def q_part(rs):
                xb = x_v[pl.ds(rs, RB), :]
                qt = jax.lax.dot_general(wt_s[0:D, :], xb, NT, preferred_element_type=F32)
                qt = qt * qscale
                track(1, qt)
                qf = qt.astype(BF16).astype(F32).reshape(H // 2, 2 * DH, RB)
                row = jax.lax.broadcasted_iota(I32, (H // 2, 24, RB), 1)
                zpad = jnp.zeros((H // 2, 8, RB), F32)
                for par, win in ((0, jnp.where(row < DH, qf[:, 0:24], 0.0)),
                                 (1, jnp.where(row >= 4, qf[:, 16:40], 0.0))):
                    win = jnp.concatenate([win, zpad], axis=1).reshape(H // 2 * 32, RB)
                    qh_s[par, :, :, pl.ds(rs, RB)] = pltpu.bitcast(
                        win.astype(BF16), U32).reshape(H // 2, 16, RB)
                qf_s[:, :, pl.ds(rs, RB)] = qf
                for d in range(DH):
                    qb_s[0, d, :, pl.ds(rs, RB)] = jnp.broadcast_to(qf[0, d:d + 1, :], (8, RB))

            def v_part(rs):
                xb = x_v[pl.ds(rs, RB), :]
                vt = jax.lax.dot_general(wt_s[D:2 * D, :], xb, NT, preferred_element_type=F32)
                track(2, vt)
                vt = vt.astype(BF16).astype(F32).reshape(H // 2, 2 * DH, RB)
                row = jax.lax.broadcasted_iota(I32, (H // 2, 24, RB), 1)
                vt_s[0, :, :, pl.ds(rs, RB)] = jnp.where(row < DH, vt[:, 0:24, :], 1.0)
                vt_s[1, :, :, pl.ds(rs, RB)] = jnp.where(row >= 4, vt[:, 16:40, :], 1.0)

            def k_split(rs):
                h0 = pl.multiple_of(rs // 2, RB // 2)
                for j, part in enumerate(split_pairs(kn_s[pl.ds(h0, RB // 2), :])):
                    kp_s[j, pl.ds(h0, RB // 2), :] = part

            def u_part(u, ktail):
                ru = pl.multiple_of(r0 + u * BLK, BLK)
                kc = k_v[pl.ds(ru, BLK), :].astype(F32)
                e3 = jnp.concatenate([ktail, kc], axis=0).reshape(BLK // 8 + 1, 8, D)
                sub = jax.lax.broadcasted_iota(I32, (BLK // 8, 8, D), 1)
                ksh = kc * shk[0:1, :]
                for j in range(1, KS):
                    rot = pltpu.roll(e3, j, 1)
                    sh = jnp.where(sub >= j, rot[1:], rot[:-1]).reshape(BLK, D)
                    ksh = ksh + sh * shk[j:j + 1, :]
                kv = (ksh * v_v[pl.ds(ru, BLK), :].astype(F32)).astype(BF16)
                kv_s[pl.ds(ru, BLK), :] = kv.astype(F32) * ssd
                uf_s[:, rb * (QB // BLK) + u] = jnp.dot(
                    fwd_ref[...], kv, preferred_element_type=F32).reshape(NG, 16, D)
                return kc[BLK - 8:, :]

            def h_part(u, prev):
                ru = pl.multiple_of(r0 + u * BLK, BLK)
                raw = jax.lax.dot_general(fwd_ref[...], h_v[:, pl.ds(ru, BLK)], NT,
                                          preferred_element_type=F32)
                hf_s[:, rb * (QB // BLK) + u] = fold(raw, prev)
                return raw

            ktail = kf_s[0:8, :]
            prev = hp_s[...]
            for sub in range(QB // RB):
                rs = pl.multiple_of(r0 + sub * RB, RB)
                k_split(rs)
                q_part(rs)
                ktail = u_part(2 * sub, ktail)
                prev = h_part(2 * sub, prev)
                prev = h_part(2 * sub + 1, prev)
                if sub == QB // RB - 1:
                    hp_s[...] = prev
                v_part(rs)
                ktail = u_part(2 * sub + 1, ktail)
            kf_s[0:8, :] = ktail
            return carry

        jax.lax.fori_loop(0, NQB, qvproj, 0)

    pl.run_scoped(
        pre_phase,
        pltpu.VMEM((S, D), BF16),
        pltpu.VMEM((D, S), BF16),
        pltpu.VMEM((D, 3 * D), BF16),
        pltpu.VMEM((2 * D, D), BF16),
        pltpu.VMEM((32, D), F32),
        pltpu.VMEM((2 * BLK, D), F32),
        pltpu.VMEM((S // 2, D), U32),
        pltpu.VMEM((2 * BLK, BLK), BF16),
        pltpu.VMEM((KS, D), BF16),
        pltpu.VMEM((D,), BF16),
        pltpu.VMEM((D,), BF16),
    )

    def post_phase(s2, m2, zf_s, ot_s, ss):
        def freq_steps(g, chunks):
            steps = []
            for c in chunks:
                cols = slice(c * 128, (c + 1) * 128) if isinstance(c, int) else c
                for i in range(NB):
                    st = {}
                    for m0 in range(0, i + 1, FE):
                        ms = list(range(m0, min(i + 1, m0 + FE)))

                        def step(anchor, i=i, cols=cols, ms=ms, st=st):
                            for m in ms:
                                ur = uf_s[g, m, 0:8, cols]
                                ui = uf_s[g, m, 8:16, cols]
                                hr = hf_s[g, i - m, 0:8, cols]
                                hi = hf_s[g, i - m, 8:16, cols]
                                if m == ms[0]:
                                    ur = anchor(ur)
                                tr = ur * hr - ui * hi
                                ti = ur * hi + ui * hr
                                st["r"] = tr if m == 0 else st["r"] + tr
                                st["i"] = ti if m == 0 else st["i"] + ti
                            if ms[-1] == i:
                                zf_s[g, i, 0:8, cols] = st["r"]
                                zf_s[g, i, 8:16, cols] = st["i"]
                        steps.append((len(ms), step))
            return steps

        kmax = jnp.max(bd_s[0])
        qmax = jnp.max(bd_s[1])
        vmax = jnp.max(bd_s[2])
        live = jnp.logical_not(kmax < 0.0)

        def tie_to(tie):
            def anchor(v):
                t = tie if tie.dtype == v.dtype else pltpu.bitcast(tie, v.dtype)
                if v.shape[0] > 8:
                    t = jnp.concatenate([t] * (v.shape[0] // 8), axis=0)
                return jnp.where(live, v, t)
            return anchor

        def stage(h_qk, par_qk, h_pv, fsteps):
            par_pv = 1 - par_qk
            mr = SM // NC
            jq = h_qk >> 1
            j_nx = 0 if isinstance(h_qk, int) else jnp.minimum(h_qk + 1, H - 1) >> 1
            ftl = _timeline(fsteps, 0, NU - 0.5)

            def prep_q(anchor, t):
                tc = slice(t * 128, (t + 1) * 128)
                blk = anchor(qf_s[j_nx, par_pv * 16:par_pv * 16 + 24, tc])
                for d in range(DH):
                    rr = par_pv * 4 + d
                    qb_s[par_pv, d, :, tc] = jnp.broadcast_to(blk[rr:rr + 1, :], (8, 128))

            psteps = []
            for i in range(DH):
                psteps.append((1, lambda anchor, i=i: build_kb(j_nx, par_pv, i, anchor)))
                if i < S // 128:
                    psteps.append((1, lambda anchor, i=i: prep_q(anchor, i)))
            ptl = _timeline(psteps, 0, NU * 0.9)
            if h_pv is not None:
                j = h_pv >> 1
            for sb in range(NSB):
                cols = slice(sb * SB, (sb + 1) * SB)
                vsteps = []
                for kg in range(R // PK):
                    for qq in range(SB // PQ):
                        st = {}
                        for d0 in range(0, DH, AE):
                            def step(anchor, kg=kg, qq=qq, d0=d0, st=st, sb=sb):
                                q0 = sb * SB + qq * PQ
                                for d in range(d0, d0 + AE):
                                    kb = kb_s[par_qk, d, kg * PK:(kg + 1) * PK, :]
                                    if d == d0:
                                        kb = anchor(kb)
                                    qr = qb_s[par_qk, d, :, q0:q0 + PQ]
                                    t = (jnp.concatenate([kb] * (PQ // 128), axis=1)
                                         * jnp.concatenate([qr] * (PK // 8), axis=0))
                                    st["a"] = t if d == 0 else st["a"] + t
                                if d0 + AE == DH:
                                    s2[par_qk, SM + kg * PK:SM + (kg + 1) * PK,
                                       q0:q0 + PQ] = jnp.exp2(st["a"])
                            vsteps.append((1, step))
                vtl = _timeline(vsteps, 0, NC - 0.25)
                acc = None
                for c in range(NC):
                    u = sb * NC + c
                    kc = pltpu.bitcast(kp_s[jq, c * mr // 2:(c + 1) * mr // 2, :], BF16)
                    qt = qh_s[par_qk, jq, :, cols]
                    if par_qk == 1:
                        qt = jnp.concatenate([jnp.zeros((8, SB), U32), qt], axis=0)
                    qt = pltpu.bitcast(qt, BF16)
                    s = jnp.dot(kc[:, 0:qt.shape[0]], qt, preferred_element_type=F32)
                    s2[par_qk, c * mr:(c + 1) * mr, cols] = jnp.exp2(s)
                    ties = s
                    if h_pv is not None:
                        r = jnp.dot(vt_s[par_pv, j, :, c * CK:(c + 1) * CK],
                                    s2[par_pv, c * CK:(c + 1) * CK, cols],
                                    preferred_element_type=F32)
                        if acc is None:
                            z = tie_to(s[0:8, 0:128])(jnp.zeros((8, 128), F32))
                            z = jnp.concatenate([z] * 3, axis=0)
                            acc = jnp.concatenate([z] * (SB // 128), axis=1)
                        acc = acc + r
                        if u < NU - 1:
                            ties = jnp.concatenate([s, r], axis=0)
                    ng = ties.shape[0] // 8
                    for col, tl in ((0, vtl.get(c, [])), (1, ptl.get(u, [])), (2, ftl.get(u, []))):
                        for frac, p in tl:
                            gi = min(ng - 1, int(frac * ng))
                            p(tie_to(ties[gi * 8:(gi + 1) * 8, col * 128:(col + 1) * 128]))
                if h_pv is not None:
                    ot_s[par_pv, j, :, cols] = acc

        def fast_path():
            stage(0, 0, None, freq_steps(0, (0, 1)))

            def body(t, carry):
                @pl.when((t & 1) == 1)
                def _():
                    stage(t, 1, t - 1, freq_steps(t >> 1, (2, 3, 4)))

                @pl.when((t & 1) == 0)
                def _():
                    stage(t, 0, t - 1, freq_steps(t >> 1, (0, 1)))
                return carry

            jax.lax.fori_loop(1, H, body, 0)

        def slow_path():
            nq = S // SQ

            def block(it_qk, it_pv, wbuf):
                rbuf = 1 - wbuf
                h = it_qk // nq
                c0 = pl.multiple_of((it_qk % nq) * SQ, SQ)
                q32 = qh_s[h & 1, h >> 1, :, pl.ds(c0, SQ)]
                z = jnp.zeros((8, SQ), U32)
                qt = pltpu.bitcast(jnp.where((h & 1) == 1, jnp.concatenate([z, q32], axis=0),
                                             jnp.concatenate([q32, z], axis=0)), BF16)
                hp = it_pv // nq
                cp = pl.multiple_of((it_pv % nq) * SQ, SQ)
                m = jnp.max(m2[rbuf], axis=0, keepdims=True)
                mx = None
                acc = None
                for c in range(S // SQ):
                    rows = slice(c * SQ, (c + 1) * SQ)
                    kc = pltpu.bitcast(kp_s[h >> 1, c * SQ // 2:(c + 1) * SQ // 2, :], BF16)
                    s = jnp.dot(kc[:, 0:48], qt, preferred_element_type=F32)
                    ss[wbuf, rows, :] = s
                    cm = jnp.max(s.reshape(SQ // 8, 8, SQ), axis=0)
                    mx = cm if mx is None else jnp.maximum(mx, cm)
                    p = jnp.exp2(ss[rbuf, rows, :] - m)
                    s2[1, rows, pl.ds(cp, SQ)] = p
                    r = jnp.dot(vt_s[hp & 1, hp >> 1, :, rows], p, preferred_element_type=F32)
                    acc = r if acc is None else acc + r
                m2[wbuf] = mx
                ot_s[hp & 1, hp >> 1, :, pl.ds(cp, SQ)] = acc

            ss[1] = jnp.zeros((S, SQ), F32)
            m2[1] = jnp.zeros((8, SQ), F32)

            def body(it, carry):
                cur = jnp.minimum(it, H * nq - 1)
                prv = jnp.maximum(it - 1, 0)

                @pl.when((it & 1) == 0)
                def _():
                    block(cur, prv, 0)

                @pl.when((it & 1) == 1)
                def _():
                    block(cur, prv, 1)
                return carry

            jax.lax.fori_loop(0, H * nq + 1, body, 0)

            def fbody(i, carry):
                cols = pl.ds(pl.multiple_of((i % NCH) * 128, 128), 128)
                for _, p in freq_steps(i // NCH, (cols,)):
                    p(lambda v: v)
                return carry

            jax.lax.fori_loop(0, NG * NCH, fbody, 0)

        safe = jnp.logical_and(
            kmax * qmax * (1.02 * DH) <= SCORE_BOUND,
            jnp.logical_and(vmax <= 2.0 ** 30, vmax >= 2.0 ** -20))

        @pl.when(safe)
        def _():
            fast_path()

        @pl.when(jnp.logical_not(safe))
        def _():
            slow_path()

        cp_inv.wait()
        cp_wo.wait()
        nb = SB // BLK
        for sb in range(NSB):
            c0 = sb * SB
            acc = None
            ga = []
            for c in range(NC):
                r = jnp.dot(vt_s[1, H // 2 - 1, :, c * CK:(c + 1) * CK],
                            s2[1, c * CK:(c + 1) * CK, c0:c0 + SB], preferred_element_type=F32)
                acc = r if acc is None else acc + r
                if c % (NC // nb) == 0:
                    i = sb * nb + c // (NC // nb)
                    rows = slice(i * BLK, (i + 1) * BLK)
                    y = jnp.dot(inv_ref[...], zf_s[:, i].reshape(2 * BLK, D),
                                preferred_element_type=F32)
                    gx = x_v[rows, :].astype(F32) * jnp.concatenate([g_s[rows, :]] * NCH, axis=1)
                    ga.append(gx * (y + kv_s[rows, :]))
            for i in range(SB // FB):
                rows = slice(c0 + i * FB, c0 + (i + 1) * FB)
                oe = ot_s[0, :, :, rows]
                oo = jnp.concatenate([ot_s[1, 0:H // 2 - 1, :, rows],
                                      acc[None, :, i * FB:(i + 1) * FB]], axis=0)
                low = jax.lax.broadcasted_iota(I32, (H // 2, 8, FB), 1) < 4
                den = jnp.where(low, oo[:, 0:8], oe[:, 16:24])
                inv = pl.reciprocal(den, approx=True)
                inv = inv * (2.0 - den * inv)
                o = jnp.concatenate(
                    [oe[:, 0:16] * inv[:, 4:5],
                     jnp.where(low, oe[:, 16:24], oo[:, 0:8]) * pltpu.roll(inv, 4, 1),
                     oo[:, 8:24] * inv[:, 0:1]], axis=1)
                o = o.reshape(D, FB).T.astype(BF16)
                bb = jnp.dot(o, wo_v[...], preferred_element_type=F32)
                g1 = 1.0 - g_s[rows, :]
                out_v[rows, :] = (ga[i] + jnp.concatenate([g1] * NCH, axis=1) * bb).astype(BF16)
                pltpu.make_async_copy(out_v.at[rows, :], out_hbm.at[0, rows, :],
                                      sems.at[SEM_OUT]).start()
        pltpu.make_async_copy(out_v, out_hbm.at[0], sems.at[SEM_OUT]).wait()

    pl.run_scoped(
        post_phase,
        pltpu.VMEM((2, S, S), F32),
        pltpu.VMEM((2, 8, SQ), F32),
        pltpu.VMEM((NG, NB, 16, D), F32),
        pltpu.VMEM((2, H // 2, 24, S), F32),
        pltpu.VMEM((2, S, SQ), F32),
    )


@jax.jit
def pallas_gated_mix__ssm_conv_h3__mha_block__prompt_kernel(
    A_q: jax.Array,
    A_k: jax.Array,
    A_v: jax.Array,
    A_shift_k: jax.Array,
    A_ssm_k: jax.Array,
    A_ssm_D: jax.Array,
    B_x: jax.Array,
    B_wqkv: jax.Array,
    B_wo: jax.Array,
    gate_w: jax.Array,
):
    fwd, inv = _dft_consts()
    fwd = jnp.asarray(fwd, dtype=BF16)
    inv = jnp.asarray(inv, dtype=BF16).astype(F32)
    hbm = pl.BlockSpec(memory_space=pl.ANY)
    scratch = [
        pltpu.VMEM((S, D), BF16),
        pltpu.VMEM((S, D), BF16),
        pltpu.VMEM((D, D), BF16),
        pltpu.VMEM((H // 2, S // 2, 128), U32),
        pltpu.VMEM((2, H // 2, 16, S), U32),
        pltpu.VMEM((2, H // 2, 24, S), F32),
        pltpu.VMEM((S, D), F32),
        pltpu.VMEM((S, 128), F32),
        pltpu.VMEM((NG, NB, 16, D), F32),
        pltpu.VMEM((NG, NB, 16, D), F32),
        pltpu.VMEM((H // 2, R, 128), F32),
        pltpu.VMEM((2, DH, R, 128), F32),
        pltpu.VMEM((H // 2, 2 * DH, S), F32),
        pltpu.VMEM((2, DH, 8, S), F32),
        pltpu.VMEM((4, 8, 128), F32),
        pltpu.VMEM((BLK, 2 * BLK), F32),
        pltpu.SemaphoreType.DMA((NSEM,)),
    ]
    return pl.pallas_call(
        _kernel,
        out_shape=jax.ShapeDtypeStruct((1, S, D), BF16),
        in_specs=[hbm] * 11,
        out_specs=hbm,
        scratch_shapes=scratch,
        compiler_params=pltpu.CompilerParams(vmem_limit_bytes=127 * 1024 * 1024),
    )(A_q, A_k, A_v, A_shift_k.T, A_ssm_k, A_ssm_D, B_wqkv, B_wo, gate_w, fwd, inv)
```

```python
import math

import jax
import jax.numpy as jnp
import numpy as np
import jax.experimental.pallas as pl
import jax.experimental.pallas.tpu as pltpu

S = 2048
D = 640
H = 32
DH = 20
KS = 4
NCH = D // 128
BLK = 128
NB = S // BLK
NG = BLK // 8
CK = 128
SB = 512
NC = S // CK
NSB = S // SB
NU = NC * NSB
RB = 256
NRB = S // RB
NPEEL = 3
QB = 512
NQB = S // QB
R = 288
R0 = 256
SM = S - R
PK, PQ = 32, 256
AE = 3
FE = 2
SQ = 256
SCORE_BOUND = 80.0
F32 = jnp.float32
BF16 = jnp.bfloat16
U32 = jnp.uint32
I32 = jnp.int32
NT = (((1,), (1,)), ((), ()))

SEM_WK, SEM_WQ, SEM_WV, SEM_WO, SEM_OUT = 0, 1, 2, 3, 4
SEM_GW, SEM_SHK, SEM_SSD, SEM_FWD, SEM_INV = 5, 6, 7, 8, 9
SEM_X = 10
SEM_K = SEM_X + NRB
SEM_V = SEM_K + NQB
SEM_H = SEM_V + NQB
NSEM = SEM_H + NQB


def _dft_consts():
    f = np.concatenate([np.arange(0, BLK, 2), np.arange(1, BLK, 2)]).astype(np.float64)
    n = np.arange(BLK, dtype=np.float64)
    ang = 2.0 * np.pi * (f[:, None] + 0.5) * n[None, :] / (2 * BLK)
    re = np.cos(ang).reshape(NG, 8, BLK)
    im = -np.sin(ang).reshape(NG, 8, BLK)
    fwd = np.concatenate([re, im], axis=1).reshape(2 * BLK, BLK)
    inv = fwd.T / BLK
    return fwd, inv


def _timeline(steps, t1, edges):
    total = sum(w for w, _ in steps)
    out = {}
    acc = 0
    for w, p in steps:
        cyc = t1 * acc / total / NU * edges[-1]
        acc += w
        u = max(i for i in range(NU) if edges[i] <= cyc)
        out.setdefault(u, []).append(((cyc - edges[u]) / (edges[u + 1] - edges[u]), p))
    return out


def _kernel(x_hbm, k_hbm, v_hbm, shk_hbm, h_hbm, ssd_hbm, w_hbm, wo_hbm, gw_hbm,
            fwd_hbm, inv_hbm, out_hbm,
            x_v, k_v, wo_v, kp_s, qh_s, vt_s, kv_s, g_s, uf_s, hf_s,
            kfp, kb_s, qf_s, qb_s, bd_s, inv_ref, fl_s, sems):
    out_v = k_v
    cp_wo = pltpu.make_async_copy(wo_hbm, wo_v, sems.at[SEM_WO])
    cp_inv = pltpu.make_async_copy(inv_hbm, inv_ref, sems.at[SEM_INV])

    def build_kb(j, par, d, anchor=None, lo=0):
        t = jnp.full((8, 128), par * DH + d, I32)
        if anchor is not None:
            t = anchor(t) & 127
        idx = jnp.concatenate([t] * ((R - lo) // 8), axis=0)
        kb_s[par, d, lo:R, :] = jnp.take_along_axis(
            kfp[j, lo:R, :], idx, axis=1, mode="promise_in_bounds")

    def pre_phase(v_v, h_v, w_v, wt_s, kf_s, hp_s, kn_s, fwd_ref, shk_ref, ssd_ref, gw_ref):
        def w_copy(part, sem):
            return pltpu.make_async_copy(w_hbm.at[:, part * D:(part + 1) * D],
                                         w_v.at[:, part * D:(part + 1) * D], sems.at[sem])

        def x_copy(i):
            r0 = pl.multiple_of(i * RB, RB)
            return pltpu.make_async_copy(x_hbm.at[0, pl.ds(r0, RB), :],
                                         x_v.at[pl.ds(r0, RB), :], sems.at[SEM_X + i])

        def kvh_copies(i):
            r0 = pl.multiple_of(i * QB, QB)
            return (
                pltpu.make_async_copy(k_hbm.at[0, pl.ds(r0, QB), :],
                                      k_v.at[pl.ds(r0, QB), :], sems.at[SEM_K + i]),
                pltpu.make_async_copy(v_hbm.at[0, pl.ds(r0, QB), :],
                                      v_v.at[pl.ds(r0, QB), :], sems.at[SEM_V + i]),
                pltpu.make_async_copy(h_hbm.at[:, pl.ds(r0, QB)],
                                      h_v.at[:, pl.ds(r0, QB)], sems.at[SEM_H + i]),
            )

        cp_gw = pltpu.make_async_copy(gw_hbm, gw_ref, sems.at[SEM_GW])
        cp_small = (
            pltpu.make_async_copy(shk_hbm, shk_ref, sems.at[SEM_SHK]),
            pltpu.make_async_copy(ssd_hbm, ssd_ref, sems.at[SEM_SSD]),
            pltpu.make_async_copy(fwd_hbm, fwd_ref, sems.at[SEM_FWD]),
        )
        x_copy(0).start()
        w_copy(1, SEM_WK).start()
        cp_gw.start()
        for i in range(1, NRB):
            x_copy(i).start()
        for cp in cp_small:
            cp.start()
        w_copy(0, SEM_WQ).start()
        w_copy(2, SEM_WV).start()
        for i in range(NQB):
            for cp in kvh_copies(i):
                cp.start()
        cp_wo.start()
        cp_inv.start()

        kf_s[0:8, :] = jnp.zeros((8, D), F32)
        hp_s[...] = jnp.zeros((2 * BLK, D), F32)
        bd_s[...] = jnp.zeros((4, 8, 128), F32)

        def track(i, val):
            a = jnp.abs(val)
            a = jnp.max(a.reshape(a.shape[0] // 8, 8, a.shape[1]), axis=0)
            m = bd_s[i]
            for c in range(a.shape[1] // 128):
                m = jnp.maximum(m, a[:, c * 128:(c + 1) * 128])
            bd_s[i] = m

        def split_pairs(val):
            lane = jax.lax.broadcasted_iota(I32, (val.shape[0], 128), 1)
            parts = [val[:, c * 128:(c + 1) * 128] for c in range(NCH)]
            out = []
            for j in range(H // 2):
                c, sh = divmod(2 * DH * j, 128)
                src = parts[c]
                if sh + 2 * DH > 128:
                    src = jnp.where(lane >= 64, src, parts[c + 1])
                out.append(pltpu.roll(src, 128 - sh, 1) if sh else src)
            return out

        def kproj(rb):
            r0 = pl.multiple_of(rb * RB, RB)
            xb = x_v[pl.ds(r0, RB), :]
            kk = jnp.dot(xb, w_v[:, D:2 * D], preferred_element_type=F32)
            track(0, kk)
            kp = pltpu.bitcast(kk.astype(BF16), U32)
            h0 = pl.multiple_of(rb * (RB // 2), RB // 2)
            kn_s[pl.ds(h0, RB // 2), :] = kp
            if isinstance(rb, int) and (rb + 1) * RB > SM:
                lo = max(SM, rb * RB)
                for j, part in enumerate(split_pairs(kp[(lo - rb * RB) // 2:, :])):
                    kfp[j, lo - SM:(rb + 1) * RB - SM, :] = pltpu.bitcast(part, BF16).astype(F32)
            gw = gw_ref[...].astype(F32).reshape(1, D)
            g = jax.nn.sigmoid(jnp.sum(xb.astype(F32) * gw, axis=-1, keepdims=True))
            g_s[pl.ds(r0, RB), :] = jnp.broadcast_to(g, (RB, 128))

        w_copy(1, SEM_WK).wait()
        cp_gw.wait()

        def kproj_loop(rb, carry):
            x_copy(rb).wait()
            kproj(rb)
            return carry

        jax.lax.fori_loop(0, NRB - NPEEL, kproj_loop, 0)
        for i in range(NRB - NPEEL, NRB):
            x_copy(i).wait()
        w_copy(0, SEM_WQ).wait()
        w_copy(2, SEM_WV).wait()
        for cp in cp_small:
            cp.wait()
        fl_s[0] = jnp.max(bd_s[0])
        kproj(NRB - 1)
        wt_s[0:D, :] = w_v[:, 0:D].astype(F32).T.astype(BF16)
        wt_s[D:2 * D, :] = w_v[:, 2 * D:3 * D].astype(F32).T.astype(BF16)
        for i in range(NRB - 2, NRB - NPEEL - 1, -1):
            kproj(i)
        for d in range(DH):
            build_kb(0, 0, d, lo=R - R0)

        qscale = (DH ** -0.5) * math.log2(math.e)

        def fold(cur, prev):
            cur = cur.reshape(NG, 16, D)
            prev = prev.reshape(NG, 16, D)
            hg = NG // 2
            lo = jnp.concatenate(
                [cur[:hg, 0:8] - prev[:hg, 8:16], cur[:hg, 8:16] + prev[:hg, 0:8]], axis=1)
            hi = jnp.concatenate(
                [cur[hg:, 0:8] + prev[hg:, 8:16], cur[hg:, 8:16] - prev[hg:, 0:8]], axis=1)
            return jnp.concatenate([lo, hi], axis=0)

        def qvproj(rb, carry):
            for cp in kvh_copies(rb):
                cp.wait()
            ssd = ssd_ref[...].astype(F32).reshape(1, D)
            shk = shk_ref[...].astype(F32)
            r0 = pl.multiple_of(rb * QB, QB)

            def q_part(rs):
                xb = x_v[pl.ds(rs, RB), :]
                qt = jax.lax.dot_general(wt_s[0:D, :], xb, NT, preferred_element_type=F32)
                qt = qt * qscale
                track(1, qt)
                qf = qt.astype(BF16).astype(F32).reshape(H // 2, 2 * DH, RB)
                row = jax.lax.broadcasted_iota(I32, (H // 2, 24, RB), 1)
                zpad = jnp.zeros((H // 2, 8, RB), F32)
                for par, win in ((0, jnp.where(row < DH, qf[:, 0:24], 0.0)),
                                 (1, jnp.where(row >= 4, qf[:, 16:40], 0.0))):
                    win = jnp.concatenate([win, zpad], axis=1).reshape(H // 2 * 32, RB)
                    qh_s[par, :, :, pl.ds(rs, RB)] = pltpu.bitcast(
                        win.astype(BF16), U32).reshape(H // 2, 16, RB)
                qf_s[:, :, pl.ds(rs, RB)] = qf
                for d in range(DH):
                    qb_s[0, d, :, pl.ds(rs, RB)] = jnp.broadcast_to(qf[0, d:d + 1, :], (8, RB))

            def v_part(rs):
                xb = x_v[pl.ds(rs, RB), :]
                vt = jax.lax.dot_general(wt_s[D:2 * D, :], xb, NT, preferred_element_type=F32)
                track(2, vt)
                vt = vt.astype(BF16).astype(F32).reshape(H // 2, 2 * DH, RB)
                row = jax.lax.broadcasted_iota(I32, (H // 2, 24, RB), 1)
                vt_s[0, :, :, pl.ds(rs, RB)] = jnp.where(row < DH, vt[:, 0:24, :], 1.0)
                vt_s[1, :, :, pl.ds(rs, RB)] = jnp.where(row >= 4, vt[:, 16:40, :], 1.0)

            def k_split(rs):
                h0 = pl.multiple_of(rs // 2, RB // 2)
                for j, part in enumerate(split_pairs(kn_s[pl.ds(h0, RB // 2), :])):
                    kp_s[j, pl.ds(h0, RB // 2), :] = part

            def u_part(u, ktail):
                ru = pl.multiple_of(r0 + u * BLK, BLK)
                kc = k_v[pl.ds(ru, BLK), :].astype(F32)
                e3 = jnp.concatenate([ktail, kc], axis=0).reshape(BLK // 8 + 1, 8, D)
                sub = jax.lax.broadcasted_iota(I32, (BLK // 8, 8, D), 1)
                ksh = kc * shk[0:1, :]
                for j in range(1, KS):
                    rot = pltpu.roll(e3, j, 1)
                    sh = jnp.where(sub >= j, rot[1:], rot[:-1]).reshape(BLK, D)
                    ksh = ksh + sh * shk[j:j + 1, :]
                kv = (ksh * v_v[pl.ds(ru, BLK), :].astype(F32)).astype(BF16)
                kv_s[pl.ds(ru, BLK), :] = kv.astype(F32) * ssd
                uf_s[:, rb * (QB // BLK) + u] = jnp.dot(
                    fwd_ref[...], kv, preferred_element_type=F32).reshape(NG, 16, D)
                return kc[BLK - 8:, :]

            def h_part(u, prev):
                ru = pl.multiple_of(r0 + u * BLK, BLK)
                raw = jax.lax.dot_general(fwd_ref[...], h_v[:, pl.ds(ru, BLK)], NT,
                                          preferred_element_type=F32)
                hf_s[:, rb * (QB // BLK) + u] = fold(raw, prev)
                return raw

            ktail = kf_s[0:8, :]
            prev = hp_s[...]
            for sub in range(QB // RB):
                rs = pl.multiple_of(r0 + sub * RB, RB)
                k_split(rs)
                q_part(rs)
                ktail = u_part(2 * sub, ktail)
                prev = h_part(2 * sub, prev)
                prev = h_part(2 * sub + 1, prev)
                if sub == QB // RB - 1:
                    hp_s[...] = prev
                v_part(rs)
                ktail = u_part(2 * sub + 1, ktail)
            kf_s[0:8, :] = ktail
            return carry

        jax.lax.fori_loop(0, NQB, qvproj, 0)

    pl.run_scoped(
        pre_phase,
        pltpu.VMEM((S, D), BF16),
        pltpu.VMEM((D, S), BF16),
        pltpu.VMEM((D, 3 * D), BF16),
        pltpu.VMEM((2 * D, D), BF16),
        pltpu.VMEM((32, D), F32),
        pltpu.VMEM((2 * BLK, D), F32),
        pltpu.VMEM((S // 2, D), U32),
        pltpu.VMEM((2 * BLK, BLK), BF16),
        pltpu.VMEM((KS, D), BF16),
        pltpu.VMEM((D,), BF16),
        pltpu.VMEM((D,), BF16),
    )

    def post_phase(s2, m2, zf_s, ot_s, ss):
        def freq_steps(g, chunks):
            steps = []
            for c in chunks:
                cols = slice(c * 128, (c + 1) * 128) if isinstance(c, int) else c
                for i in range(NB):
                    st = {}
                    for m0 in range(0, i + 1, FE):
                        ms = list(range(m0, min(i + 1, m0 + FE)))

                        def step(anchor, i=i, cols=cols, ms=ms, st=st):
                            for m in ms:
                                ur = uf_s[g, m, 0:8, cols]
                                ui = uf_s[g, m, 8:16, cols]
                                hr = hf_s[g, i - m, 0:8, cols]
                                hi = hf_s[g, i - m, 8:16, cols]
                                if m == ms[0]:
                                    ur = anchor(ur)
                                tr = ur * hr - ui * hi
                                ti = ur * hi + ui * hr
                                st["r"] = tr if m == 0 else st["r"] + tr
                                st["i"] = ti if m == 0 else st["i"] + ti
                            if ms[-1] == i:
                                zf_s[g, i, 0:8, cols] = st["r"]
                                zf_s[g, i, 8:16, cols] = st["i"]
                        steps.append((len(ms), step))
            return steps

        kmax = jnp.max(bd_s[0])
        qmax = jnp.max(bd_s[1])
        vmax = jnp.max(bd_s[2])
        live = jnp.logical_not(fl_s[0] < 0.0)

        def tie_to(tie):
            def anchor(v):
                t = tie if tie.dtype == v.dtype else pltpu.bitcast(tie, v.dtype)
                if v.shape[0] > 8:
                    t = jnp.concatenate([t] * (v.shape[0] // 8), axis=0)
                return jnp.where(live, v, t)
            return anchor

        def stage(h_qk, par_qk, h_pv, fsteps, rv=R):
            par_pv = 1 - par_qk
            bounds = [min(S - rv, (((S - rv) * c // NC) + 15) // 16 * 16) for c in range(NC + 1)]
            jq = h_qk >> 1
            j_nx = 0 if isinstance(h_qk, int) else jnp.minimum(h_qk + 1, H - 1) >> 1
            edges = [0]
            for u in range(NU):
                edges.append(edges[-1] + bounds[u % NC + 1] - bounds[u % NC]
                             + (24 if h_pv is not None else 0))
            ftl = _timeline(fsteps, NU * (1 - 0.008), edges)

            def prep_q(anchor, t):
                tc = slice(t * 128, (t + 1) * 128)
                blk = anchor(qf_s[j_nx, par_pv * 16:par_pv * 16 + 24, tc])
                for d in range(DH):
                    rr = par_pv * 4 + d
                    qb_s[par_pv, d, :, tc] = jnp.broadcast_to(blk[rr:rr + 1, :], (8, 128))

            psteps = []
            for i in range(DH):
                psteps.append((1, lambda anchor, i=i: build_kb(j_nx, par_pv, i, anchor)))
                if i < S // 128:
                    psteps.append((1, lambda anchor, i=i: prep_q(anchor, i)))
            ptl = _timeline(psteps, NU * (1 - 0.06), edges)
            if h_pv is not None:
                j = h_pv >> 1

            vsteps = []
            for sb in range(NSB):
                for k0 in range(R - rv, R, PK):
                    for qq in range(SB // PQ):
                        st = {}
                        for d0 in range(0, DH, AE):
                            def step(anchor, k0=k0, q0=sb * SB + qq * PQ, d0=d0, st=st):
                                for d in range(d0, min(DH, d0 + AE)):
                                    kb = kb_s[par_qk, d, k0:k0 + PK, :]
                                    if d == d0:
                                        w = (d0 // AE) % (PK // 8)
                                        kb = jnp.concatenate(
                                            [anchor(kb[i * 8:(i + 1) * 8]) if i == w
                                             else kb[i * 8:(i + 1) * 8]
                                             for i in range(PK // 8)], axis=0)
                                    qr = qb_s[par_qk, d, :, q0:q0 + PQ]
                                    t = (jnp.concatenate([kb] * (PQ // 128), axis=1)
                                         * jnp.concatenate([qr] * (PK // 8), axis=0))
                                    st["a"] = t if d == 0 else st["a"] + t
                                if d0 + AE >= DH:
                                    s2[par_qk, SM + k0:SM + k0 + PK,
                                       q0:q0 + PQ] = jnp.exp2(st["a"])
                            vsteps.append((min(DH, d0 + AE) - d0, step))
            vtl = _timeline(vsteps, NU - 0.25, edges)

            acc = None
            for sb in range(NSB):
                cols = slice(sb * SB, (sb + 1) * SB)
                for c in range(NC):
                    u = sb * NC + c
                    r0, r1 = bounds[c], bounds[c + 1]
                    kc = pltpu.bitcast(kp_s[jq, r0 // 2:r1 // 2, :], BF16)
                    qt = qh_s[par_qk, jq, :, cols]
                    if par_qk == 1:
                        qt = jnp.concatenate([jnp.zeros((8, SB), U32), qt], axis=0)
                    qt = pltpu.bitcast(qt, BF16)
                    s = jnp.dot(kc[:, 0:qt.shape[0]], qt, preferred_element_type=F32)
                    s2[par_qk, r0:r1, cols] = jnp.exp2(s)
                    ties = s
                    if h_pv is not None:
                        ct, kq = divmod(u, NSB)
                        pc = slice(ct * 128, (ct + 1) * 128)
                        rs = [jnp.dot(vt_s[par_pv, j, :, kq * SB + i * CK:kq * SB + (i + 1) * CK],
                                      s2[par_pv, kq * SB + i * CK:kq * SB + (i + 1) * CK, pc],
                                      preferred_element_type=F32) for i in range(SB // CK)]
                        if kq == 0:
                            z = tie_to(s[0:8, 0:128])(jnp.zeros((8, 128), F32))
                            acc = jnp.concatenate([z] * 3, axis=0)
                        for rr in rs:
                            acc = acc + rr
                        if kq == NSB - 1:
                            ot_s[par_pv, j, :, pc] = acc
                        if u < NU - 1:
                            ties = jnp.concatenate([s, jnp.concatenate(rs, axis=1)], axis=0)
                    ng = ties.shape[0] // 8
                    for col, tl in ((0, vtl.get(u, [])), (1, ptl.get(u, [])), (2, ftl.get(u, []))):
                        for frac, p in tl:
                            gi = min(ng - 1, int(frac * ng))
                            p(tie_to(ties[gi * 8:(gi + 1) * 8, col * 128:(col + 1) * 128]))

        def fast_path():
            def body(t, carry):
                @pl.when((t & 1) == 1)
                def _():
                    stage(t, 1, t - 1, freq_steps(t >> 1, (2, 3, 4)))

                @pl.when((t & 1) == 0)
                def _():
                    stage(t, 0, t - 1, freq_steps(t >> 1, (0, 1)))
                return carry

            jax.lax.fori_loop(1, H, body, 0)

        def slow_path():
            nq = S // SQ

            def block(it_qk, it_pv, wbuf):
                rbuf = 1 - wbuf
                h = it_qk // nq
                c0 = pl.multiple_of((it_qk % nq) * SQ, SQ)
                q32 = qh_s[h & 1, h >> 1, :, pl.ds(c0, SQ)]
                z = jnp.zeros((8, SQ), U32)
                qt = pltpu.bitcast(jnp.where((h & 1) == 1, jnp.concatenate([z, q32], axis=0),
                                             jnp.concatenate([q32, z], axis=0)), BF16)
                hp = it_pv // nq
                cp = pl.multiple_of((it_pv % nq) * SQ, SQ)
                m = jnp.max(m2[rbuf], axis=0, keepdims=True)
                mx = None
                acc = None
                for c in range(S // SQ):
                    rows = slice(c * SQ, (c + 1) * SQ)
                    kc = pltpu.bitcast(kp_s[h >> 1, c * SQ // 2:(c + 1) * SQ // 2, :], BF16)
                    s = jnp.dot(kc[:, 0:48], qt, preferred_element_type=F32)
                    ss[wbuf, rows, :] = s
                    cm = jnp.max(s.reshape(SQ // 8, 8, SQ), axis=0)
                    mx = cm if mx is None else jnp.maximum(mx, cm)
                    p = jnp.exp2(ss[rbuf, rows, :] - m)
                    s2[1, rows, pl.ds(cp, SQ)] = p
                    r = jnp.dot(vt_s[hp & 1, hp >> 1, :, rows], p, preferred_element_type=F32)
                    acc = r if acc is None else acc + r
                m2[wbuf] = mx
                ot_s[hp & 1, hp >> 1, :, pl.ds(cp, SQ)] = acc

            ss[1] = jnp.zeros((S, SQ), F32)
            m2[1] = jnp.zeros((8, SQ), F32)

            def body(it, carry):
                cur = jnp.minimum(it, H * nq - 1)
                prv = jnp.maximum(it - 1, 0)

                @pl.when((it & 1) == 0)
                def _():
                    block(cur, prv, 0)

                @pl.when((it & 1) == 1)
                def _():
                    block(cur, prv, 1)
                return carry

            jax.lax.fori_loop(0, H * nq + 1, body, 0)

            def fbody(i, carry):
                cols = pl.ds(pl.multiple_of((i % NCH) * 128, 128), 128)
                for _, p in freq_steps(i // NCH, (cols,)):
                    p(lambda v: v)
                return carry

            jax.lax.fori_loop(0, NG * NCH, fbody, 0)

        safe = jnp.logical_and(
            kmax * qmax * (1.02 * DH) <= SCORE_BOUND,
            jnp.logical_and(vmax <= 2.0 ** 30, vmax >= 2.0 ** -20))

        stage(0, 0, None, freq_steps(0, (0, 1)), rv=R0)

        jax.lax.cond(safe, fast_path, slow_path)

        cp_inv.wait()
        cp_wo.wait()
        accs = [None] * NSB
        ga = {}

        def pv_last(sb, c):
            cols = slice(sb * SB, (sb + 1) * SB)
            r = jnp.dot(vt_s[1, H // 2 - 1, :, c * CK:(c + 1) * CK],
                        s2[1, c * CK:(c + 1) * CK, cols], preferred_element_type=F32)
            accs[sb] = r if accs[sb] is None else accs[sb] + r

        def inv_block(i):
            rows = slice(i * BLK, (i + 1) * BLK)
            y = jnp.dot(inv_ref[...], zf_s[:, i].reshape(2 * BLK, D), preferred_element_type=F32)
            gx = x_v[rows, :].astype(F32) * jnp.concatenate([g_s[rows, :]] * NCH, axis=1)
            ga[i] = gx * (y + kv_s[rows, :])

        def out_block(i):
            sb, ii = divmod(i, SB // BLK)
            rows = slice(i * BLK, (i + 1) * BLK)
            oe = ot_s[0, :, :, rows]
            oo = jnp.concatenate([ot_s[1, 0:H // 2 - 1, :, rows],
                                  accs[sb][None, :, ii * BLK:(ii + 1) * BLK]], axis=0)
            low = jax.lax.broadcasted_iota(I32, (H // 2, 8, BLK), 1) < 4
            den = jnp.where(low, oo[:, 0:8], oe[:, 16:24])
            inv = pl.reciprocal(den, approx=True)
            inv = inv * (2.0 - den * inv)
            o = jnp.concatenate(
                [oe[:, 0:16] * inv[:, 4:5],
                 jnp.where(low, oe[:, 16:24], oo[:, 0:8]) * pltpu.roll(inv, 4, 1),
                 oo[:, 8:24] * inv[:, 0:1]], axis=1)
            o = o.reshape(D, BLK).T.astype(BF16)
            bb = jnp.dot(o, wo_v[...], preferred_element_type=F32)
            g1 = 1.0 - g_s[rows, :]
            out_v[rows, :] = (ga[i] + jnp.concatenate([g1] * NCH, axis=1) * bb).astype(BF16)
            pltpu.make_async_copy(out_v.at[rows, :], out_hbm.at[0, rows, :],
                                  sems.at[SEM_OUT]).start()

        nb = SB // BLK
        for i in range(nb):
            if i < nb - 1:
                for c in range(i * NC // (nb - 1), (i + 1) * NC // (nb - 1)):
                    pv_last(0, c)
            inv_block(i)
        for i in range(NB):
            out_block(i)
            sb, ii = divmod(i, nb)
            if sb + 1 < NSB:
                for c in range(ii * NC // nb, (ii + 1) * NC // nb):
                    pv_last(sb + 1, c)
                inv_block(i + nb)
        pltpu.make_async_copy(out_v, out_hbm.at[0], sems.at[SEM_OUT]).wait()

    pl.run_scoped(
        post_phase,
        pltpu.VMEM((2, S, S + 128), F32),
        pltpu.VMEM((2, 8, SQ), F32),
        pltpu.VMEM((NG, NB, 16, D), F32),
        pltpu.VMEM((2, H // 2, 24, S), F32),
        pltpu.VMEM((2, S, SQ), F32),
    )


@jax.jit
def pallas_gated_mix__ssm_conv_h3__mha_block__prompt_kernel(
    A_q: jax.Array,
    A_k: jax.Array,
    A_v: jax.Array,
    A_shift_k: jax.Array,
    A_ssm_k: jax.Array,
    A_ssm_D: jax.Array,
    B_x: jax.Array,
    B_wqkv: jax.Array,
    B_wo: jax.Array,
    gate_w: jax.Array,
):
    fwd, inv = _dft_consts()
    fwd = jnp.asarray(fwd, dtype=BF16)
    inv = jnp.asarray(inv, dtype=BF16).astype(F32)
    hbm = pl.BlockSpec(memory_space=pl.ANY)
    scratch = [
        pltpu.VMEM((S, D), BF16),
        pltpu.VMEM((S, D), BF16),
        pltpu.VMEM((D, D), BF16),
        pltpu.VMEM((H // 2, S // 2, 128), U32),
        pltpu.VMEM((2, H // 2, 16, S), U32),
        pltpu.VMEM((2, H // 2, 24, S), F32),
        pltpu.VMEM((S, D), F32),
        pltpu.VMEM((S, 128), F32),
        pltpu.VMEM((NG, NB, 16, D), F32),
        pltpu.VMEM((NG, NB, 16, D), F32),
        pltpu.VMEM((H // 2, R, 128), F32),
        pltpu.VMEM((2, DH, R, 128), F32),
        pltpu.VMEM((H // 2, 2 * DH, S), F32),
        pltpu.VMEM((2, DH, 8, S), F32),
        pltpu.VMEM((4, 8, 128), F32),
        pltpu.VMEM((BLK, 2 * BLK), F32),
        pltpu.SMEM((1,), F32),
        pltpu.SemaphoreType.DMA((NSEM,)),
    ]
    return pl.pallas_call(
        _kernel,
        out_shape=jax.ShapeDtypeStruct((1, S, D), BF16),
        in_specs=[hbm] * 11,
        out_specs=hbm,
        scratch_shapes=scratch,
        compiler_params=pltpu.CompilerParams(vmem_limit_bytes=127 * 1024 * 1024),
    )(A_q, A_k, A_v, A_shift_k.T, A_ssm_k, A_ssm_D, B_wqkv, B_wo, gate_w, fwd, inv)
```

```python
import math

import jax
import jax.numpy as jnp
import numpy as np
import jax.experimental.pallas as pl
import jax.experimental.pallas.tpu as pltpu

S = 2048
D = 640
H = 32
DH = 20
KS = 4
NCH = D // 128
BLK = 128
NB = S // BLK
NG = BLK // 8
CK = 128
SB = 512
NC = S // CK
NSB = S // SB
NU = NC * NSB
RB = 256
NRB = S // RB
NPEEL = 3
QB = 512
NQB = S // QB
R = 288
R0 = 256
SM = S - R
PK, PQ = 32, 256
AE = 3
FE = 2
SQ = 256
SCORE_BOUND = 80.0
F32 = jnp.float32
BF16 = jnp.bfloat16
U32 = jnp.uint32
I32 = jnp.int32
NT = (((1,), (1,)), ((), ()))

SEM_WK, SEM_WQ, SEM_WV, SEM_WO, SEM_OUT = 0, 1, 2, 3, 4
SEM_GW, SEM_SHK, SEM_SSD, SEM_FWD, SEM_INV = 5, 6, 7, 8, 9
SEM_X = 10
SEM_K = SEM_X + NRB
SEM_V = SEM_K + NQB
SEM_H = SEM_V + NQB
NSEM = SEM_H + NQB


def _dft_consts():
    f = np.concatenate([np.arange(0, BLK, 2), np.arange(1, BLK, 2)]).astype(np.float64)
    n = np.arange(BLK, dtype=np.float64)
    ang = 2.0 * np.pi * (f[:, None] + 0.5) * n[None, :] / (2 * BLK)
    re = np.cos(ang).reshape(NG, 8, BLK)
    im = -np.sin(ang).reshape(NG, 8, BLK)
    fwd = np.concatenate([re, im], axis=1).reshape(2 * BLK, BLK)
    inv = fwd.T / BLK
    return fwd, inv


def _timeline(steps, t1, edges):
    total = sum(w for w, _ in steps)
    out = {}
    acc = 0
    for w, p in steps:
        cyc = t1 * acc / total / NU * edges[-1]
        acc += w
        u = max(i for i in range(NU) if edges[i] <= cyc)
        out.setdefault(u, []).append(((cyc - edges[u]) / (edges[u + 1] - edges[u]), p))
    return out


def _kernel(x_hbm, k_hbm, v_hbm, shk_hbm, h_hbm, ssd_hbm, w_hbm, wo_hbm, gw_hbm,
            fwd_hbm, inv_hbm, out_hbm,
            x_v, k_v, wo_v, kp_s, qh_s, vt_s, kv_s, g_s, uf_s, hf_s,
            kfp, kb_s, qf_s, qb_s, bd_s, inv_ref, fl_s, sems):
    out_v = k_v
    cp_wo = pltpu.make_async_copy(wo_hbm, wo_v, sems.at[SEM_WO])
    cp_inv = pltpu.make_async_copy(inv_hbm, inv_ref, sems.at[SEM_INV])

    def build_kb(j, par, d, anchor=None, lo=0):
        t = jnp.full((8, 128), par * DH + d, I32)
        if anchor is not None:
            t = anchor(t) & 127
        idx = jnp.concatenate([t] * ((R - lo) // 8), axis=0)
        kb_s[par, d, lo:R, :] = jnp.take_along_axis(
            kfp[j, lo:R, :], idx, axis=1, mode="promise_in_bounds")

    def pre_phase(v_v, h_v, w_v, wt_s, kf_s, hp_s, kn_s, fwd_ref, shk_ref, ssd_ref, gw_ref):
        def w_copy(part, sem):
            return pltpu.make_async_copy(w_hbm.at[:, part * D:(part + 1) * D],
                                         w_v.at[:, part * D:(part + 1) * D], sems.at[sem])

        def x_copy(i):
            r0 = pl.multiple_of(i * RB, RB)
            return pltpu.make_async_copy(x_hbm.at[0, pl.ds(r0, RB), :],
                                         x_v.at[pl.ds(r0, RB), :], sems.at[SEM_X + i])

        def kvh_copies(i):
            r0 = pl.multiple_of(i * QB, QB)
            return (
                pltpu.make_async_copy(k_hbm.at[0, pl.ds(r0, QB), :],
                                      k_v.at[pl.ds(r0, QB), :], sems.at[SEM_K + i]),
                pltpu.make_async_copy(v_hbm.at[0, pl.ds(r0, QB), :],
                                      v_v.at[pl.ds(r0, QB), :], sems.at[SEM_V + i]),
                pltpu.make_async_copy(h_hbm.at[:, pl.ds(r0, QB)],
                                      h_v.at[:, pl.ds(r0, QB)], sems.at[SEM_H + i]),
            )

        cp_gw = pltpu.make_async_copy(gw_hbm, gw_ref, sems.at[SEM_GW])
        cp_small = (
            pltpu.make_async_copy(shk_hbm, shk_ref, sems.at[SEM_SHK]),
            pltpu.make_async_copy(ssd_hbm, ssd_ref, sems.at[SEM_SSD]),
            pltpu.make_async_copy(fwd_hbm, fwd_ref, sems.at[SEM_FWD]),
        )
        x_copy(0).start()
        w_copy(1, SEM_WK).start()
        cp_gw.start()
        for i in range(1, NRB):
            x_copy(i).start()
        for cp in cp_small:
            cp.start()
        w_copy(0, SEM_WQ).start()
        w_copy(2, SEM_WV).start()
        for i in range(NQB):
            for cp in kvh_copies(i):
                cp.start()
        cp_wo.start()
        cp_inv.start()

        kf_s[0:8, :] = jnp.zeros((8, D), F32)
        hp_s[...] = jnp.zeros((2 * BLK, D), F32)
        bd_s[...] = jnp.zeros((4, 8, 128), F32)

        def track(i, val):
            a = jnp.abs(val)
            a = jnp.max(a.reshape(a.shape[0] // 8, 8, a.shape[1]), axis=0)
            m = bd_s[i]
            for c in range(a.shape[1] // 128):
                m = jnp.maximum(m, a[:, c * 128:(c + 1) * 128])
            bd_s[i] = m

        def split_pairs(val):
            lane = jax.lax.broadcasted_iota(I32, (val.shape[0], 128), 1)
            parts = [val[:, c * 128:(c + 1) * 128] for c in range(NCH)]
            out = []
            for j in range(H // 2):
                c, sh = divmod(2 * DH * j, 128)
                src = parts[c]
                if sh + 2 * DH > 128:
                    src = jnp.where(lane >= 64, src, parts[c + 1])
                out.append(pltpu.roll(src, 128 - sh, 1) if sh else src)
            return out

        def kproj(rb):
            r0 = pl.multiple_of(rb * RB, RB)
            xb = x_v[pl.ds(r0, RB), :]
            kk = jnp.dot(xb, w_v[:, D:2 * D], preferred_element_type=F32)
            track(0, kk)
            kp = pltpu.bitcast(kk.astype(BF16), U32)
            h0 = pl.multiple_of(rb * (RB // 2), RB // 2)
            kn_s[pl.ds(h0, RB // 2), :] = kp
            if isinstance(rb, int) and (rb + 1) * RB > SM:
                lo = max(SM, rb * RB)
                for j, part in enumerate(split_pairs(kp[(lo - rb * RB) // 2:, :])):
                    kfp[j, lo - SM:(rb + 1) * RB - SM, :] = pltpu.bitcast(part, BF16).astype(F32)
            gw = gw_ref[...].astype(F32).reshape(1, D)
            g = jax.nn.sigmoid(jnp.sum(xb.astype(F32) * gw, axis=-1, keepdims=True))
            g_s[pl.ds(r0, RB), :] = jnp.broadcast_to(g, (RB, 128))

        w_copy(1, SEM_WK).wait()
        cp_gw.wait()

        def kproj_loop(rb, carry):
            x_copy(rb).wait()
            kproj(rb)
            return carry

        jax.lax.fori_loop(0, NRB - NPEEL, kproj_loop, 0)
        for i in range(NRB - NPEEL, NRB):
            x_copy(i).wait()
        w_copy(0, SEM_WQ).wait()
        w_copy(2, SEM_WV).wait()
        for cp in cp_small:
            cp.wait()
        fl_s[0] = jnp.max(bd_s[0])
        kproj(NRB - 1)
        wt_s[0:D, :] = w_v[:, 0:D].astype(F32).T.astype(BF16)
        wt_s[D:2 * D, :] = w_v[:, 2 * D:3 * D].astype(F32).T.astype(BF16)
        for i in range(NRB - 2, NRB - NPEEL - 1, -1):
            kproj(i)
        for d in range(DH):
            build_kb(0, 0, d, lo=R - R0)

        qscale = (DH ** -0.5) * math.log2(math.e)

        def fold(cur, prev):
            cur = cur.reshape(NG, 16, D)
            prev = prev.reshape(NG, 16, D)
            hg = NG // 2
            lo = jnp.concatenate(
                [cur[:hg, 0:8] - prev[:hg, 8:16], cur[:hg, 8:16] + prev[:hg, 0:8]], axis=1)
            hi = jnp.concatenate(
                [cur[hg:, 0:8] + prev[hg:, 8:16], cur[hg:, 8:16] - prev[hg:, 0:8]], axis=1)
            return jnp.concatenate([lo, hi], axis=0)

        def qvproj(rb, carry):
            for cp in kvh_copies(rb):
                cp.wait()
            ssd = ssd_ref[...].astype(F32).reshape(1, D)
            shk = shk_ref[...].astype(F32)
            r0 = pl.multiple_of(rb * QB, QB)

            def q_part(rs):
                xb = x_v[pl.ds(rs, RB), :]
                qt = jax.lax.dot_general(wt_s[0:D, :], xb, NT, preferred_element_type=F32)
                qt = qt * qscale
                track(1, qt)
                qf = qt.reshape(H // 2, 2 * DH, RB)
                row = jax.lax.broadcasted_iota(I32, (H // 2, 24, RB), 1)
                zpad = jnp.zeros((H // 2, 8, RB), F32)
                for par, win in ((0, jnp.where(row < DH, qf[:, 0:24], 0.0)),
                                 (1, jnp.where(row >= 4, qf[:, 16:40], 0.0))):
                    win = jnp.concatenate([win, zpad], axis=1).reshape(H // 2 * 32, RB)
                    qh_s[par, :, :, pl.ds(rs, RB)] = pltpu.bitcast(
                        win.astype(BF16), U32).reshape(H // 2, 16, RB)
                qf_s[:, :, pl.ds(rs, RB)] = qf
                for d in range(DH):
                    qb_s[0, d, :, pl.ds(rs, RB)] = jnp.broadcast_to(qf[0, d:d + 1, :], (8, RB))

            def v_part(rs):
                xb = x_v[pl.ds(rs, RB), :]
                vt = jax.lax.dot_general(wt_s[D:2 * D, :], xb, NT, preferred_element_type=F32)
                track(2, vt)
                vt = vt.reshape(H // 2, 2 * DH, RB)
                row = jax.lax.broadcasted_iota(I32, (H // 2, 24, RB), 1)
                vt_s[0, :, :, pl.ds(rs, RB)] = jnp.where(row < DH, vt[:, 0:24, :], 1.0)
                vt_s[1, :, :, pl.ds(rs, RB)] = jnp.where(row >= 4, vt[:, 16:40, :], 1.0)

            def k_split(rs):
                h0 = pl.multiple_of(rs // 2, RB // 2)
                for j, part in enumerate(split_pairs(kn_s[pl.ds(h0, RB // 2), :])):
                    kp_s[j, pl.ds(h0, RB // 2), :] = part

            def u_part(u, ktail):
                ru = pl.multiple_of(r0 + u * BLK, BLK)
                kc = k_v[pl.ds(ru, BLK), :].astype(F32)
                e3 = jnp.concatenate([ktail, kc], axis=0).reshape(BLK // 8 + 1, 8, D)
                sub = jax.lax.broadcasted_iota(I32, (BLK // 8, 8, D), 1)
                ksh = kc * shk[0:1, :]
                for j in range(1, KS):
                    rot = pltpu.roll(e3, j, 1)
                    sh = jnp.where(sub >= j, rot[1:], rot[:-1]).reshape(BLK, D)
                    ksh = ksh + sh * shk[j:j + 1, :]
                kv = ksh * v_v[pl.ds(ru, BLK), :].astype(F32)
                kv_s[pl.ds(ru, BLK), :] = kv * ssd
                uf_s[:, rb * (QB // BLK) + u] = jnp.dot(
                    fwd_ref[...], kv.astype(BF16),
                    preferred_element_type=F32).reshape(NG, 16, D)
                return kc[BLK - 8:, :]

            def h_part(u, prev):
                ru = pl.multiple_of(r0 + u * BLK, BLK)
                raw = jax.lax.dot_general(fwd_ref[...], h_v[:, pl.ds(ru, BLK)], NT,
                                          preferred_element_type=F32)
                hf_s[:, rb * (QB // BLK) + u] = fold(raw, prev)
                return raw

            ktail = kf_s[0:8, :]
            prev = hp_s[...]
            for sub in range(QB // RB):
                rs = pl.multiple_of(r0 + sub * RB, RB)
                k_split(rs)
                q_part(rs)
                ktail = u_part(2 * sub, ktail)
                prev = h_part(2 * sub, prev)
                prev = h_part(2 * sub + 1, prev)
                if sub == QB // RB - 1:
                    hp_s[...] = prev
                v_part(rs)
                ktail = u_part(2 * sub + 1, ktail)
            kf_s[0:8, :] = ktail
            return carry

        jax.lax.fori_loop(0, NQB, qvproj, 0)

    pl.run_scoped(
        pre_phase,
        pltpu.VMEM((S, D), BF16),
        pltpu.VMEM((D, S), BF16),
        pltpu.VMEM((D, 3 * D), BF16),
        pltpu.VMEM((2 * D, D), BF16),
        pltpu.VMEM((32, D), F32),
        pltpu.VMEM((2 * BLK, D), F32),
        pltpu.VMEM((S // 2, D), U32),
        pltpu.VMEM((2 * BLK, BLK), BF16),
        pltpu.VMEM((KS, D), BF16),
        pltpu.VMEM((D,), BF16),
        pltpu.VMEM((D,), BF16),
    )

    def post_phase(s2, m2, zf_s, ot_s, ss):
        def freq_steps(g, chunks):
            steps = []
            for c in chunks:
                cols = slice(c * 128, (c + 1) * 128) if isinstance(c, int) else c
                for i in range(NB):
                    st = {}
                    for m0 in range(0, i + 1, FE):
                        ms = list(range(m0, min(i + 1, m0 + FE)))

                        def step(anchor, i=i, cols=cols, ms=ms, st=st):
                            for m in ms:
                                ur = uf_s[g, m, 0:8, cols]
                                ui = uf_s[g, m, 8:16, cols]
                                hr = hf_s[g, i - m, 0:8, cols]
                                hi = hf_s[g, i - m, 8:16, cols]
                                if m == ms[0]:
                                    ur = anchor(ur)
                                tr = ur * hr - ui * hi
                                ti = ur * hi + ui * hr
                                st["r"] = tr if m == 0 else st["r"] + tr
                                st["i"] = ti if m == 0 else st["i"] + ti
                            if ms[-1] == i:
                                zf_s[g, i, 0:8, cols] = st["r"]
                                zf_s[g, i, 8:16, cols] = st["i"]
                        steps.append((len(ms), step))
            return steps

        kmax = jnp.max(bd_s[0])
        qmax = jnp.max(bd_s[1])
        vmax = jnp.max(bd_s[2])
        live = jnp.logical_not(fl_s[0] < 0.0)

        def tie_to(tie):
            def anchor(v):
                t = tie if tie.dtype == v.dtype else pltpu.bitcast(tie, v.dtype)
                if v.shape[0] > 8:
                    t = jnp.concatenate([t] * (v.shape[0] // 8), axis=0)
                return jnp.where(live, v, t)
            return anchor

        def stage(h_qk, par_qk, h_pv, fsteps, rv=R):
            par_pv = 1 - par_qk
            bounds = [min(S - rv, (((S - rv) * c // NC) + 15) // 16 * 16) for c in range(NC + 1)]
            jq = h_qk >> 1
            j_nx = 0 if isinstance(h_qk, int) else jnp.minimum(h_qk + 1, H - 1) >> 1
            edges = [0]
            for u in range(NU):
                edges.append(edges[-1] + bounds[u % NC + 1] - bounds[u % NC]
                             + (24 if h_pv is not None else 0))
            ftl = _timeline(fsteps, NU * (1 - 0.008), edges)

            def prep_q(anchor, t):
                tc = slice(t * 128, (t + 1) * 128)
                blk = anchor(qf_s[j_nx, par_pv * 16:par_pv * 16 + 24, tc])
                for d in range(DH):
                    rr = par_pv * 4 + d
                    qb_s[par_pv, d, :, tc] = jnp.broadcast_to(blk[rr:rr + 1, :], (8, 128))

            psteps = []
            for i in range(DH):
                psteps.append((1, lambda anchor, i=i: build_kb(j_nx, par_pv, i, anchor)))
                if i < S // 128:
                    psteps.append((1, lambda anchor, i=i: prep_q(anchor, i)))
            ptl = _timeline(psteps, NU * (1 - 0.06), edges)
            if h_pv is not None:
                j = h_pv >> 1

            vsteps = []
            for sb in range(NSB):
                for k0 in range(R - rv, R, PK):
                    for qq in range(SB // PQ):
                        st = {}
                        for d0 in range(0, DH, AE):
                            def step(anchor, k0=k0, q0=sb * SB + qq * PQ, d0=d0, st=st):
                                for d in range(d0, min(DH, d0 + AE)):
                                    kb = kb_s[par_qk, d, k0:k0 + PK, :]
                                    if d == d0:
                                        w = (d0 // AE) % (PK // 8)
                                        kb = jnp.concatenate(
                                            [anchor(kb[i * 8:(i + 1) * 8]) if i == w
                                             else kb[i * 8:(i + 1) * 8]
                                             for i in range(PK // 8)], axis=0)
                                    qr = qb_s[par_qk, d, :, q0:q0 + PQ]
                                    t = (jnp.concatenate([kb] * (PQ // 128), axis=1)
                                         * jnp.concatenate([qr] * (PK // 8), axis=0))
                                    st["a"] = t if d == 0 else st["a"] + t
                                if d0 + AE >= DH:
                                    s2[par_qk, SM + k0:SM + k0 + PK,
                                       q0:q0 + PQ] = jnp.exp2(st["a"])
                            vsteps.append((min(DH, d0 + AE) - d0, step))
            vtl = _timeline(vsteps, NU - 0.25, edges)

            acc = None
            for sb in range(NSB):
                cols = slice(sb * SB, (sb + 1) * SB)
                for c in range(NC):
                    u = sb * NC + c
                    r0, r1 = bounds[c], bounds[c + 1]
                    kc = pltpu.bitcast(kp_s[jq, r0 // 2:r1 // 2, :], BF16)
                    qt = qh_s[par_qk, jq, :, cols]
                    if par_qk == 1:
                        qt = jnp.concatenate([jnp.zeros((8, SB), U32), qt], axis=0)
                    qt = pltpu.bitcast(qt, BF16)
                    s = jnp.dot(kc[:, 0:qt.shape[0]], qt, preferred_element_type=F32)
                    s2[par_qk, r0:r1, cols] = jnp.exp2(s)
                    ties = s
                    if h_pv is not None:
                        ct, kq = divmod(u, NSB)
                        pc = slice(ct * 128, (ct + 1) * 128)
                        rs = [jnp.dot(vt_s[par_pv, j, :, kq * SB + i * CK:kq * SB + (i + 1) * CK],
                                      s2[par_pv, kq * SB + i * CK:kq * SB + (i + 1) * CK, pc],
                                      preferred_element_type=F32) for i in range(SB // CK)]
                        if kq == 0:
                            z = tie_to(s[0:8, 0:128])(jnp.zeros((8, 128), F32))
                            acc = jnp.concatenate([z] * 3, axis=0)
                        for rr in rs:
                            acc = acc + rr
                        if kq == NSB - 1:
                            ot_s[par_pv, j, :, pc] = acc
                        if u < NU - 1:
                            ties = jnp.concatenate([s, jnp.concatenate(rs, axis=1)], axis=0)
                    ng = ties.shape[0] // 8
                    for col, tl in ((0, vtl.get(u, [])), (1, ptl.get(u, [])), (2, ftl.get(u, []))):
                        for frac, p in tl:
                            gi = min(ng - 1, int(frac * ng))
                            p(tie_to(ties[gi * 8:(gi + 1) * 8, col * 128:(col + 1) * 128]))

        def fast_path():
            def body(t, carry):
                @pl.when((t & 1) == 1)
                def _():
                    stage(t, 1, t - 1, freq_steps(t >> 1, (2, 3, 4)))

                @pl.when((t & 1) == 0)
                def _():
                    stage(t, 0, t - 1, freq_steps(t >> 1, (0, 1)))
                return carry

            jax.lax.fori_loop(1, H, body, 0)

        def slow_path():
            nq = S // SQ

            def block(it_qk, it_pv, wbuf):
                rbuf = 1 - wbuf
                h = it_qk // nq
                c0 = pl.multiple_of((it_qk % nq) * SQ, SQ)
                q32 = qh_s[h & 1, h >> 1, :, pl.ds(c0, SQ)]
                z = jnp.zeros((8, SQ), U32)
                qt = pltpu.bitcast(jnp.where((h & 1) == 1, jnp.concatenate([z, q32], axis=0),
                                             jnp.concatenate([q32, z], axis=0)), BF16)
                hp = it_pv // nq
                cp = pl.multiple_of((it_pv % nq) * SQ, SQ)
                m = jnp.max(m2[rbuf], axis=0, keepdims=True)
                mx = None
                acc = None
                for c in range(S // SQ):
                    rows = slice(c * SQ, (c + 1) * SQ)
                    kc = pltpu.bitcast(kp_s[h >> 1, c * SQ // 2:(c + 1) * SQ // 2, :], BF16)
                    s = jnp.dot(kc[:, 0:48], qt, preferred_element_type=F32)
                    ss[wbuf, rows, :] = s
                    cm = jnp.max(s.reshape(SQ // 8, 8, SQ), axis=0)
                    mx = cm if mx is None else jnp.maximum(mx, cm)
                    p = jnp.exp2(ss[rbuf, rows, :] - m)
                    s2[1, rows, pl.ds(cp, SQ)] = p
                    r = jnp.dot(vt_s[hp & 1, hp >> 1, :, rows], p, preferred_element_type=F32)
                    acc = r if acc is None else acc + r
                m2[wbuf] = mx
                ot_s[hp & 1, hp >> 1, :, pl.ds(cp, SQ)] = acc

            ss[1] = jnp.zeros((S, SQ), F32)
            m2[1] = jnp.zeros((8, SQ), F32)

            def body(it, carry):
                cur = jnp.minimum(it, H * nq - 1)
                prv = jnp.maximum(it - 1, 0)

                @pl.when((it & 1) == 0)
                def _():
                    block(cur, prv, 0)

                @pl.when((it & 1) == 1)
                def _():
                    block(cur, prv, 1)
                return carry

            jax.lax.fori_loop(0, H * nq + 1, body, 0)

            def fbody(i, carry):
                cols = pl.ds(pl.multiple_of((i % NCH) * 128, 128), 128)
                for _, p in freq_steps(i // NCH, (cols,)):
                    p(lambda v: v)
                return carry

            jax.lax.fori_loop(0, NG * NCH, fbody, 0)

        safe = jnp.logical_and(
            kmax * qmax * (1.02 * DH) <= SCORE_BOUND,
            jnp.logical_and(vmax <= 2.0 ** 30, vmax >= 2.0 ** -20))

        stage(0, 0, None, freq_steps(0, (0, 1)), rv=R0)

        jax.lax.cond(safe, fast_path, slow_path)

        cp_inv.wait()
        cp_wo.wait()
        accs = [None] * NSB
        ga = {}

        def pv_last(sb, c):
            cols = slice(sb * SB, (sb + 1) * SB)
            r = jnp.dot(vt_s[1, H // 2 - 1, :, c * CK:(c + 1) * CK],
                        s2[1, c * CK:(c + 1) * CK, cols], preferred_element_type=F32)
            accs[sb] = r if accs[sb] is None else accs[sb] + r

        def inv_block(i):
            rows = slice(i * BLK, (i + 1) * BLK)
            y = jnp.dot(inv_ref[...], zf_s[:, i].reshape(2 * BLK, D), preferred_element_type=F32)
            gx = x_v[rows, :].astype(F32) * jnp.concatenate([g_s[rows, :]] * NCH, axis=1)
            ga[i] = gx * (y + kv_s[rows, :])

        def out_block(i):
            sb, ii = divmod(i, SB // BLK)
            rows = slice(i * BLK, (i + 1) * BLK)
            oe = ot_s[0, :, :, rows]
            oo = jnp.concatenate([ot_s[1, 0:H // 2 - 1, :, rows],
                                  accs[sb][None, :, ii * BLK:(ii + 1) * BLK]], axis=0)
            low = jax.lax.broadcasted_iota(I32, (H // 2, 8, BLK), 1) < 4
            den = jnp.where(low, oo[:, 0:8], oe[:, 16:24])
            inv = pl.reciprocal(den, approx=True)
            inv = inv * (2.0 - den * inv)
            o = jnp.concatenate(
                [oe[:, 0:16] * inv[:, 4:5],
                 jnp.where(low, oe[:, 16:24], oo[:, 0:8]) * pltpu.roll(inv, 4, 1),
                 oo[:, 8:24] * inv[:, 0:1]], axis=1)
            o = o.reshape(D, BLK).T.astype(BF16)
            bb = jnp.dot(o, wo_v[...], preferred_element_type=F32)
            g1 = 1.0 - g_s[rows, :]
            out_v[rows, :] = (ga[i] + jnp.concatenate([g1] * NCH, axis=1) * bb).astype(BF16)
            pltpu.make_async_copy(out_v.at[rows, :], out_hbm.at[0, rows, :],
                                  sems.at[SEM_OUT]).start()

        nb = SB // BLK
        for i in range(nb):
            if i < nb - 1:
                for c in range(i * NC // (nb - 1), (i + 1) * NC // (nb - 1)):
                    pv_last(0, c)
            inv_block(i)
        for i in range(NB):
            out_block(i)
            sb, ii = divmod(i, nb)
            if sb + 1 < NSB:
                for c in range(ii * NC // nb, (ii + 1) * NC // nb):
                    pv_last(sb + 1, c)
                inv_block(i + nb)
        pltpu.make_async_copy(out_v, out_hbm.at[0], sems.at[SEM_OUT]).wait()

    pl.run_scoped(
        post_phase,
        pltpu.VMEM((2, S, S + 128), F32),
        pltpu.VMEM((2, 8, SQ), F32),
        pltpu.VMEM((NG, NB, 16, D), F32),
        pltpu.VMEM((2, H // 2, 24, S), F32),
        pltpu.VMEM((2, S, SQ), F32),
    )


@jax.jit
def pallas_gated_mix__ssm_conv_h3__mha_block__prompt_kernel(
    A_q: jax.Array,
    A_k: jax.Array,
    A_v: jax.Array,
    A_shift_k: jax.Array,
    A_ssm_k: jax.Array,
    A_ssm_D: jax.Array,
    B_x: jax.Array,
    B_wqkv: jax.Array,
    B_wo: jax.Array,
    gate_w: jax.Array,
):
    fwd, inv = _dft_consts()
    fwd = jnp.asarray(fwd, dtype=BF16)
    inv = jnp.asarray(inv, dtype=BF16).astype(F32)
    hbm = pl.BlockSpec(memory_space=pl.ANY)
    scratch = [
        pltpu.VMEM((S, D), BF16),
        pltpu.VMEM((S, D), BF16),
        pltpu.VMEM((D, D), BF16),
        pltpu.VMEM((H // 2, S // 2, 128), U32),
        pltpu.VMEM((2, H // 2, 16, S), U32),
        pltpu.VMEM((2, H // 2, 24, S), F32),
        pltpu.VMEM((S, D), F32),
        pltpu.VMEM((S, 128), F32),
        pltpu.VMEM((NG, NB, 16, D), F32),
        pltpu.VMEM((NG, NB, 16, D), F32),
        pltpu.VMEM((H // 2, R, 128), F32),
        pltpu.VMEM((2, DH, R, 128), F32),
        pltpu.VMEM((H // 2, 2 * DH, S), F32),
        pltpu.VMEM((2, DH, 8, S), F32),
        pltpu.VMEM((4, 8, 128), F32),
        pltpu.VMEM((BLK, 2 * BLK), F32),
        pltpu.SMEM((1,), F32),
        pltpu.SemaphoreType.DMA((NSEM,)),
    ]
    return pl.pallas_call(
        _kernel,
        out_shape=jax.ShapeDtypeStruct((1, S, D), BF16),
        in_specs=[hbm] * 11,
        out_specs=hbm,
        scratch_shapes=scratch,
        compiler_params=pltpu.CompilerParams(vmem_limit_bytes=127 * 1024 * 1024),
    )(A_q, A_k, A_v, A_shift_k.T, A_ssm_k, A_ssm_D, B_wqkv, B_wo, gate_w, fwd, inv)
```

```python
import math

import jax
import jax.numpy as jnp
import numpy as np
import jax.experimental.pallas as pl
import jax.experimental.pallas.tpu as pltpu

S = 2048
D = 640
H = 32
DH = 20
KS = 4
NCH = D // 128
BLK = 128
NB = S // BLK
NG = BLK // 8
CK = 128
SB = 512
NC = S // CK
NSB = S // SB
NU = NC * NSB
RB = 256
NRB = S // RB
NPEEL = 3
QB = 512
NQB = S // QB
R = 288
R0 = 256
SM = S - R
PK, PQ = 32, 256
AE = 3
FE = 2
SQ = 256
SCORE_BOUND = 80.0
F32 = jnp.float32
BF16 = jnp.bfloat16
U32 = jnp.uint32
I32 = jnp.int32
NT = (((1,), (1,)), ((), ()))

SEM_WK, SEM_WQ, SEM_WV, SEM_WO, SEM_OUT = 0, 1, 2, 3, 4
SEM_GW, SEM_SHK, SEM_SSD, SEM_FWD, SEM_INV = 5, 6, 7, 8, 9
SEM_X = 10
SEM_K = SEM_X + NRB
SEM_V = SEM_K + NQB
SEM_H = SEM_V + NQB
NSEM = SEM_H + NQB


def _dft_consts():
    f = np.concatenate([np.arange(0, BLK, 2), np.arange(1, BLK, 2)]).astype(np.float64)
    n = np.arange(BLK, dtype=np.float64)
    ang = 2.0 * np.pi * (f[:, None] + 0.5) * n[None, :] / (2 * BLK)
    re = np.cos(ang).reshape(NG, 8, BLK)
    im = -np.sin(ang).reshape(NG, 8, BLK)
    fwd = np.concatenate([re, im], axis=1).reshape(2 * BLK, BLK)
    inv = fwd.T / BLK
    return fwd, inv


def _timeline(steps, t1, edges):
    total = sum(w for w, _ in steps)
    out = {}
    acc = 0
    for w, p in steps:
        cyc = t1 * acc / total / NU * edges[-1]
        acc += w
        u = max(i for i in range(NU) if edges[i] <= cyc)
        out.setdefault(u, []).append(((cyc - edges[u]) / (edges[u + 1] - edges[u]), p))
    return out


def _kernel(x_hbm, k_hbm, v_hbm, shk_hbm, h_hbm, ssd_hbm, w_hbm, wo_hbm, gw_hbm,
            fwd_hbm, inv_hbm, out_hbm,
            x_v, k_v, wo_v, kp_s, qh_s, vt_s, kv_s, g_s, uf_s, hf_s,
            kfp, kb_s, qf_s, qb_s, bd_s, inv_ref, fl_s, sems):
    out_v = k_v
    cp_wo = pltpu.make_async_copy(wo_hbm, wo_v, sems.at[SEM_WO])
    cp_inv = pltpu.make_async_copy(inv_hbm, inv_ref, sems.at[SEM_INV])

    def build_kb(j, par, d, anchor=None, lo=0):
        t = jnp.full((8, 128), par * DH + d, I32)
        if anchor is not None:
            t = anchor(t) & 127
        idx = jnp.concatenate([t] * ((R - lo) // 8), axis=0)
        kb_s[par, d, lo:R, :] = jnp.take_along_axis(
            kfp[j, lo:R, :], idx, axis=1, mode="promise_in_bounds")

    def pre_phase(v_v, h_v, w_v, wt_s, kf_s, hp_s, kn_s, fwd_ref, shk_ref, ssd_ref, gw_ref):
        def w_copy(part, sem):
            return pltpu.make_async_copy(w_hbm.at[:, part * D:(part + 1) * D],
                                         w_v.at[:, part * D:(part + 1) * D], sems.at[sem])

        def x_copy(i):
            r0 = pl.multiple_of(i * RB, RB)
            return pltpu.make_async_copy(x_hbm.at[0, pl.ds(r0, RB), :],
                                         x_v.at[pl.ds(r0, RB), :], sems.at[SEM_X + i])

        def kvh_copies(i):
            r0 = pl.multiple_of(i * QB, QB)
            return (
                pltpu.make_async_copy(k_hbm.at[0, pl.ds(r0, QB), :],
                                      k_v.at[pl.ds(r0, QB), :], sems.at[SEM_K + i]),
                pltpu.make_async_copy(v_hbm.at[0, pl.ds(r0, QB), :],
                                      v_v.at[pl.ds(r0, QB), :], sems.at[SEM_V + i]),
                pltpu.make_async_copy(h_hbm.at[:, pl.ds(r0, QB)],
                                      h_v.at[:, pl.ds(r0, QB)], sems.at[SEM_H + i]),
            )

        cp_gw = pltpu.make_async_copy(gw_hbm, gw_ref, sems.at[SEM_GW])
        cp_small = (
            pltpu.make_async_copy(shk_hbm, shk_ref, sems.at[SEM_SHK]),
            pltpu.make_async_copy(ssd_hbm, ssd_ref, sems.at[SEM_SSD]),
            pltpu.make_async_copy(fwd_hbm, fwd_ref, sems.at[SEM_FWD]),
        )
        x_copy(0).start()
        w_copy(1, SEM_WK).start()
        cp_gw.start()
        for i in range(1, NRB):
            x_copy(i).start()
        for cp in cp_small:
            cp.start()
        w_copy(0, SEM_WQ).start()
        w_copy(2, SEM_WV).start()
        for i in range(NQB):
            for cp in kvh_copies(i):
                cp.start()
        cp_wo.start()
        cp_inv.start()

        kf_s[0:8, :] = jnp.zeros((8, D), F32)
        hp_s[...] = jnp.zeros((2 * BLK, D), F32)
        bd_s[...] = jnp.zeros((4, 8, 128), F32)

        def track(i, val):
            a = jnp.abs(val)
            a = jnp.max(a.reshape(a.shape[0] // 8, 8, a.shape[1]), axis=0)
            m = bd_s[i]
            for c in range(a.shape[1] // 128):
                m = jnp.maximum(m, a[:, c * 128:(c + 1) * 128])
            bd_s[i] = m

        def split_pairs(val):
            lane = jax.lax.broadcasted_iota(I32, (val.shape[0], 128), 1)
            parts = [val[:, c * 128:(c + 1) * 128] for c in range(NCH)]
            out = []
            for j in range(H // 2):
                c, sh = divmod(2 * DH * j, 128)
                src = parts[c]
                if sh + 2 * DH > 128:
                    src = jnp.where(lane >= 64, src, parts[c + 1])
                out.append(pltpu.roll(src, 128 - sh, 1) if sh else src)
            return out

        def kproj(rb):
            r0 = pl.multiple_of(rb * RB, RB)
            xb = x_v[pl.ds(r0, RB), :]
            kk = jnp.dot(xb, w_v[:, D:2 * D], preferred_element_type=F32)
            track(0, kk)
            kp = pltpu.bitcast(kk.astype(BF16), U32)
            h0 = pl.multiple_of(rb * (RB // 2), RB // 2)
            kn_s[pl.ds(h0, RB // 2), :] = kp
            if isinstance(rb, int) and (rb + 1) * RB > SM:
                lo = max(SM, rb * RB)
                for j, part in enumerate(split_pairs(kp[(lo - rb * RB) // 2:, :])):
                    kfp[j, lo - SM:(rb + 1) * RB - SM, :] = pltpu.bitcast(part, BF16).astype(F32)
            gw = gw_ref[...].astype(F32).reshape(1, D)
            g = jax.nn.sigmoid(jnp.sum(xb.astype(F32) * gw, axis=-1, keepdims=True))
            g_s[pl.ds(r0, RB), :] = jnp.broadcast_to(g, (RB, 128))

        w_copy(1, SEM_WK).wait()
        cp_gw.wait()

        def kproj_loop(rb, carry):
            x_copy(rb).wait()
            kproj(rb)
            return carry

        jax.lax.fori_loop(0, NRB - NPEEL, kproj_loop, 0)
        for i in range(NRB - NPEEL, NRB):
            x_copy(i).wait()
        w_copy(0, SEM_WQ).wait()
        w_copy(2, SEM_WV).wait()
        for cp in cp_small:
            cp.wait()
        fl_s[0] = jnp.max(bd_s[0])
        kproj(NRB - 1)
        wt_s[0:D, :] = w_v[:, 0:D].astype(F32).T.astype(BF16)
        wt_s[D:2 * D, :] = w_v[:, 2 * D:3 * D].astype(F32).T.astype(BF16)
        for i in range(NRB - 2, NRB - NPEEL - 1, -1):
            kproj(i)
        for d in range(DH):
            build_kb(0, 0, d, lo=R - R0)

        qscale = (DH ** -0.5) * math.log2(math.e)

        def fold(cur, prev):
            cur = cur.reshape(NG, 16, D)
            prev = prev.reshape(NG, 16, D)
            hg = NG // 2
            lo = jnp.concatenate(
                [cur[:hg, 0:8] - prev[:hg, 8:16], cur[:hg, 8:16] + prev[:hg, 0:8]], axis=1)
            hi = jnp.concatenate(
                [cur[hg:, 0:8] + prev[hg:, 8:16], cur[hg:, 8:16] - prev[hg:, 0:8]], axis=1)
            return jnp.concatenate([lo, hi], axis=0)

        def qvproj(rb, carry):
            for cp in kvh_copies(rb):
                cp.wait()
            ssd = ssd_ref[...].astype(F32).reshape(1, D)
            shk = shk_ref[...].astype(F32)
            r0 = pl.multiple_of(rb * QB, QB)

            def q_part(rs):
                xb = x_v[pl.ds(rs, RB), :]
                qt = jax.lax.dot_general(wt_s[0:D, :], xb, NT, preferred_element_type=F32)
                qt = qt * qscale
                track(1, qt)
                qf = qt.reshape(H // 2, 2 * DH, RB)
                row = jax.lax.broadcasted_iota(I32, (H // 2, 24, RB), 1)
                zpad = jnp.zeros((H // 2, 8, RB), F32)
                for par, win in ((0, jnp.where(row < DH, qf[:, 0:24], 0.0)),
                                 (1, jnp.where(row >= 4, qf[:, 16:40], 0.0))):
                    win = jnp.concatenate([win, zpad], axis=1).reshape(H // 2 * 32, RB)
                    qh_s[par, :, :, pl.ds(rs, RB)] = pltpu.bitcast(
                        win.astype(BF16), U32).reshape(H // 2, 16, RB)
                qf_s[:, :, pl.ds(rs, RB)] = qf
                for d in range(DH):
                    qb_s[0, d, :, pl.ds(rs, RB)] = jnp.broadcast_to(qf[0, d:d + 1, :], (8, RB))

            def v_part(rs):
                xb = x_v[pl.ds(rs, RB), :]
                vt = jax.lax.dot_general(wt_s[D:2 * D, :], xb, NT, preferred_element_type=F32)
                track(2, vt)
                vt = vt.reshape(H // 2, 2 * DH, RB)
                row = jax.lax.broadcasted_iota(I32, (H // 2, 24, RB), 1)
                vt_s[0, :, :, pl.ds(rs, RB)] = jnp.where(row < DH, vt[:, 0:24, :], 1.0)
                vt_s[1, :, :, pl.ds(rs, RB)] = jnp.where(row >= 4, vt[:, 16:40, :], 1.0)

            def k_split(rs):
                h0 = pl.multiple_of(rs // 2, RB // 2)
                for j, part in enumerate(split_pairs(kn_s[pl.ds(h0, RB // 2), :])):
                    kp_s[j, pl.ds(h0, RB // 2), :] = part

            def u_part(u, ktail):
                ru = pl.multiple_of(r0 + u * BLK, BLK)
                kc = k_v[pl.ds(ru, BLK), :].astype(F32)
                e3 = jnp.concatenate([ktail, kc], axis=0).reshape(BLK // 8 + 1, 8, D)
                sub = jax.lax.broadcasted_iota(I32, (BLK // 8, 8, D), 1)
                ksh = kc * shk[0:1, :]
                for j in range(1, KS):
                    rot = pltpu.roll(e3, j, 1)
                    sh = jnp.where(sub >= j, rot[1:], rot[:-1]).reshape(BLK, D)
                    ksh = ksh + sh * shk[j:j + 1, :]
                kv = ksh * v_v[pl.ds(ru, BLK), :].astype(F32)
                kv_s[pl.ds(ru, BLK), :] = kv * ssd
                uf_s[:, rb * (QB // BLK) + u] = jnp.dot(
                    fwd_ref[...], kv.astype(BF16),
                    preferred_element_type=F32).reshape(NG, 16, D)
                return kc[BLK - 8:, :]

            def h_part(u, prev):
                ru = pl.multiple_of(r0 + u * BLK, BLK)
                raw = jax.lax.dot_general(fwd_ref[...], h_v[:, pl.ds(ru, BLK)], NT,
                                          preferred_element_type=F32)
                hf_s[:, rb * (QB // BLK) + u] = fold(raw, prev)
                return raw

            ktail = kf_s[0:8, :]
            prev = hp_s[...]
            for sub in range(QB // RB):
                rs = pl.multiple_of(r0 + sub * RB, RB)
                k_split(rs)
                q_part(rs)
                ktail = u_part(2 * sub, ktail)
                prev = h_part(2 * sub, prev)
                prev = h_part(2 * sub + 1, prev)
                if sub == QB // RB - 1:
                    hp_s[...] = prev
                v_part(rs)
                ktail = u_part(2 * sub + 1, ktail)
            kf_s[0:8, :] = ktail
            return carry

        jax.lax.fori_loop(0, NQB, qvproj, 0)

    pl.run_scoped(
        pre_phase,
        pltpu.VMEM((S, D), BF16),
        pltpu.VMEM((D, S), BF16),
        pltpu.VMEM((D, 3 * D), BF16),
        pltpu.VMEM((2 * D, D), BF16),
        pltpu.VMEM((32, D), F32),
        pltpu.VMEM((2 * BLK, D), F32),
        pltpu.VMEM((S // 2, D), U32),
        pltpu.VMEM((2 * BLK, BLK), BF16),
        pltpu.VMEM((KS, D), BF16),
        pltpu.VMEM((D,), BF16),
        pltpu.VMEM((D,), BF16),
    )

    def post_phase(s2, m2, zf_s, ot_s, ss):
        def freq_steps(g, chunks):
            steps = []
            for c in chunks:
                cols = slice(c * 128, (c + 1) * 128) if isinstance(c, int) else c
                for i in range(NB):
                    st = {}
                    for m0 in range(0, i + 1, FE):
                        ms = list(range(m0, min(i + 1, m0 + FE)))

                        def step(anchor, i=i, cols=cols, ms=ms, st=st):
                            for m in ms:
                                ur = uf_s[g, m, 0:8, cols]
                                ui = uf_s[g, m, 8:16, cols]
                                hr = hf_s[g, i - m, 0:8, cols]
                                hi = hf_s[g, i - m, 8:16, cols]
                                if m == ms[0]:
                                    ur = anchor(ur)
                                tr = ur * hr - ui * hi
                                ti = ur * hi + ui * hr
                                st["r"] = tr if m == 0 else st["r"] + tr
                                st["i"] = ti if m == 0 else st["i"] + ti
                            if ms[-1] == i:
                                zf_s[g, i, 0:8, cols] = st["r"]
                                zf_s[g, i, 8:16, cols] = st["i"]
                        steps.append((len(ms), step))
            return steps

        kmax = jnp.max(bd_s[0])
        qmax = jnp.max(bd_s[1])
        vmax = jnp.max(bd_s[2])
        live = jnp.logical_not(fl_s[0] < 0.0)

        def tie_to(tie):
            def anchor(v):
                t = tie if tie.dtype == v.dtype else pltpu.bitcast(tie, v.dtype)
                if v.shape[0] > 8:
                    t = jnp.concatenate([t] * (v.shape[0] // 8), axis=0)
                return jnp.where(live, v, t)
            return anchor

        def stage(h_qk, par_qk, h_pv, fsteps, rv=R):
            par_pv = 1 - par_qk
            bounds = [min(S - rv, (((S - rv) * c // NC) + 15) // 16 * 16) for c in range(NC + 1)]
            jq = h_qk >> 1
            j_nx = 0 if isinstance(h_qk, int) else jnp.minimum(h_qk + 1, H - 1) >> 1
            edges = [0]
            for u in range(NU):
                edges.append(edges[-1] + bounds[u % NC + 1] - bounds[u % NC]
                             + (24 if h_pv is not None else 0))
            ftl = _timeline(fsteps, NU * (1 - 0.008), edges)

            def prep_q(anchor, t):
                tc = slice(t * 128, (t + 1) * 128)
                blk = anchor(qf_s[j_nx, par_pv * 16:par_pv * 16 + 24, tc])
                for d in range(DH):
                    rr = par_pv * 4 + d
                    qb_s[par_pv, d, :, tc] = jnp.broadcast_to(blk[rr:rr + 1, :], (8, 128))

            psteps = []
            for i in range(DH):
                psteps.append((1, lambda anchor, i=i: build_kb(j_nx, par_pv, i, anchor)))
                if i < S // 128:
                    psteps.append((1, lambda anchor, i=i: prep_q(anchor, i)))
            ptl = _timeline(psteps, NU * (1 - 0.06), edges)
            if h_pv is not None:
                j = h_pv >> 1

            vsteps = []
            for sb in range(NSB):
                for k0 in range(R - rv, R, PK):
                    for qq in range(SB // PQ):
                        st = {}
                        for d0 in range(0, DH, AE):
                            def step(anchor, k0=k0, q0=sb * SB + qq * PQ, d0=d0, st=st):
                                for d in range(d0, min(DH, d0 + AE)):
                                    kb = kb_s[par_qk, d, k0:k0 + PK, :]
                                    if d == d0:
                                        w = (d0 // AE) % (PK // 8)
                                        kb = jnp.concatenate(
                                            [anchor(kb[i * 8:(i + 1) * 8]) if i == w
                                             else kb[i * 8:(i + 1) * 8]
                                             for i in range(PK // 8)], axis=0)
                                    qr = qb_s[par_qk, d, :, q0:q0 + PQ]
                                    t = (jnp.concatenate([kb] * (PQ // 128), axis=1)
                                         * jnp.concatenate([qr] * (PK // 8), axis=0))
                                    st["a"] = t if d == 0 else st["a"] + t
                                if d0 + AE >= DH:
                                    s2[par_qk, SM + k0:SM + k0 + PK,
                                       q0:q0 + PQ] = jnp.exp2(st["a"])
                            vsteps.append((min(DH, d0 + AE) - d0, step))
            vtl = _timeline(vsteps, NU - 0.25, edges)

            acc = None
            for sb in range(NSB):
                cols = slice(sb * SB, (sb + 1) * SB)
                for c in range(NC):
                    u = sb * NC + c
                    r0, r1 = bounds[c], bounds[c + 1]
                    kc = pltpu.bitcast(kp_s[jq, r0 // 2:r1 // 2, :], BF16)
                    qt = qh_s[par_qk, jq, :, cols]
                    if par_qk == 1:
                        qt = jnp.concatenate([jnp.zeros((8, SB), U32), qt], axis=0)
                    qt = pltpu.bitcast(qt, BF16)
                    s = jnp.dot(kc[:, 0:qt.shape[0]], qt, preferred_element_type=F32)
                    s2[par_qk, r0:r1, cols] = jnp.exp2(s)
                    ties = s
                    if h_pv is not None:
                        ct, kq = divmod(u, NSB)
                        pc = slice(ct * 128, (ct + 1) * 128)
                        rs = [jnp.dot(vt_s[par_pv, j, :, kq * SB + i * CK:kq * SB + (i + 1) * CK],
                                      s2[par_pv, kq * SB + i * CK:kq * SB + (i + 1) * CK, pc],
                                      preferred_element_type=F32) for i in range(SB // CK)]
                        if kq == 0:
                            z = tie_to(s[0:8, 0:128])(jnp.zeros((8, 128), F32))
                            acc = jnp.concatenate([z] * 3, axis=0)
                        for rr in rs:
                            acc = acc + rr
                        if kq == NSB - 1:
                            ot_s[par_pv, j, :, pc] = acc
                        if u < NU - 1:
                            ties = jnp.concatenate([s, jnp.concatenate(rs, axis=1)], axis=0)
                    ng = ties.shape[0] // 8
                    for col, tl in ((0, vtl.get(u, [])), (1, ptl.get(u, [])), (2, ftl.get(u, []))):
                        for frac, p in tl:
                            gi = min(ng - 1, int(frac * ng))
                            p(tie_to(ties[gi * 8:(gi + 1) * 8, col * 128:(col + 1) * 128]))

        def fast_path():
            def body(i, carry):
                stage(2 * i + 1, 1, 2 * i, freq_steps(i, (2, 3, 4)))

                @pl.when(i < H // 2 - 1)
                def _():
                    stage(2 * i + 2, 0, 2 * i + 1, freq_steps(i + 1, (0, 1)))
                return carry

            jax.lax.fori_loop(0, H // 2, body, 0)

        def slow_path():
            nq = S // SQ

            def block(it_qk, it_pv, wbuf):
                rbuf = 1 - wbuf
                h = it_qk // nq
                c0 = pl.multiple_of((it_qk % nq) * SQ, SQ)
                q32 = qh_s[h & 1, h >> 1, :, pl.ds(c0, SQ)]
                z = jnp.zeros((8, SQ), U32)
                qt = pltpu.bitcast(jnp.where((h & 1) == 1, jnp.concatenate([z, q32], axis=0),
                                             jnp.concatenate([q32, z], axis=0)), BF16)
                hp = it_pv // nq
                cp = pl.multiple_of((it_pv % nq) * SQ, SQ)
                m = jnp.max(m2[rbuf], axis=0, keepdims=True)
                mx = None
                acc = None
                for c in range(S // SQ):
                    rows = slice(c * SQ, (c + 1) * SQ)
                    kc = pltpu.bitcast(kp_s[h >> 1, c * SQ // 2:(c + 1) * SQ // 2, :], BF16)
                    s = jnp.dot(kc[:, 0:48], qt, preferred_element_type=F32)
                    ss[wbuf, rows, :] = s
                    cm = jnp.max(s.reshape(SQ // 8, 8, SQ), axis=0)
                    mx = cm if mx is None else jnp.maximum(mx, cm)
                    p = jnp.exp2(ss[rbuf, rows, :] - m)
                    s2[1, rows, pl.ds(cp, SQ)] = p
                    r = jnp.dot(vt_s[hp & 1, hp >> 1, :, rows], p, preferred_element_type=F32)
                    acc = r if acc is None else acc + r
                m2[wbuf] = mx
                ot_s[hp & 1, hp >> 1, :, pl.ds(cp, SQ)] = acc

            ss[1] = jnp.zeros((S, SQ), F32)
            m2[1] = jnp.zeros((8, SQ), F32)

            def body(it, carry):
                cur = jnp.minimum(it, H * nq - 1)
                prv = jnp.maximum(it - 1, 0)

                @pl.when((it & 1) == 0)
                def _():
                    block(cur, prv, 0)

                @pl.when((it & 1) == 1)
                def _():
                    block(cur, prv, 1)
                return carry

            jax.lax.fori_loop(0, H * nq + 1, body, 0)

            def fbody(i, carry):
                cols = pl.ds(pl.multiple_of((i % NCH) * 128, 128), 128)
                for _, p in freq_steps(i // NCH, (cols,)):
                    p(lambda v: v)
                return carry

            jax.lax.fori_loop(0, NG * NCH, fbody, 0)

        safe = jnp.logical_and(
            kmax * qmax * (1.02 * DH) <= SCORE_BOUND,
            jnp.logical_and(vmax <= 2.0 ** 30, vmax >= 2.0 ** -20))

        stage(0, 0, None, freq_steps(0, (0, 1)), rv=R0)

        jax.lax.cond(safe, fast_path, slow_path)

        cp_inv.wait()
        cp_wo.wait()
        accs = [None] * NSB
        ga = {}

        def pv_last(sb, c):
            cols = slice(sb * SB, (sb + 1) * SB)
            r = jnp.dot(vt_s[1, H // 2 - 1, :, c * CK:(c + 1) * CK],
                        s2[1, c * CK:(c + 1) * CK, cols], preferred_element_type=F32)
            accs[sb] = r if accs[sb] is None else accs[sb] + r

        def inv_block(i):
            rows = slice(i * BLK, (i + 1) * BLK)
            y = jnp.dot(inv_ref[...], zf_s[:, i].reshape(2 * BLK, D), preferred_element_type=F32)
            gx = x_v[rows, :].astype(F32) * jnp.concatenate([g_s[rows, :]] * NCH, axis=1)
            ga[i] = gx * (y + kv_s[rows, :])

        def out_block(i):
            sb, ii = divmod(i, SB // BLK)
            rows = slice(i * BLK, (i + 1) * BLK)
            oe = ot_s[0, :, :, rows]
            oo = jnp.concatenate([ot_s[1, 0:H // 2 - 1, :, rows],
                                  accs[sb][None, :, ii * BLK:(ii + 1) * BLK]], axis=0)
            low = jax.lax.broadcasted_iota(I32, (H // 2, 8, BLK), 1) < 4
            den = jnp.where(low, oo[:, 0:8], oe[:, 16:24])
            inv = pl.reciprocal(den, approx=True)
            inv = inv * (2.0 - den * inv)
            o = jnp.concatenate(
                [oe[:, 0:16] * inv[:, 4:5],
                 jnp.where(low, oe[:, 16:24], oo[:, 0:8]) * pltpu.roll(inv, 4, 1),
                 oo[:, 8:24] * inv[:, 0:1]], axis=1)
            o = o.reshape(D, BLK).T.astype(BF16)
            bb = jnp.dot(o, wo_v[...], preferred_element_type=F32)
            g1 = 1.0 - g_s[rows, :]
            out_v[rows, :] = (ga[i] + jnp.concatenate([g1] * NCH, axis=1) * bb).astype(BF16)
            pltpu.make_async_copy(out_v.at[rows, :], out_hbm.at[0, rows, :],
                                  sems.at[SEM_OUT]).start()

        nb = SB // BLK
        for i in range(nb):
            if i < nb - 1:
                for c in range(i * NC // (nb - 1), (i + 1) * NC // (nb - 1)):
                    pv_last(0, c)
            inv_block(i)
        for i in range(NB):
            out_block(i)
            sb, ii = divmod(i, nb)
            if sb + 1 < NSB:
                for c in range(ii * NC // nb, (ii + 1) * NC // nb):
                    pv_last(sb + 1, c)
                inv_block(i + nb)
        pltpu.make_async_copy(out_v, out_hbm.at[0], sems.at[SEM_OUT]).wait()

    pl.run_scoped(
        post_phase,
        pltpu.VMEM((2, S, S + 128), F32),
        pltpu.VMEM((2, 8, SQ), F32),
        pltpu.VMEM((NG, NB, 16, D), F32),
        pltpu.VMEM((2, H // 2, 24, S), F32),
        pltpu.VMEM((2, S, SQ), F32),
    )


@jax.jit
def pallas_gated_mix__ssm_conv_h3__mha_block__prompt_kernel(
    A_q: jax.Array,
    A_k: jax.Array,
    A_v: jax.Array,
    A_shift_k: jax.Array,
    A_ssm_k: jax.Array,
    A_ssm_D: jax.Array,
    B_x: jax.Array,
    B_wqkv: jax.Array,
    B_wo: jax.Array,
    gate_w: jax.Array,
):
    fwd, inv = _dft_consts()
    fwd = jnp.asarray(fwd, dtype=BF16)
    inv = jnp.asarray(inv, dtype=BF16).astype(F32)
    hbm = pl.BlockSpec(memory_space=pl.ANY)
    scratch = [
        pltpu.VMEM((S, D), BF16),
        pltpu.VMEM((S, D), BF16),
        pltpu.VMEM((D, D), BF16),
        pltpu.VMEM((H // 2, S // 2, 128), U32),
        pltpu.VMEM((2, H // 2, 16, S), U32),
        pltpu.VMEM((2, H // 2, 24, S), F32),
        pltpu.VMEM((S, D), F32),
        pltpu.VMEM((S, 128), F32),
        pltpu.VMEM((NG, NB, 16, D), F32),
        pltpu.VMEM((NG, NB, 16, D), F32),
        pltpu.VMEM((H // 2, R, 128), F32),
        pltpu.VMEM((2, DH, R, 128), F32),
        pltpu.VMEM((H // 2, 2 * DH, S), F32),
        pltpu.VMEM((2, DH, 8, S + 128), F32),
        pltpu.VMEM((4, 8, 128), F32),
        pltpu.VMEM((BLK, 2 * BLK), F32),
        pltpu.SMEM((1,), F32),
        pltpu.SemaphoreType.DMA((NSEM,)),
    ]
    return pl.pallas_call(
        _kernel,
        out_shape=jax.ShapeDtypeStruct((1, S, D), BF16),
        in_specs=[hbm] * 11,
        out_specs=hbm,
        scratch_shapes=scratch,
        compiler_params=pltpu.CompilerParams(vmem_limit_bytes=127 * 1024 * 1024),
    )(A_q, A_k, A_v, A_shift_k.T, A_ssm_k, A_ssm_D, B_wqkv, B_wo, gate_w, fwd, inv)
```

```python
import math

import jax
import jax.numpy as jnp
import numpy as np
import jax.experimental.pallas as pl
import jax.experimental.pallas.tpu as pltpu

S = 2048
D = 640
H = 32
DH = 20
KS = 4
NCH = D // 128
BLK = 128
NB = S // BLK
NG = BLK // 8
CK = 128
SB = 512
NC = S // CK
NSB = S // SB
NU = NC * NSB
RB = 256
NRB = S // RB
NPEEL = 3
QB = 512
NQB = S // QB
R = 288
R0 = 256
SM = S - R
PK, PQ = 32, 256
AE = 3
FE = 2
SQ = 256
SCORE_BOUND = 80.0
F32 = jnp.float32
BF16 = jnp.bfloat16
U32 = jnp.uint32
I32 = jnp.int32
NT = (((1,), (1,)), ((), ()))

SEM_WK, SEM_WQ, SEM_WV, SEM_WO, SEM_OUT = 0, 1, 2, 3, 4
SEM_GW, SEM_SHK, SEM_SSD, SEM_FWD, SEM_INV = 5, 6, 7, 8, 9
SEM_X = 10
SEM_K = SEM_X + NRB
SEM_V = SEM_K + NQB
SEM_H = SEM_V + NQB
NSEM = SEM_H + NQB


def _dft_consts():
    f = np.concatenate([np.arange(0, BLK, 2), np.arange(1, BLK, 2)]).astype(np.float64)
    n = np.arange(BLK, dtype=np.float64)
    ang = 2.0 * np.pi * (f[:, None] + 0.5) * n[None, :] / (2 * BLK)
    re = np.cos(ang).reshape(NG, 8, BLK)
    im = -np.sin(ang).reshape(NG, 8, BLK)
    fwd = np.concatenate([re, im], axis=1).reshape(2 * BLK, BLK)
    inv = fwd.T / BLK
    return fwd, inv


def _timeline(steps, t1, edges):
    total = sum(w for w, _ in steps)
    out = {}
    acc = 0
    for w, p in steps:
        cyc = t1 * acc / total / NU * edges[-1]
        acc += w
        u = max(i for i in range(NU) if edges[i] <= cyc)
        out.setdefault(u, []).append(((cyc - edges[u]) / (edges[u + 1] - edges[u]), p))
    return out


def _kernel(x_hbm, k_hbm, v_hbm, shk_hbm, h_hbm, ssd_hbm, w_hbm, wo_hbm, gw_hbm,
            fwd_hbm, inv_hbm, out_hbm,
            x_v, k_v, wo_v, kp_s, qh_s, vt_s, kv_s, g_s, uf_s, hf_s,
            kfp, kb_s, qf_s, qb_s, bd_s, inv_ref, fl_s, sems):
    out_v = k_v
    cp_wo = pltpu.make_async_copy(wo_hbm, wo_v, sems.at[SEM_WO])
    cp_inv = pltpu.make_async_copy(inv_hbm, inv_ref, sems.at[SEM_INV])

    def build_kb(j, par, d, anchor=None, lo=0):
        t = jnp.full((8, 128), par * DH + d, I32)
        if anchor is not None:
            t = anchor(t) & 127
        idx = jnp.concatenate([t] * ((R - lo) // 8), axis=0)
        kb_s[par, d, lo:R, :] = jnp.take_along_axis(
            kfp[j, lo:R, :], idx, axis=1, mode="promise_in_bounds")

    def pre_phase(v_v, h_v, w_v, wt_s, kf_s, hp_s, kn_s, fwd_ref, shk_ref, ssd_ref, gw_ref):
        def w_copy(part, sem):
            return pltpu.make_async_copy(w_hbm.at[:, part * D:(part + 1) * D],
                                         w_v.at[:, part * D:(part + 1) * D], sems.at[sem])

        def x_copy(i):
            r0 = pl.multiple_of(i * RB, RB)
            return pltpu.make_async_copy(x_hbm.at[0, pl.ds(r0, RB), :],
                                         x_v.at[pl.ds(r0, RB), :], sems.at[SEM_X + i])

        def kvh_copies(i):
            r0 = pl.multiple_of(i * QB, QB)
            return (
                pltpu.make_async_copy(k_hbm.at[0, pl.ds(r0, QB), :],
                                      k_v.at[pl.ds(r0, QB), :], sems.at[SEM_K + i]),
                pltpu.make_async_copy(v_hbm.at[0, pl.ds(r0, QB), :],
                                      v_v.at[pl.ds(r0, QB), :], sems.at[SEM_V + i]),
                pltpu.make_async_copy(h_hbm.at[:, pl.ds(r0, QB)],
                                      h_v.at[:, pl.ds(r0, QB)], sems.at[SEM_H + i]),
            )

        cp_gw = pltpu.make_async_copy(gw_hbm, gw_ref, sems.at[SEM_GW])
        cp_small = (
            pltpu.make_async_copy(shk_hbm, shk_ref, sems.at[SEM_SHK]),
            pltpu.make_async_copy(ssd_hbm, ssd_ref, sems.at[SEM_SSD]),
            pltpu.make_async_copy(fwd_hbm, fwd_ref, sems.at[SEM_FWD]),
        )
        x_copy(0).start()
        w_copy(1, SEM_WK).start()
        cp_gw.start()
        for i in range(1, NRB):
            x_copy(i).start()
        for cp in cp_small:
            cp.start()
        w_copy(0, SEM_WQ).start()
        w_copy(2, SEM_WV).start()
        for i in range(NQB):
            for cp in kvh_copies(i):
                cp.start()
        cp_wo.start()
        cp_inv.start()

        kf_s[0:8, :] = jnp.zeros((8, D), F32)
        hp_s[...] = jnp.zeros((2 * BLK, D), F32)
        bd_s[...] = jnp.zeros((4, 8, 128), F32)

        def track(i, val):
            a = jnp.abs(val)
            a = jnp.max(a.reshape(a.shape[0] // 8, 8, a.shape[1]), axis=0)
            m = bd_s[i]
            for c in range(a.shape[1] // 128):
                m = jnp.maximum(m, a[:, c * 128:(c + 1) * 128])
            bd_s[i] = m

        def split_pairs(val):
            lane = jax.lax.broadcasted_iota(I32, (val.shape[0], 128), 1)
            parts = [val[:, c * 128:(c + 1) * 128] for c in range(NCH)]
            out = []
            for j in range(H // 2):
                c, sh = divmod(2 * DH * j, 128)
                src = parts[c]
                if sh + 2 * DH > 128:
                    src = jnp.where(lane >= 64, src, parts[c + 1])
                out.append(pltpu.roll(src, 128 - sh, 1) if sh else src)
            return out

        def kproj(rb):
            r0 = pl.multiple_of(rb * RB, RB)
            xb = x_v[pl.ds(r0, RB), :]
            kk = jnp.dot(xb, w_v[:, D:2 * D], preferred_element_type=F32)
            track(0, kk)
            kp = pltpu.bitcast(kk.astype(BF16), U32)
            h0 = pl.multiple_of(rb * (RB // 2), RB // 2)
            kn_s[pl.ds(h0, RB // 2), :] = kp
            if isinstance(rb, int) and (rb + 1) * RB > SM:
                lo = max(SM, rb * RB)
                for j, part in enumerate(split_pairs(kp[(lo - rb * RB) // 2:, :])):
                    kfp[j, lo - SM:(rb + 1) * RB - SM, :] = pltpu.bitcast(part, BF16).astype(F32)
            gw = gw_ref[...].astype(F32).reshape(1, D)
            g = jax.nn.sigmoid(jnp.sum(xb.astype(F32) * gw, axis=-1, keepdims=True))
            g_s[pl.ds(r0, RB), :] = jnp.broadcast_to(g, (RB, 128))

        w_copy(1, SEM_WK).wait()
        cp_gw.wait()

        def kproj_loop(rb, carry):
            x_copy(rb).wait()
            kproj(rb)
            return carry

        jax.lax.fori_loop(0, NRB - NPEEL, kproj_loop, 0)
        for i in range(NRB - NPEEL, NRB):
            x_copy(i).wait()
        w_copy(0, SEM_WQ).wait()
        w_copy(2, SEM_WV).wait()
        for cp in cp_small:
            cp.wait()
        kproj(NRB - 1)
        wt_s[0:D, :] = w_v[:, 0:D].astype(F32).T.astype(BF16)
        wt_s[D:2 * D, :] = w_v[:, 2 * D:3 * D].astype(F32).T.astype(BF16)
        for i in range(NRB - 2, NRB - NPEEL - 1, -1):
            kproj(i)
        for d in range(DH):
            build_kb(0, 0, d, lo=R - R0)

        qscale = (DH ** -0.5) * math.log2(math.e)

        def fold(cur, prev):
            cur = cur.reshape(NG, 16, D)
            prev = prev.reshape(NG, 16, D)
            hg = NG // 2
            lo = jnp.concatenate(
                [cur[:hg, 0:8] - prev[:hg, 8:16], cur[:hg, 8:16] + prev[:hg, 0:8]], axis=1)
            hi = jnp.concatenate(
                [cur[hg:, 0:8] + prev[hg:, 8:16], cur[hg:, 8:16] - prev[hg:, 0:8]], axis=1)
            return jnp.concatenate([lo, hi], axis=0)

        def qvproj(rb, carry):
            for cp in kvh_copies(rb):
                cp.wait()
            ssd = ssd_ref[...].astype(F32).reshape(1, D)
            shk = shk_ref[...].astype(F32)
            r0 = pl.multiple_of(rb * QB, QB)

            def q_part(rs):
                xb = x_v[pl.ds(rs, RB), :]
                qt = jax.lax.dot_general(wt_s[0:D, :], xb, NT, preferred_element_type=F32)
                qt = qt * qscale
                track(1, qt)
                qf = qt.reshape(H // 2, 2 * DH, RB)
                row = jax.lax.broadcasted_iota(I32, (H // 2, 24, RB), 1)
                zpad = jnp.zeros((H // 2, 8, RB), F32)
                for par, win in ((0, jnp.where(row < DH, qf[:, 0:24], 0.0)),
                                 (1, jnp.where(row >= 4, qf[:, 16:40], 0.0))):
                    win = jnp.concatenate([win, zpad], axis=1).reshape(H // 2 * 32, RB)
                    qh_s[par, :, :, pl.ds(rs, RB)] = pltpu.bitcast(
                        win.astype(BF16), U32).reshape(H // 2, 16, RB)
                qf_s[:, :, pl.ds(rs, RB)] = qf
                for d in range(DH):
                    qb_s[0, d, :, pl.ds(rs, RB)] = jnp.broadcast_to(qf[0, d:d + 1, :], (8, RB))

            def v_part(rs):
                xb = x_v[pl.ds(rs, RB), :]
                vt = jax.lax.dot_general(wt_s[D:2 * D, :], xb, NT, preferred_element_type=F32)
                track(2, vt)
                vt = vt.reshape(H // 2, 2 * DH, RB)
                row = jax.lax.broadcasted_iota(I32, (H // 2, 24, RB), 1)
                vt_s[0, :, :, pl.ds(rs, RB)] = jnp.where(row < DH, vt[:, 0:24, :], 1.0)
                vt_s[1, :, :, pl.ds(rs, RB)] = jnp.where(row >= 4, vt[:, 16:40, :], 1.0)

            def k_split(rs):
                h0 = pl.multiple_of(rs // 2, RB // 2)
                for j, part in enumerate(split_pairs(kn_s[pl.ds(h0, RB // 2), :])):
                    kp_s[j, pl.ds(h0, RB // 2), :] = part

            def u_part(u, ktail):
                ru = pl.multiple_of(r0 + u * BLK, BLK)
                kc = k_v[pl.ds(ru, BLK), :].astype(F32)
                e3 = jnp.concatenate([ktail, kc], axis=0).reshape(BLK // 8 + 1, 8, D)
                sub = jax.lax.broadcasted_iota(I32, (BLK // 8, 8, D), 1)
                ksh = kc * shk[0:1, :]
                for j in range(1, KS):
                    rot = pltpu.roll(e3, j, 1)
                    sh = jnp.where(sub >= j, rot[1:], rot[:-1]).reshape(BLK, D)
                    ksh = ksh + sh * shk[j:j + 1, :]
                kv = ksh * v_v[pl.ds(ru, BLK), :].astype(F32)
                kv_s[pl.ds(ru, BLK), :] = kv * ssd
                uf_s[:, rb * (QB // BLK) + u] = jnp.dot(
                    fwd_ref[...], kv.astype(BF16),
                    preferred_element_type=F32).reshape(NG, 16, D)
                return kc[BLK - 8:, :]

            def h_part(u, prev):
                ru = pl.multiple_of(r0 + u * BLK, BLK)
                raw = jax.lax.dot_general(fwd_ref[...], h_v[:, pl.ds(ru, BLK)], NT,
                                          preferred_element_type=F32)
                hf_s[:, rb * (QB // BLK) + u] = fold(raw, prev)
                return raw

            ktail = kf_s[0:8, :]
            prev = hp_s[...]
            for sub in range(QB // RB):
                rs = pl.multiple_of(r0 + sub * RB, RB)
                k_split(rs)
                q_part(rs)
                ktail = u_part(2 * sub, ktail)
                prev = h_part(2 * sub, prev)
                prev = h_part(2 * sub + 1, prev)
                if sub == QB // RB - 1:
                    hp_s[...] = prev
                v_part(rs)
                ktail = u_part(2 * sub + 1, ktail)
            kf_s[0:8, :] = ktail
            return carry + rb

        fl_s[0] = jax.lax.fori_loop(0, NQB, qvproj, jnp.int32(0))

    pl.run_scoped(
        pre_phase,
        pltpu.VMEM((S, D), BF16),
        pltpu.VMEM((D, S), BF16),
        pltpu.VMEM((D, 3 * D), BF16),
        pltpu.VMEM((2 * D, D), BF16),
        pltpu.VMEM((32, D), F32),
        pltpu.VMEM((2 * BLK, D), F32),
        pltpu.VMEM((S // 2, D), U32),
        pltpu.VMEM((2 * BLK, BLK), BF16),
        pltpu.VMEM((KS, D), BF16),
        pltpu.VMEM((D,), BF16),
        pltpu.VMEM((D,), BF16),
    )

    def post_phase(s2, m2, zf_s, ot_s, ss):
        def freq_steps(g, chunks):
            steps = []
            for c in chunks:
                cols = slice(c * 128, (c + 1) * 128) if isinstance(c, int) else c
                for i in range(NB):
                    st = {}
                    for m0 in range(0, i + 1, FE):
                        ms = list(range(m0, min(i + 1, m0 + FE)))

                        def step(anchor, i=i, cols=cols, ms=ms, st=st):
                            for m in ms:
                                ur = uf_s[g, m, 0:8, cols]
                                ui = uf_s[g, m, 8:16, cols]
                                hr = hf_s[g, i - m, 0:8, cols]
                                hi = hf_s[g, i - m, 8:16, cols]
                                if m == ms[0]:
                                    ur = anchor(ur)
                                tr = ur * hr - ui * hi
                                ti = ur * hi + ui * hr
                                st["r"] = tr if m == 0 else st["r"] + tr
                                st["i"] = ti if m == 0 else st["i"] + ti
                            if ms[-1] == i:
                                zf_s[g, i, 0:8, cols] = st["r"]
                                zf_s[g, i, 8:16, cols] = st["i"]
                        steps.append((len(ms), step))
            return steps

        kmax = jnp.max(bd_s[0])
        qmax = jnp.max(bd_s[1])
        vmax = jnp.max(bd_s[2])
        live = fl_s[0] >= 0

        def tie_to(tie):
            def anchor(v):
                t = tie if tie.dtype == v.dtype else pltpu.bitcast(tie, v.dtype)
                if v.shape[0] > 8:
                    t = jnp.concatenate([t] * (v.shape[0] // 8), axis=0)
                return jnp.where(live, v, t)
            return anchor

        def stage(h_qk, par_qk, h_pv, fsteps, rv=R):
            par_pv = 1 - par_qk
            bounds = [min(S - rv, (((S - rv) * c // NC) + 15) // 16 * 16) for c in range(NC + 1)]
            jq = h_qk >> 1
            j_nx = 0 if isinstance(h_qk, int) else jnp.minimum(h_qk + 1, H - 1) >> 1
            edges = [0]
            for u in range(NU):
                edges.append(edges[-1] + bounds[u % NC + 1] - bounds[u % NC]
                             + (24 if h_pv is not None else 0))
            ftl = _timeline(fsteps, NU * (1 - 0.008), edges)

            def prep_q(anchor, t):
                tc = slice(t * 128, (t + 1) * 128)
                blk = anchor(qf_s[j_nx, par_pv * 16:par_pv * 16 + 24, tc])
                for d in range(DH):
                    rr = par_pv * 4 + d
                    qb_s[par_pv, d, :, tc] = jnp.broadcast_to(blk[rr:rr + 1, :], (8, 128))

            psteps = []
            for i in range(DH):
                psteps.append((1, lambda anchor, i=i: build_kb(j_nx, par_pv, i, anchor)))
                if i < S // 128:
                    psteps.append((1, lambda anchor, i=i: prep_q(anchor, i)))
            ptl = _timeline(psteps, NU * (1 - 0.06), edges)
            if h_pv is not None:
                j = h_pv >> 1

            vsteps = []
            for sb in range(NSB):
                for k0 in range(R - rv, R, PK):
                    for qq in range(SB // PQ):
                        st = {}
                        for d0 in range(0, DH, AE):
                            def step(anchor, k0=k0, q0=sb * SB + qq * PQ, d0=d0, st=st):
                                for d in range(d0, min(DH, d0 + AE)):
                                    kb = kb_s[par_qk, d, k0:k0 + PK, :]
                                    if d == d0:
                                        w = (d0 // AE) % (PK // 8)
                                        kb = jnp.concatenate(
                                            [anchor(kb[i * 8:(i + 1) * 8]) if i == w
                                             else kb[i * 8:(i + 1) * 8]
                                             for i in range(PK // 8)], axis=0)
                                    qr = qb_s[par_qk, d, :, q0:q0 + PQ]
                                    t = (jnp.concatenate([kb] * (PQ // 128), axis=1)
                                         * jnp.concatenate([qr] * (PK // 8), axis=0))
                                    st["a"] = t if d == 0 else st["a"] + t
                                if d0 + AE >= DH:
                                    s2[par_qk, SM + k0:SM + k0 + PK,
                                       q0:q0 + PQ] = jnp.exp2(st["a"])
                            vsteps.append((min(DH, d0 + AE) - d0, step))
            vtl = _timeline(vsteps, NU - 0.25, edges)

            acc = None
            for sb in range(NSB):
                cols = slice(sb * SB, (sb + 1) * SB)
                for c in range(NC):
                    u = sb * NC + c
                    r0, r1 = bounds[c], bounds[c + 1]
                    kc = pltpu.bitcast(kp_s[jq, r0 // 2:r1 // 2, :], BF16)
                    qt = qh_s[par_qk, jq, :, cols]
                    if par_qk == 1:
                        qt = jnp.concatenate([jnp.zeros((8, SB), U32), qt], axis=0)
                    qt = pltpu.bitcast(qt, BF16)
                    s = jnp.dot(kc[:, 0:qt.shape[0]], qt, preferred_element_type=F32)
                    s2[par_qk, r0:r1, cols] = jnp.exp2(s)
                    ties = s
                    if h_pv is not None:
                        ct, kq = divmod(u, NSB)
                        pc = slice(ct * 128, (ct + 1) * 128)
                        rs = [jnp.dot(vt_s[par_pv, j, :, kq * SB + i * CK:kq * SB + (i + 1) * CK],
                                      s2[par_pv, kq * SB + i * CK:kq * SB + (i + 1) * CK, pc],
                                      preferred_element_type=F32) for i in range(SB // CK)]
                        if kq == 0:
                            z = tie_to(s[0:8, 0:128])(jnp.zeros((8, 128), F32))
                            acc = jnp.concatenate([z] * 3, axis=0)
                        for rr in rs:
                            acc = acc + rr
                        if kq == NSB - 1:
                            ot_s[par_pv, j, :, pc] = acc
                        if u < NU - 1:
                            ties = jnp.concatenate([s, jnp.concatenate(rs, axis=1)], axis=0)
                    ng = ties.shape[0] // 8
                    for col, tl in ((0, vtl.get(u, [])), (1, ptl.get(u, [])), (2, ftl.get(u, []))):
                        for frac, p in tl:
                            gi = min(ng - 1, int(frac * ng))
                            p(tie_to(ties[gi * 8:(gi + 1) * 8, col * 128:(col + 1) * 128]))

        def fast_path():
            def body(i, carry):
                stage(2 * i + 1, 1, 2 * i, freq_steps(i, (2, 3, 4)))

                @pl.when(i < H // 2 - 1)
                def _():
                    stage(2 * i + 2, 0, 2 * i + 1, freq_steps(i + 1, (0, 1)))
                return carry

            jax.lax.fori_loop(0, H // 2, body, 0)

        def slow_path():
            nq = S // SQ

            def block(it_qk, it_pv, wbuf):
                rbuf = 1 - wbuf
                h = it_qk // nq
                c0 = pl.multiple_of((it_qk % nq) * SQ, SQ)
                q32 = qh_s[h & 1, h >> 1, :, pl.ds(c0, SQ)]
                z = jnp.zeros((8, SQ), U32)
                qt = pltpu.bitcast(jnp.where((h & 1) == 1, jnp.concatenate([z, q32], axis=0),
                                             jnp.concatenate([q32, z], axis=0)), BF16)
                hp = it_pv // nq
                cp = pl.multiple_of((it_pv % nq) * SQ, SQ)
                m = jnp.max(m2[rbuf], axis=0, keepdims=True)
                mx = None
                acc = None
                for c in range(S // SQ):
                    rows = slice(c * SQ, (c + 1) * SQ)
                    kc = pltpu.bitcast(kp_s[h >> 1, c * SQ // 2:(c + 1) * SQ // 2, :], BF16)
                    s = jnp.dot(kc[:, 0:48], qt, preferred_element_type=F32)
                    ss[wbuf, rows, :] = s
                    cm = jnp.max(s.reshape(SQ // 8, 8, SQ), axis=0)
                    mx = cm if mx is None else jnp.maximum(mx, cm)
                    p = jnp.exp2(ss[rbuf, rows, :] - m)
                    s2[1, rows, pl.ds(cp, SQ)] = p
                    r = jnp.dot(vt_s[hp & 1, hp >> 1, :, rows], p, preferred_element_type=F32)
                    acc = r if acc is None else acc + r
                m2[wbuf] = mx
                ot_s[hp & 1, hp >> 1, :, pl.ds(cp, SQ)] = acc

            ss[1] = jnp.zeros((S, SQ), F32)
            m2[1] = jnp.zeros((8, SQ), F32)

            def body(it, carry):
                cur = jnp.minimum(it, H * nq - 1)
                prv = jnp.maximum(it - 1, 0)

                @pl.when((it & 1) == 0)
                def _():
                    block(cur, prv, 0)

                @pl.when((it & 1) == 1)
                def _():
                    block(cur, prv, 1)
                return carry

            jax.lax.fori_loop(0, H * nq + 1, body, 0)

            def fbody(i, carry):
                cols = pl.ds(pl.multiple_of((i % NCH) * 128, 128), 128)
                for _, p in freq_steps(i // NCH, (cols,)):
                    p(lambda v: v)
                return carry

            jax.lax.fori_loop(0, NG * NCH, fbody, 0)

        safe = jnp.logical_and(
            kmax * qmax * (1.02 * DH) <= SCORE_BOUND,
            jnp.logical_and(vmax <= 2.0 ** 30, vmax >= 2.0 ** -20))

        stage(0, 0, None, freq_steps(0, (0, 1)), rv=R0)

        jax.lax.cond(safe, fast_path, slow_path)

        cp_inv.wait()
        cp_wo.wait()
        accs = [None] * NSB
        ga = {}

        def pv_last(sb, c):
            cols = slice(sb * SB, (sb + 1) * SB)
            r = jnp.dot(vt_s[1, H // 2 - 1, :, c * CK:(c + 1) * CK],
                        s2[1, c * CK:(c + 1) * CK, cols], preferred_element_type=F32)
            accs[sb] = r if accs[sb] is None else accs[sb] + r

        def inv_block(i):
            rows = slice(i * BLK, (i + 1) * BLK)
            y = jnp.dot(inv_ref[...], zf_s[:, i].reshape(2 * BLK, D), preferred_element_type=F32)
            gx = x_v[rows, :].astype(F32) * jnp.concatenate([g_s[rows, :]] * NCH, axis=1)
            ga[i] = gx * (y + kv_s[rows, :])

        def out_block(i):
            sb, ii = divmod(i, SB // BLK)
            rows = slice(i * BLK, (i + 1) * BLK)
            oe = ot_s[0, :, :, rows]
            oo = jnp.concatenate([ot_s[1, 0:H // 2 - 1, :, rows],
                                  accs[sb][None, :, ii * BLK:(ii + 1) * BLK]], axis=0)
            low = jax.lax.broadcasted_iota(I32, (H // 2, 8, BLK), 1) < 4
            den = jnp.where(low, oo[:, 0:8], oe[:, 16:24])
            inv = pl.reciprocal(den, approx=True)
            inv = inv * (2.0 - den * inv)
            o = jnp.concatenate(
                [oe[:, 0:16] * inv[:, 4:5],
                 jnp.where(low, oe[:, 16:24], oo[:, 0:8]) * pltpu.roll(inv, 4, 1),
                 oo[:, 8:24] * inv[:, 0:1]], axis=1)
            o = o.reshape(D, BLK).T.astype(BF16)
            bb = jnp.dot(o, wo_v[...], preferred_element_type=F32)
            g1 = 1.0 - g_s[rows, :]
            out_v[rows, :] = (ga[i] + jnp.concatenate([g1] * NCH, axis=1) * bb).astype(BF16)
            pltpu.make_async_copy(out_v.at[rows, :], out_hbm.at[0, rows, :],
                                  sems.at[SEM_OUT]).start()

        nb = SB // BLK
        for i in range(nb):
            if i < nb - 1:
                for c in range(i * NC // (nb - 1), (i + 1) * NC // (nb - 1)):
                    pv_last(0, c)
            inv_block(i)
        for i in range(NB):
            out_block(i)
            sb, ii = divmod(i, nb)
            if sb + 1 < NSB:
                for c in range(ii * NC // nb, (ii + 1) * NC // nb):
                    pv_last(sb + 1, c)
                inv_block(i + nb)
        pltpu.make_async_copy(out_v, out_hbm.at[0], sems.at[SEM_OUT]).wait()

    pl.run_scoped(
        post_phase,
        pltpu.VMEM((2, S, S + 128), F32),
        pltpu.VMEM((2, 8, SQ), F32),
        pltpu.VMEM((NG, NB, 16, D), F32),
        pltpu.VMEM((2, H // 2, 24, S), F32),
        pltpu.VMEM((2, S, SQ), F32),
    )


@jax.jit
def pallas_gated_mix__ssm_conv_h3__mha_block__prompt_kernel(
    A_q: jax.Array,
    A_k: jax.Array,
    A_v: jax.Array,
    A_shift_k: jax.Array,
    A_ssm_k: jax.Array,
    A_ssm_D: jax.Array,
    B_x: jax.Array,
    B_wqkv: jax.Array,
    B_wo: jax.Array,
    gate_w: jax.Array,
):
    fwd, inv = _dft_consts()
    fwd = jnp.asarray(fwd, dtype=BF16)
    inv = jnp.asarray(inv, dtype=BF16).astype(F32)
    hbm = pl.BlockSpec(memory_space=pl.ANY)
    scratch = [
        pltpu.VMEM((S, D), BF16),
        pltpu.VMEM((S, D), BF16),
        pltpu.VMEM((D, D), BF16),
        pltpu.VMEM((H // 2, S // 2, 128), U32),
        pltpu.VMEM((2, H // 2, 16, S), U32),
        pltpu.VMEM((2, H // 2, 24, S), F32),
        pltpu.VMEM((S, D), F32),
        pltpu.VMEM((S, 128), F32),
        pltpu.VMEM((NG, NB, 16, D), F32),
        pltpu.VMEM((NG, NB, 16, D), F32),
        pltpu.VMEM((H // 2, R, 128), F32),
        pltpu.VMEM((2, DH, R, 128), F32),
        pltpu.VMEM((H // 2, 2 * DH, S), F32),
        pltpu.VMEM((2, DH, 8, S + 128), F32),
        pltpu.VMEM((4, 8, 128), F32),
        pltpu.VMEM((BLK, 2 * BLK), F32),
        pltpu.SMEM((1,), I32),
        pltpu.SemaphoreType.DMA((NSEM,)),
    ]
    return pl.pallas_call(
        _kernel,
        out_shape=jax.ShapeDtypeStruct((1, S, D), BF16),
        in_specs=[hbm] * 11,
        out_specs=hbm,
        scratch_shapes=scratch,
        compiler_params=pltpu.CompilerParams(vmem_limit_bytes=127 * 1024 * 1024),
    )(A_q, A_k, A_v, A_shift_k.T, A_ssm_k, A_ssm_D, B_wqkv, B_wo, gate_w, fwd, inv)
```

```python
import math

import jax
import jax.numpy as jnp
import numpy as np
import jax.experimental.pallas as pl
import jax.experimental.pallas.tpu as pltpu

S = 2048
D = 640
H = 32
DH = 20
KS = 4
NCH = D // 128
BLK = 128
NB = S // BLK
NG = BLK // 8
CK = 128
SB = 512
NC = S // CK
NSB = S // SB
NU = NC * NSB
RB = 256
NRB = S // RB
NPEEL = 3
QB = 512
NQB = S // QB
R = 288
R0 = 256
SM = S - R
PK, PQ = 32, 256
AE = 3
FE = 2
MA, MB = 2, 4
WA = 256
SQ = 128
SK = 512
SCORE_BOUND = 80.0
F32 = jnp.float32
BF16 = jnp.bfloat16
U32 = jnp.uint32
I32 = jnp.int32
NT = (((1,), (1,)), ((), ()))

SEM_WK, SEM_WQ, SEM_WV, SEM_WO, SEM_OUT = 0, 1, 2, 3, 4
SEM_GW, SEM_SHK, SEM_SSD, SEM_FWD, SEM_INV = 5, 6, 7, 8, 9
SEM_WK2 = 10
SEM_X = 11
SEM_K = SEM_X + NRB
SEM_V = SEM_K + NQB
SEM_H = SEM_V + NQB
NSEM = SEM_H + NQB


def _dft_consts():
    f = np.concatenate([np.arange(0, BLK, 2), np.arange(1, BLK, 2)]).astype(np.float64)
    n = np.arange(BLK, dtype=np.float64)
    ang = 2.0 * np.pi * (f[:, None] + 0.5) * n[None, :] / (2 * BLK)
    re = np.cos(ang).reshape(NG, 8, BLK)
    im = -np.sin(ang).reshape(NG, 8, BLK)
    fwd = np.concatenate([re, im], axis=1).reshape(2 * BLK, BLK)
    inv = fwd.T / BLK
    return fwd, inv


def _timeline(steps, t1, edges):
    total = sum(w for w, _ in steps)
    out = {}
    acc = 0
    for w, p in steps:
        cyc = t1 * acc / total / NU * edges[-1]
        acc += w
        u = max(i for i in range(NU) if edges[i] <= cyc)
        out.setdefault(u, []).append(((cyc - edges[u]) / (edges[u + 1] - edges[u]), p))
    return out


def _kernel(x_hbm, k_hbm, v_hbm, shk_hbm, h_hbm, ssd_hbm, w_hbm, wo_hbm, gw_hbm,
            fwd_hbm, inv_hbm, out_hbm,
            x_v, k_v, wo_v, kp_s, qh_s, vt_s, kv_s, g_s, uf_s, hf_s,
            kfp, kb_s, qf_s, qb_s, bd_s, inv_ref, fl_s, sems):
    out_v = k_v
    cp_wo = pltpu.make_async_copy(wo_hbm, wo_v, sems.at[SEM_WO])
    cp_inv = pltpu.make_async_copy(inv_hbm, inv_ref, sems.at[SEM_INV])

    def build_kb(j, par, d, anchor=None, lo=0):
        t = jnp.full((8, 128), par * DH + d, I32)
        if anchor is not None:
            t = anchor(t) & 127
        idx = jnp.concatenate([t] * ((R - lo) // 8), axis=0)
        kb_s[par, d, lo:R, :] = jnp.take_along_axis(
            kfp[j, lo:R, :], idx, axis=1, mode="promise_in_bounds")

    def pre_phase(v_v, h_v, w_v, wt_s, kf_s, hp_s, kn_s, fwd_ref, shk_ref, ssd_ref, gw_ref):
        def w_copy(part, sem):
            return pltpu.make_async_copy(w_hbm.at[:, part * D:(part + 1) * D],
                                         w_v.at[:, part * D:(part + 1) * D], sems.at[sem])

        def wk_copy(lo, hi, sem):
            return pltpu.make_async_copy(w_hbm.at[:, D + lo:D + hi],
                                         w_v.at[:, D + lo:D + hi], sems.at[sem])

        def x_copy(i):
            r0 = pl.multiple_of(i * RB, RB)
            return pltpu.make_async_copy(x_hbm.at[0, pl.ds(r0, RB), :],
                                         x_v.at[pl.ds(r0, RB), :], sems.at[SEM_X + i])

        def kvh_copies(i):
            r0 = pl.multiple_of(i * QB, QB)
            return (
                pltpu.make_async_copy(k_hbm.at[0, pl.ds(r0, QB), :],
                                      k_v.at[pl.ds(r0, QB), :], sems.at[SEM_K + i]),
                pltpu.make_async_copy(v_hbm.at[0, pl.ds(r0, QB), :],
                                      v_v.at[pl.ds(r0, QB), :], sems.at[SEM_V + i]),
                pltpu.make_async_copy(h_hbm.at[:, pl.ds(r0, QB)],
                                      h_v.at[:, pl.ds(r0, QB)], sems.at[SEM_H + i]),
            )

        cp_gw = pltpu.make_async_copy(gw_hbm, gw_ref, sems.at[SEM_GW])
        cp_small = (
            pltpu.make_async_copy(shk_hbm, shk_ref, sems.at[SEM_SHK]),
            pltpu.make_async_copy(ssd_hbm, ssd_ref, sems.at[SEM_SSD]),
            pltpu.make_async_copy(fwd_hbm, fwd_ref, sems.at[SEM_FWD]),
        )
        cp_gw.start()
        x_copy(0).start()
        wk_copy(0, WA, SEM_WK).start()
        wk_copy(WA, D, SEM_WK2).start()
        for i in range(1, NRB):
            x_copy(i).start()
        for cp in cp_small:
            cp.start()
        w_copy(0, SEM_WQ).start()
        w_copy(2, SEM_WV).start()
        for i in range(NQB):
            for cp in kvh_copies(i):
                cp.start()
        cp_wo.start()
        cp_inv.start()

        kf_s[0:8, :] = jnp.zeros((8, D), F32)
        hp_s[...] = jnp.zeros((2 * BLK, D), F32)
        bd_s[...] = jnp.zeros((4, 8, 128), F32)

        def track(i, val):
            a = jnp.abs(val)
            a = jnp.max(a.reshape(a.shape[0] // 8, 8, a.shape[1]), axis=0)
            m = bd_s[i]
            for c in range(a.shape[1] // 128):
                m = jnp.maximum(m, a[:, c * 128:(c + 1) * 128])
            bd_s[i] = m

        def split_pairs(val):
            lane = jax.lax.broadcasted_iota(I32, (val.shape[0], 128), 1)
            parts = [val[:, c * 128:(c + 1) * 128] for c in range(NCH)]
            out = []
            for j in range(H // 2):
                c, sh = divmod(2 * DH * j, 128)
                src = parts[c]
                if sh + 2 * DH > 128:
                    src = jnp.where(lane >= 64, src, parts[c + 1])
                out.append(pltpu.roll(src, 128 - sh, 1) if sh else src)
            return out

        def gate(r0):
            gw = gw_ref[...].astype(F32).reshape(1, D)
            xb = x_v[pl.ds(r0, RB), :].astype(F32)
            g = jax.nn.sigmoid(jnp.sum(xb * gw, axis=-1, keepdims=True))
            g_s[pl.ds(r0, RB), :] = jnp.broadcast_to(g, (RB, 128))

        def kproj(rb, head=None):
            r0 = pl.multiple_of(rb * RB, RB)
            xb = x_v[pl.ds(r0, RB), :]
            if head is None:
                kk = jnp.dot(xb, w_v[:, D:2 * D], preferred_element_type=F32)
            else:
                rest = jnp.concatenate(
                    [jnp.dot(xb[i * RB // MB:(i + 1) * RB // MB], w_v[:, D + WA:2 * D],
                             preferred_element_type=F32) for i in range(MB)], axis=0)
                kk = jnp.concatenate([head, rest], axis=1)
            track(0, kk)
            kp = pltpu.bitcast(kk.astype(BF16), U32)
            h0 = pl.multiple_of(rb * (RB // 2), RB // 2)
            kn_s[pl.ds(h0, RB // 2), :] = kp
            if isinstance(rb, int) and (rb + 1) * RB > SM:
                lo = max(SM, rb * RB)
                for j, part in enumerate(split_pairs(kp[(lo - rb * RB) // 2:, :])):
                    kfp[j, lo - SM:(rb + 1) * RB - SM, :] = pltpu.bitcast(part, BF16).astype(F32)
            if head is None:
                gate(r0)

        cp_gw.wait()
        x_copy(0).wait()
        gate(0)
        wk_copy(0, WA, SEM_WK).wait()
        head = jnp.concatenate(
            [jnp.dot(x_v[i * RB // MA:(i + 1) * RB // MA, :], w_v[:, D:D + WA],
                     preferred_element_type=F32) for i in range(MA)], axis=0)
        wk_copy(WA, D, SEM_WK2).wait()
        kproj(0, head)

        def kproj_loop(rb, carry):
            x_copy(rb).wait()
            kproj(rb)
            return carry

        jax.lax.fori_loop(1, NRB - NPEEL, kproj_loop, 0)
        for i in range(NRB - NPEEL, NRB):
            x_copy(i).wait()
        w_copy(0, SEM_WQ).wait()
        w_copy(2, SEM_WV).wait()
        for cp in cp_small:
            cp.wait()
        kproj(NRB - 1)
        wt_s[0:D, :] = w_v[:, 0:D].astype(F32).T.astype(BF16)
        wt_s[D:2 * D, :] = w_v[:, 2 * D:3 * D].astype(F32).T.astype(BF16)
        for i in range(NRB - 2, NRB - NPEEL - 1, -1):
            kproj(i)
        for d in range(DH):
            build_kb(0, 0, d, lo=R - R0)

        qscale = (DH ** -0.5) * math.log2(math.e)

        def fold(cur, prev):
            cur = cur.reshape(NG, 16, D)
            prev = prev.reshape(NG, 16, D)
            hg = NG // 2
            lo = jnp.concatenate(
                [cur[:hg, 0:8] - prev[:hg, 8:16], cur[:hg, 8:16] + prev[:hg, 0:8]], axis=1)
            hi = jnp.concatenate(
                [cur[hg:, 0:8] + prev[hg:, 8:16], cur[hg:, 8:16] - prev[hg:, 0:8]], axis=1)
            return jnp.concatenate([lo, hi], axis=0)

        def qvproj(rb, carry):
            for cp in kvh_copies(rb):
                cp.wait()
            ssd = ssd_ref[...].astype(F32).reshape(1, D)
            shk = shk_ref[...].astype(F32)
            r0 = pl.multiple_of(rb * QB, QB)

            def q_part(rs):
                xb = x_v[pl.ds(rs, RB), :]
                qt = jax.lax.dot_general(wt_s[0:D, :], xb, NT, preferred_element_type=F32)
                qt = qt * qscale
                track(1, qt)
                qf = qt.reshape(H // 2, 2 * DH, RB)
                row = jax.lax.broadcasted_iota(I32, (H // 2, 24, RB), 1)
                zpad = jnp.zeros((H // 2, 8, RB), F32)
                for par, win in ((0, jnp.where(row < DH, qf[:, 0:24], 0.0)),
                                 (1, jnp.where(row >= 4, qf[:, 16:40], 0.0))):
                    win = jnp.concatenate([win, zpad], axis=1).reshape(H // 2 * 32, RB)
                    qh_s[par, :, :, pl.ds(rs, RB)] = pltpu.bitcast(
                        win.astype(BF16), U32).reshape(H // 2, 16, RB)
                qf_s[:, :, pl.ds(rs, RB)] = qf
                for d in range(DH):
                    qb_s[0, d, :, pl.ds(rs, RB)] = jnp.broadcast_to(qf[0, d:d + 1, :], (8, RB))

            def v_part(rs):
                xb = x_v[pl.ds(rs, RB), :]
                vt = jax.lax.dot_general(wt_s[D:2 * D, :], xb, NT, preferred_element_type=F32)
                track(2, vt)
                vt = vt.reshape(H // 2, 2 * DH, RB)
                row = jax.lax.broadcasted_iota(I32, (H // 2, 24, RB), 1)
                vt_s[0, :, :, pl.ds(rs, RB)] = jnp.where(row < DH, vt[:, 0:24, :], 1.0)
                vt_s[1, :, :, pl.ds(rs, RB)] = jnp.where(row >= 4, vt[:, 16:40, :], 1.0)

            def k_split(rs):
                h0 = pl.multiple_of(rs // 2, RB // 2)
                for j, part in enumerate(split_pairs(kn_s[pl.ds(h0, RB // 2), :])):
                    kp_s[j, pl.ds(h0, RB // 2), :] = part

            def u_part(u, ktail):
                ru = pl.multiple_of(r0 + u * BLK, BLK)
                kc = k_v[pl.ds(ru, BLK), :].astype(F32)
                e3 = jnp.concatenate([ktail, kc], axis=0).reshape(BLK // 8 + 1, 8, D)
                sub = jax.lax.broadcasted_iota(I32, (BLK // 8, 8, D), 1)
                ksh = kc * shk[0:1, :]
                for j in range(1, KS):
                    rot = pltpu.roll(e3, j, 1)
                    sh = jnp.where(sub >= j, rot[1:], rot[:-1]).reshape(BLK, D)
                    ksh = ksh + sh * shk[j:j + 1, :]
                kv = ksh * v_v[pl.ds(ru, BLK), :].astype(F32)
                kv_s[pl.ds(ru, BLK), :] = kv * ssd
                uf_s[:, rb * (QB // BLK) + u] = jnp.dot(
                    fwd_ref[...], kv.astype(BF16),
                    preferred_element_type=F32).reshape(NG, 16, D)
                return kc[BLK - 8:, :]

            def h_part(u, prev):
                ru = pl.multiple_of(r0 + u * BLK, BLK)
                raw = jax.lax.dot_general(fwd_ref[...], h_v[:, pl.ds(ru, BLK)], NT,
                                          preferred_element_type=F32)
                hf_s[:, rb * (QB // BLK) + u] = fold(raw, prev)
                return raw

            ktail = kf_s[0:8, :]
            prev = hp_s[...]
            for sub in range(QB // RB):
                rs = pl.multiple_of(r0 + sub * RB, RB)
                k_split(rs)
                q_part(rs)
                ktail = u_part(2 * sub, ktail)
                prev = h_part(2 * sub, prev)
                prev = h_part(2 * sub + 1, prev)
                if sub == QB // RB - 1:
                    hp_s[...] = prev
                v_part(rs)
                ktail = u_part(2 * sub + 1, ktail)
            kf_s[0:8, :] = ktail
            return carry + rb

        fl_s[0] = jax.lax.fori_loop(0, NQB, qvproj, jnp.int32(0))

    pl.run_scoped(
        pre_phase,
        pltpu.VMEM((S, D), BF16),
        pltpu.VMEM((D, S), BF16),
        pltpu.VMEM((D, 3 * D), BF16),
        pltpu.VMEM((2 * D, D), BF16),
        pltpu.VMEM((32, D), F32),
        pltpu.VMEM((2 * BLK, D), F32),
        pltpu.VMEM((S // 2, D), U32),
        pltpu.VMEM((2 * BLK, BLK), BF16),
        pltpu.VMEM((KS, D), BF16),
        pltpu.VMEM((D,), BF16),
        pltpu.VMEM((D,), BF16),
    )

    def post_phase(s2, m2, zf_s, ot_s, ss):
        def freq_steps(g, chunks):
            steps = []
            for c in chunks:
                cols = slice(c * 128, (c + 1) * 128) if isinstance(c, int) else c
                for i in range(NB):
                    st = {}
                    for m0 in range(0, i + 1, FE):
                        ms = list(range(m0, min(i + 1, m0 + FE)))

                        def step(anchor, i=i, cols=cols, ms=ms, st=st):
                            for m in ms:
                                ur = uf_s[g, m, 0:8, cols]
                                ui = uf_s[g, m, 8:16, cols]
                                hr = hf_s[g, i - m, 0:8, cols]
                                hi = hf_s[g, i - m, 8:16, cols]
                                if m == ms[0]:
                                    ur = anchor(ur)
                                tr = ur * hr - ui * hi
                                ti = ur * hi + ui * hr
                                st["r"] = tr if m == 0 else st["r"] + tr
                                st["i"] = ti if m == 0 else st["i"] + ti
                            if ms[-1] == i:
                                zf_s[g, i, 0:8, cols] = st["r"]
                                zf_s[g, i, 8:16, cols] = st["i"]
                        steps.append((len(ms), step))
            return steps

        kmax = jnp.max(bd_s[0])
        qmax = jnp.max(bd_s[1])
        vmax = jnp.max(bd_s[2])
        live = fl_s[0] >= 0

        def tie_to(tie):
            def anchor(v):
                t = tie if tie.dtype == v.dtype else pltpu.bitcast(tie, v.dtype)
                if v.shape[0] > 8:
                    t = jnp.concatenate([t] * (v.shape[0] // 8), axis=0)
                return jnp.where(live, v, t)
            return anchor

        def stage(h_qk, par_qk, h_pv, fsteps, rv=R):
            par_pv = 1 - par_qk
            bounds = [min(S - rv, (((S - rv) * c // NC) + 15) // 16 * 16) for c in range(NC + 1)]
            jq = h_qk >> 1
            j_nx = 0 if isinstance(h_qk, int) else jnp.minimum(h_qk + 1, H - 1) >> 1
            edges = [0]
            for u in range(NU):
                edges.append(edges[-1] + bounds[u % NC + 1] - bounds[u % NC]
                             + (24 if h_pv is not None else 0))
            ftl = _timeline(fsteps, NU * (1 - 0.008), edges)

            def prep_q(anchor, t):
                tc = slice(t * 128, (t + 1) * 128)
                blk = anchor(qf_s[j_nx, par_pv * 16:par_pv * 16 + 24, tc])
                for d in range(DH):
                    rr = par_pv * 4 + d
                    qb_s[par_pv, d, :, tc] = jnp.broadcast_to(blk[rr:rr + 1, :], (8, 128))

            psteps = []
            for i in range(DH):
                psteps.append((1, lambda anchor, i=i: build_kb(j_nx, par_pv, i, anchor)))
                if i < S // 128:
                    psteps.append((1, lambda anchor, i=i: prep_q(anchor, i)))
            ptl = _timeline(psteps, NU * (1 - 0.06), edges)
            if h_pv is not None:
                j = h_pv >> 1

            vsteps = []
            for sb in range(NSB):
                for k0 in range(R - rv, R, PK):
                    for qq in range(SB // PQ):
                        st = {}
                        for d0 in range(0, DH, AE):
                            def step(anchor, k0=k0, q0=sb * SB + qq * PQ, d0=d0, st=st):
                                for d in range(d0, min(DH, d0 + AE)):
                                    kb = kb_s[par_qk, d, k0:k0 + PK, :]
                                    if d == d0:
                                        w = (d0 // AE) % (PK // 8)
                                        kb = jnp.concatenate(
                                            [anchor(kb[i * 8:(i + 1) * 8]) if i == w
                                             else kb[i * 8:(i + 1) * 8]
                                             for i in range(PK // 8)], axis=0)
                                    qr = qb_s[par_qk, d, :, q0:q0 + PQ]
                                    t = (jnp.concatenate([kb] * (PQ // 128), axis=1)
                                         * jnp.concatenate([qr] * (PK // 8), axis=0))
                                    st["a"] = t if d == 0 else st["a"] + t
                                if d0 + AE >= DH:
                                    s2[par_qk, SM + k0:SM + k0 + PK,
                                       q0:q0 + PQ] = jnp.exp2(st["a"])
                            vsteps.append((min(DH, d0 + AE) - d0, step))
            vtl = _timeline(vsteps, NU - 0.25, edges)

            acc = None
            for sb in range(NSB):
                cols = slice(sb * SB, (sb + 1) * SB)
                for c in range(NC):
                    u = sb * NC + c
                    r0, r1 = bounds[c], bounds[c + 1]
                    kc = pltpu.bitcast(kp_s[jq, r0 // 2:r1 // 2, :], BF16)
                    qt = qh_s[par_qk, jq, :, cols]
                    if par_qk == 1:
                        qt = jnp.concatenate([jnp.zeros((8, SB), U32), qt], axis=0)
                    qt = pltpu.bitcast(qt, BF16)
                    s = jnp.dot(kc[:, 0:qt.shape[0]], qt, preferred_element_type=F32)
                    s2[par_qk, r0:r1, cols] = jnp.exp2(s)
                    ties = s
                    if h_pv is not None:
                        ct, kq = divmod(u, NSB)
                        pc = slice(ct * 128, (ct + 1) * 128)
                        rs = [jnp.dot(vt_s[par_pv, j, :, kq * SB + i * CK:kq * SB + (i + 1) * CK],
                                      s2[par_pv, kq * SB + i * CK:kq * SB + (i + 1) * CK, pc],
                                      preferred_element_type=F32) for i in range(SB // CK)]
                        if kq == 0:
                            z = tie_to(s[0:8, 0:128])(jnp.zeros((8, 128), F32))
                            acc = jnp.concatenate([z] * 3, axis=0)
                        for rr in rs:
                            acc = acc + rr
                        if kq == NSB - 1:
                            ot_s[par_pv, j, :, pc] = acc
                        if u < NU - 1:
                            ties = jnp.concatenate([s, jnp.concatenate(rs, axis=1)], axis=0)
                    ng = ties.shape[0] // 8
                    for col, tl in ((0, vtl.get(u, [])), (1, ptl.get(u, [])), (2, ftl.get(u, []))):
                        for frac, p in tl:
                            gi = min(ng - 1, int(frac * ng))
                            p(tie_to(ties[gi * 8:(gi + 1) * 8, col * 128:(col + 1) * 128]))

        def fast_path():
            def body(i, carry):
                stage(2 * i + 1, 1, 2 * i, freq_steps(i, (2, 3, 4)))

                @pl.when(i < H // 2 - 1)
                def _():
                    stage(2 * i + 2, 0, 2 * i + 1, freq_steps(i + 1, (0, 1)))
                return carry

            jax.lax.fori_loop(0, H // 2, body, 0)

        def slow_path():
            nq = S // SQ

            def block(it_qk, it_pv, wbuf):
                rbuf = 1 - wbuf
                h = it_qk // nq
                c0 = pl.multiple_of((it_qk % nq) * SQ, SQ)
                q32 = qh_s[h & 1, h >> 1, :, pl.ds(c0, SQ)]
                z = jnp.zeros((8, SQ), U32)
                qt = pltpu.bitcast(jnp.where((h & 1) == 1, jnp.concatenate([z, q32], axis=0),
                                             jnp.concatenate([q32, z], axis=0)), BF16)
                hp = it_pv // nq
                cp = pl.multiple_of((it_pv % nq) * SQ, SQ)
                m = jnp.max(m2[rbuf], axis=0, keepdims=True)
                mx = None
                acc = None
                for c in range(S // SK):
                    rows = slice(c * SK, (c + 1) * SK)
                    kc = pltpu.bitcast(kp_s[h >> 1, c * SK // 2:(c + 1) * SK // 2, :], BF16)
                    s = jnp.dot(kc[:, 0:48], qt, preferred_element_type=F32)
                    ss[wbuf, rows, :] = s
                    cm = jnp.max(s.reshape(SK // 8, 8, SQ), axis=0)
                    mx = cm if mx is None else jnp.maximum(mx, cm)
                    p = jnp.exp2(ss[rbuf, rows, :] - m)
                    s2[1, rows, pl.ds(cp, SQ)] = p
                    r = jnp.dot(vt_s[hp & 1, hp >> 1, :, rows], p, preferred_element_type=F32)
                    acc = r if acc is None else acc + r
                m2[wbuf] = mx
                ot_s[hp & 1, hp >> 1, :, pl.ds(cp, SQ)] = acc

            ss[1] = jnp.zeros((S, SQ), F32)
            m2[1] = jnp.zeros((8, SQ), F32)

            def body(it, carry):
                cur = jnp.minimum(it, H * nq - 1)
                prv = jnp.maximum(it - 1, 0)

                @pl.when((it & 1) == 0)
                def _():
                    block(cur, prv, 0)

                @pl.when((it & 1) == 1)
                def _():
                    block(cur, prv, 1)
                return carry

            jax.lax.fori_loop(0, H * nq + 1, body, 0)

            def fbody(i, carry):
                cols = pl.ds(pl.multiple_of((i % NCH) * 128, 128), 128)
                for _, p in freq_steps(i // NCH, (cols,)):
                    p(lambda v: v)
                return carry

            jax.lax.fori_loop(0, NG * NCH, fbody, 0)

        safe = jnp.logical_and(
            kmax * qmax * (1.02 * DH) <= SCORE_BOUND,
            jnp.logical_and(vmax <= 2.0 ** 30, vmax >= 2.0 ** -20))

        stage(0, 0, None, freq_steps(0, (0, 1)), rv=R0)

        jax.lax.cond(safe, fast_path, slow_path)

        cp_inv.wait()
        cp_wo.wait()
        accs = [None] * NSB
        ga = {}

        def pv_last(sb, c):
            cols = slice(sb * SB, (sb + 1) * SB)
            r = jnp.dot(vt_s[1, H // 2 - 1, :, c * CK:(c + 1) * CK],
                        s2[1, c * CK:(c + 1) * CK, cols], preferred_element_type=F32)
            accs[sb] = r if accs[sb] is None else accs[sb] + r

        def inv_block(i):
            rows = slice(i * BLK, (i + 1) * BLK)
            y = jnp.dot(inv_ref[...], zf_s[:, i].reshape(2 * BLK, D), preferred_element_type=F32)
            gx = x_v[rows, :].astype(F32) * jnp.concatenate([g_s[rows, :]] * NCH, axis=1)
            ga[i] = gx * (y + kv_s[rows, :])

        def out_block(i):
            sb, ii = divmod(i, SB // BLK)
            rows = slice(i * BLK, (i + 1) * BLK)
            oe = ot_s[0, :, :, rows]
            oo = jnp.concatenate([ot_s[1, 0:H // 2 - 1, :, rows],
                                  accs[sb][None, :, ii * BLK:(ii + 1) * BLK]], axis=0)
            low = jax.lax.broadcasted_iota(I32, (H // 2, 8, BLK), 1) < 4
            den = jnp.where(low, oo[:, 0:8], oe[:, 16:24])
            inv = pl.reciprocal(den, approx=True)
            inv = inv * (2.0 - den * inv)
            o = jnp.concatenate(
                [oe[:, 0:16] * inv[:, 4:5],
                 jnp.where(low, oe[:, 16:24], oo[:, 0:8]) * pltpu.roll(inv, 4, 1),
                 oo[:, 8:24] * inv[:, 0:1]], axis=1)
            o = o.reshape(D, BLK).T.astype(BF16)
            bb = jnp.dot(o, wo_v[...], preferred_element_type=F32)
            g1 = 1.0 - g_s[rows, :]
            out_v[rows, :] = (ga[i] + jnp.concatenate([g1] * NCH, axis=1) * bb).astype(BF16)
            pltpu.make_async_copy(out_v.at[rows, :], out_hbm.at[0, rows, :],
                                  sems.at[SEM_OUT]).start()

        nb = SB // BLK
        for i in range(nb):
            if i < nb - 1:
                for c in range(i * NC // (nb - 1), (i + 1) * NC // (nb - 1)):
                    pv_last(0, c)
            inv_block(i)
        for i in range(NB):
            out_block(i)
            sb, ii = divmod(i, nb)
            if sb + 1 < NSB:
                for c in range(ii * NC // nb, (ii + 1) * NC // nb):
                    pv_last(sb + 1, c)
                inv_block(i + nb)
        pltpu.make_async_copy(out_v, out_hbm.at[0], sems.at[SEM_OUT]).wait()

    pl.run_scoped(
        post_phase,
        pltpu.VMEM((2, S, S + 128), F32),
        pltpu.VMEM((4, 8, SQ), F32),
        pltpu.VMEM((NG, NB, 16, D), F32),
        pltpu.VMEM((2, H // 2, 24, S), F32),
        pltpu.VMEM((2, S, SQ), F32),
    )


@jax.jit
def pallas_gated_mix__ssm_conv_h3__mha_block__prompt_kernel(
    A_q: jax.Array,
    A_k: jax.Array,
    A_v: jax.Array,
    A_shift_k: jax.Array,
    A_ssm_k: jax.Array,
    A_ssm_D: jax.Array,
    B_x: jax.Array,
    B_wqkv: jax.Array,
    B_wo: jax.Array,
    gate_w: jax.Array,
):
    fwd, inv = _dft_consts()
    fwd = jnp.asarray(fwd, dtype=BF16)
    inv = jnp.asarray(inv, dtype=BF16).astype(F32)
    hbm = pl.BlockSpec(memory_space=pl.ANY)
    scratch = [
        pltpu.VMEM((S, D), BF16),
        pltpu.VMEM((S, D), BF16),
        pltpu.VMEM((D, D), BF16),
        pltpu.VMEM((H // 2, S // 2, 128), U32),
        pltpu.VMEM((2, H // 2, 16, S), U32),
        pltpu.VMEM((2, H // 2, 24, S), F32),
        pltpu.VMEM((S, D), F32),
        pltpu.VMEM((S, 128), F32),
        pltpu.VMEM((NG, NB, 16, D), F32),
        pltpu.VMEM((NG, NB, 16, D), F32),
        pltpu.VMEM((H // 2, R, 128), F32),
        pltpu.VMEM((2, DH, R, 128), F32),
        pltpu.VMEM((H // 2, 2 * DH, S), F32),
        pltpu.VMEM((2, DH, 8, S + 128), F32),
        pltpu.VMEM((4, 8, 128), F32),
        pltpu.VMEM((BLK, 2 * BLK), F32),
        pltpu.SMEM((1,), I32),
        pltpu.SemaphoreType.DMA((NSEM,)),
    ]
    return pl.pallas_call(
        _kernel,
        out_shape=jax.ShapeDtypeStruct((1, S, D), BF16),
        in_specs=[hbm] * 11,
        out_specs=hbm,
        scratch_shapes=scratch,
        compiler_params=pltpu.CompilerParams(vmem_limit_bytes=127 * 1024 * 1024),
    )(A_q, A_k, A_v, A_shift_k.T, A_ssm_k, A_ssm_D, B_wqkv, B_wo, gate_w, fwd, inv)
```

```python
import math

import jax
import jax.numpy as jnp
import numpy as np
import jax.experimental.pallas as pl
import jax.experimental.pallas.tpu as pltpu

S = 2048
D = 640
H = 32
DH = 20
KS = 4
NCH = D // 128
BLK = 128
NB = S // BLK
NG = BLK // 8
CK = 128
SB = 512
NC = S // CK
NSB = S // SB
NU = NC * NSB
RB = 256
NRB = S // RB
NPEEL = 3
QB = 512
NQB = S // QB
RODD = (288, 304, 288, 304)
REVEN = (304, 304, 304, 304)
R0 = 256
R = max(RODD + REVEN)
RP = (R + 31) // 32 * 32
SM = S - R
PKM, PQM = 32, 256
AE = 3
FE = 2
MA, MB = 2, 4
WA = 256
SQ = 128
SK = 512
SCORE_BOUND = 80.0
F32 = jnp.float32
BF16 = jnp.bfloat16
U32 = jnp.uint32
I32 = jnp.int32
NT = (((1,), (1,)), ((), ()))

SEM_WK, SEM_WQ, SEM_WV, SEM_WO, SEM_OUT = 0, 1, 2, 3, 4
SEM_GW, SEM_SHK, SEM_SSD, SEM_FWD, SEM_INV = 5, 6, 7, 8, 9
SEM_WK2 = 10
SEM_X = 11
SEM_K = SEM_X + NRB
SEM_V = SEM_K + NQB
SEM_H = SEM_V + NQB
NSEM = SEM_H + NQB


def _dft_consts():
    f = np.concatenate([np.arange(0, BLK, 2), np.arange(1, BLK, 2)]).astype(np.float64)
    n = np.arange(BLK, dtype=np.float64)
    ang = 2.0 * np.pi * (f[:, None] + 0.5) * n[None, :] / (2 * BLK)
    re = np.cos(ang).reshape(NG, 8, BLK)
    im = -np.sin(ang).reshape(NG, 8, BLK)
    fwd = np.concatenate([re, im], axis=1).reshape(2 * BLK, BLK)
    inv = fwd.T / BLK
    return fwd, inv


def _timeline(steps, t1, edges):
    total = sum(w for w, _ in steps)
    out = {}
    acc = 0
    for w, p in steps:
        cyc = t1 * acc / total / NU * edges[-1]
        acc += w
        u = max(i for i in range(NU) if edges[i] <= cyc)
        out.setdefault(u, []).append(((cyc - edges[u]) / (edges[u + 1] - edges[u]), p))
    return out


def _kernel(x_hbm, k_hbm, v_hbm, shk_hbm, h_hbm, ssd_hbm, w_hbm, wo_hbm, gw_hbm,
            fwd_hbm, inv_hbm, out_hbm,
            x_v, k_v, wo_v, kp_s, qh_s, vt_s, kv_s, g_s, uf_s, hf_s,
            kfp, kb_s, qf_s, qb_s, bd_s, inv_ref, fl_s, sems):
    out_v = k_v
    cp_wo = pltpu.make_async_copy(wo_hbm, wo_v, sems.at[SEM_WO])
    cp_inv = pltpu.make_async_copy(inv_hbm, inv_ref, sems.at[SEM_INV])

    def build_kb(j, par, d, anchor=None, lo=0):
        t = jnp.full((8, 128), par * DH + d, I32)
        if anchor is not None:
            t = anchor(t) & 127
        idx = jnp.concatenate([t] * ((R - lo) // 8), axis=0)
        kb_s[par, d, lo:R, :] = jnp.take_along_axis(
            kfp[j, lo:R, :], idx, axis=1, mode="promise_in_bounds")

    def pre_phase(v_v, h_v, w_v, wt_s, kf_s, hp_s, kn_s, fwd_ref, shk_ref, ssd_ref, gw_ref):
        def w_copy(part, sem):
            return pltpu.make_async_copy(w_hbm.at[:, part * D:(part + 1) * D],
                                         w_v.at[:, part * D:(part + 1) * D], sems.at[sem])

        def wk_copy(lo, hi, sem):
            return pltpu.make_async_copy(w_hbm.at[:, D + lo:D + hi],
                                         w_v.at[:, D + lo:D + hi], sems.at[sem])

        def x_copy(i):
            r0 = pl.multiple_of(i * RB, RB)
            return pltpu.make_async_copy(x_hbm.at[0, pl.ds(r0, RB), :],
                                         x_v.at[pl.ds(r0, RB), :], sems.at[SEM_X + i])

        def kvh_copies(i):
            r0 = pl.multiple_of(i * QB, QB)
            return (
                pltpu.make_async_copy(k_hbm.at[0, pl.ds(r0, QB), :],
                                      k_v.at[pl.ds(r0, QB), :], sems.at[SEM_K + i]),
                pltpu.make_async_copy(v_hbm.at[0, pl.ds(r0, QB), :],
                                      v_v.at[pl.ds(r0, QB), :], sems.at[SEM_V + i]),
                pltpu.make_async_copy(h_hbm.at[:, pl.ds(r0, QB)],
                                      h_v.at[:, pl.ds(r0, QB)], sems.at[SEM_H + i]),
            )

        cp_gw = pltpu.make_async_copy(gw_hbm, gw_ref, sems.at[SEM_GW])
        cp_small = (
            pltpu.make_async_copy(shk_hbm, shk_ref, sems.at[SEM_SHK]),
            pltpu.make_async_copy(ssd_hbm, ssd_ref, sems.at[SEM_SSD]),
            pltpu.make_async_copy(fwd_hbm, fwd_ref, sems.at[SEM_FWD]),
        )
        cp_gw.start()
        x_copy(0).start()
        wk_copy(0, WA, SEM_WK).start()
        wk_copy(WA, D, SEM_WK2).start()
        for i in range(1, NRB):
            x_copy(i).start()
        for cp in cp_small:
            cp.start()
        w_copy(0, SEM_WQ).start()
        w_copy(2, SEM_WV).start()
        for i in range(NQB):
            for cp in kvh_copies(i):
                cp.start()
        cp_wo.start()
        cp_inv.start()

        kf_s[0:8, :] = jnp.zeros((8, D), F32)
        hp_s[...] = jnp.zeros((2 * BLK, D), F32)
        bd_s[...] = jnp.zeros((4, 8, 128), F32)

        def track(i, val):
            a = jnp.abs(val)
            a = jnp.max(a.reshape(a.shape[0] // 8, 8, a.shape[1]), axis=0)
            m = bd_s[i]
            for c in range(a.shape[1] // 128):
                m = jnp.maximum(m, a[:, c * 128:(c + 1) * 128])
            bd_s[i] = m

        def split_pairs(val):
            lane = jax.lax.broadcasted_iota(I32, (val.shape[0], 128), 1)
            parts = [val[:, c * 128:(c + 1) * 128] for c in range(NCH)]
            out = []
            for j in range(H // 2):
                c, sh = divmod(2 * DH * j, 128)
                src = parts[c]
                if sh + 2 * DH > 128:
                    src = jnp.where(lane >= 64, src, parts[c + 1])
                out.append(pltpu.roll(src, 128 - sh, 1) if sh else src)
            return out

        def gate(r0):
            gw = gw_ref[...].astype(F32).reshape(1, D)
            xb = x_v[pl.ds(r0, RB), :].astype(F32)
            g = jax.nn.sigmoid(jnp.sum(xb * gw, axis=-1, keepdims=True))
            g_s[pl.ds(r0, RB), :] = jnp.broadcast_to(g, (RB, 128))

        def kproj(rb, head=None):
            r0 = pl.multiple_of(rb * RB, RB)
            xb = x_v[pl.ds(r0, RB), :]
            if head is None:
                kk = jnp.dot(xb, w_v[:, D:2 * D], preferred_element_type=F32)
            else:
                rest = jnp.concatenate(
                    [jnp.dot(xb[i * RB // MB:(i + 1) * RB // MB], w_v[:, D + WA:2 * D],
                             preferred_element_type=F32) for i in range(MB)], axis=0)
                kk = jnp.concatenate([head, rest], axis=1)
            track(0, kk)
            kp = pltpu.bitcast(kk.astype(BF16), U32)
            h0 = pl.multiple_of(rb * (RB // 2), RB // 2)
            kn_s[pl.ds(h0, RB // 2), :] = kp
            if isinstance(rb, int) and (rb + 1) * RB > SM:
                lo = max(SM, rb * RB)
                for j, part in enumerate(split_pairs(kp[(lo - rb * RB) // 2:, :])):
                    kfp[j, lo - SM:(rb + 1) * RB - SM, :] = pltpu.bitcast(part, BF16).astype(F32)
            if head is None:
                gate(r0)

        cp_gw.wait()
        x_copy(0).wait()
        gate(0)
        wk_copy(0, WA, SEM_WK).wait()
        head = jnp.concatenate(
            [jnp.dot(x_v[i * RB // MA:(i + 1) * RB // MA, :], w_v[:, D:D + WA],
                     preferred_element_type=F32) for i in range(MA)], axis=0)
        wk_copy(WA, D, SEM_WK2).wait()
        kproj(0, head)

        def kproj_loop(rb, carry):
            x_copy(rb).wait()
            kproj(rb)
            return carry

        jax.lax.fori_loop(1, NRB - NPEEL, kproj_loop, 0)
        for i in range(NRB - NPEEL, NRB):
            x_copy(i).wait()
        w_copy(0, SEM_WQ).wait()
        w_copy(2, SEM_WV).wait()
        for cp in cp_small:
            cp.wait()
        kproj(NRB - 1)
        wt_s[0:D, :] = w_v[:, 0:D].astype(F32).T.astype(BF16)
        wt_s[D:2 * D, :] = w_v[:, 2 * D:3 * D].astype(F32).T.astype(BF16)
        for i in range(NRB - 2, NRB - NPEEL - 1, -1):
            kproj(i)
        for d in range(DH):
            build_kb(0, 0, d, lo=R - R0)

        qscale = (DH ** -0.5) * math.log2(math.e)

        def fold(cur, prev):
            cur = cur.reshape(NG, 16, D)
            prev = prev.reshape(NG, 16, D)
            hg = NG // 2
            lo = jnp.concatenate(
                [cur[:hg, 0:8] - prev[:hg, 8:16], cur[:hg, 8:16] + prev[:hg, 0:8]], axis=1)
            hi = jnp.concatenate(
                [cur[hg:, 0:8] + prev[hg:, 8:16], cur[hg:, 8:16] - prev[hg:, 0:8]], axis=1)
            return jnp.concatenate([lo, hi], axis=0)

        def qvproj(rb, carry):
            for cp in kvh_copies(rb):
                cp.wait()
            ssd = ssd_ref[...].astype(F32).reshape(1, D)
            shk = shk_ref[...].astype(F32)
            r0 = pl.multiple_of(rb * QB, QB)

            def q_part(rs):
                xb = x_v[pl.ds(rs, RB), :]
                qt = jax.lax.dot_general(wt_s[0:D, :], xb, NT, preferred_element_type=F32)
                qt = qt * qscale
                track(1, qt)
                qf = qt.reshape(H // 2, 2 * DH, RB)
                row = jax.lax.broadcasted_iota(I32, (H // 2, 24, RB), 1)
                zpad = jnp.zeros((H // 2, 8, RB), F32)
                for par, win in ((0, jnp.where(row < DH, qf[:, 0:24], 0.0)),
                                 (1, jnp.where(row >= 4, qf[:, 16:40], 0.0))):
                    win = jnp.concatenate([win, zpad], axis=1).reshape(H // 2 * 32, RB)
                    qh_s[par, :, :, pl.ds(rs, RB)] = pltpu.bitcast(
                        win.astype(BF16), U32).reshape(H // 2, 16, RB)
                qf_s[:, :, pl.ds(rs, RB)] = qf
                for d in range(DH):
                    qb_s[0, d, :, pl.ds(rs, RB)] = jnp.broadcast_to(qf[0, d:d + 1, :], (8, RB))

            def v_part(rs):
                xb = x_v[pl.ds(rs, RB), :]
                vt = jax.lax.dot_general(wt_s[D:2 * D, :], xb, NT, preferred_element_type=F32)
                track(2, vt)
                vt = vt.reshape(H // 2, 2 * DH, RB)
                row = jax.lax.broadcasted_iota(I32, (H // 2, 24, RB), 1)
                vt_s[0, :, :, pl.ds(rs, RB)] = jnp.where(row < DH, vt[:, 0:24, :], 1.0)
                vt_s[1, :, :, pl.ds(rs, RB)] = jnp.where(row >= 4, vt[:, 16:40, :], 1.0)

            def k_split(rs):
                h0 = pl.multiple_of(rs // 2, RB // 2)
                for j, part in enumerate(split_pairs(kn_s[pl.ds(h0, RB // 2), :])):
                    kp_s[j, pl.ds(h0, RB // 2), :] = part

            def u_part(u, ktail):
                ru = pl.multiple_of(r0 + u * BLK, BLK)
                kc = k_v[pl.ds(ru, BLK), :].astype(F32)
                e3 = jnp.concatenate([ktail, kc], axis=0).reshape(BLK // 8 + 1, 8, D)
                sub = jax.lax.broadcasted_iota(I32, (BLK // 8, 8, D), 1)
                ksh = kc * shk[0:1, :]
                for j in range(1, KS):
                    rot = pltpu.roll(e3, j, 1)
                    sh = jnp.where(sub >= j, rot[1:], rot[:-1]).reshape(BLK, D)
                    ksh = ksh + sh * shk[j:j + 1, :]
                kv = ksh * v_v[pl.ds(ru, BLK), :].astype(F32)
                kv_s[pl.ds(ru, BLK), :] = kv * ssd
                uf_s[:, rb * (QB // BLK) + u] = jnp.dot(
                    fwd_ref[...], kv.astype(BF16),
                    preferred_element_type=F32).reshape(NG, 16, D)
                return kc[BLK - 8:, :]

            def h_part(u, prev):
                ru = pl.multiple_of(r0 + u * BLK, BLK)
                raw = jax.lax.dot_general(fwd_ref[...], h_v[:, pl.ds(ru, BLK)], NT,
                                          preferred_element_type=F32)
                hf_s[:, rb * (QB // BLK) + u] = fold(raw, prev)
                return raw

            ktail = kf_s[0:8, :]
            prev = hp_s[...]
            for sub in range(QB // RB):
                rs = pl.multiple_of(r0 + sub * RB, RB)
                k_split(rs)
                q_part(rs)
                ktail = u_part(2 * sub, ktail)
                prev = h_part(2 * sub, prev)
                prev = h_part(2 * sub + 1, prev)
                if sub == QB // RB - 1:
                    hp_s[...] = prev
                v_part(rs)
                ktail = u_part(2 * sub + 1, ktail)
            kf_s[0:8, :] = ktail
            return carry + rb

        fl_s[0] = jax.lax.fori_loop(0, NQB, qvproj, jnp.int32(0))

    pl.run_scoped(
        pre_phase,
        pltpu.VMEM((S, D), BF16),
        pltpu.VMEM((D, S), BF16),
        pltpu.VMEM((D, 3 * D), BF16),
        pltpu.VMEM((2 * D, D), BF16),
        pltpu.VMEM((32, D), F32),
        pltpu.VMEM((2 * BLK, D), F32),
        pltpu.VMEM((S // 2, D), U32),
        pltpu.VMEM((2 * BLK, BLK), BF16),
        pltpu.VMEM((KS, D), BF16),
        pltpu.VMEM((D,), BF16),
        pltpu.VMEM((D,), BF16),
    )

    def post_phase(s2, m2, zf_s, ot_s, ss):
        def freq_steps(g, chunks):
            steps = []
            for c in chunks:
                cols = slice(c * 128, (c + 1) * 128) if isinstance(c, int) else c
                for i in range(NB):
                    st = {}
                    for m0 in range(0, i + 1, FE):
                        ms = list(range(m0, min(i + 1, m0 + FE)))

                        def step(anchor, i=i, cols=cols, ms=ms, st=st):
                            for m in ms:
                                ur = uf_s[g, m, 0:8, cols]
                                ui = uf_s[g, m, 8:16, cols]
                                hr = hf_s[g, i - m, 0:8, cols]
                                hi = hf_s[g, i - m, 8:16, cols]
                                if m == ms[0]:
                                    ur = anchor(ur)
                                tr = ur * hr - ui * hi
                                ti = ur * hi + ui * hr
                                st["r"] = tr if m == 0 else st["r"] + tr
                                st["i"] = ti if m == 0 else st["i"] + ti
                            if ms[-1] == i:
                                zf_s[g, i, 0:8, cols] = st["r"]
                                zf_s[g, i, 8:16, cols] = st["i"]
                        steps.append((len(ms), step))
            return steps

        kmax = jnp.max(bd_s[0])
        qmax = jnp.max(bd_s[1])
        vmax = jnp.max(bd_s[2])
        live = fl_s[0] >= 0

        def tie_to(tie):
            def anchor(v):
                t = tie if tie.dtype == v.dtype else pltpu.bitcast(tie, v.dtype)
                if v.shape[0] > 8:
                    t = jnp.concatenate([t] * (v.shape[0] // 8), axis=0)
                return jnp.where(live, v, t)
            return anchor

        def stage(h_qk, par_qk, h_pv, fsteps, rvs):
            par_pv = 1 - par_qk
            bnds = [[min(S - rv, (((S - rv) * c // NC) + 15) // 16 * 16) for c in range(NC + 1)]
                    for rv in rvs]
            jq = h_qk >> 1
            j_nx = 0 if isinstance(h_qk, int) else jnp.minimum(h_qk + 1, H - 1) >> 1
            edges = [0]
            for u in range(NU):
                edges.append(edges[-1] + bnds[u // NC][u % NC + 1] - bnds[u // NC][u % NC]
                             + (24 if h_pv is not None else 0))
            ftl = _timeline(fsteps, NU - 0.512, edges)

            def prep_q(anchor, t, v):
                tc = slice(t * 128, (t + 1) * 128)
                r0 = par_pv * 16 + v * 8
                blk = anchor(qf_s[j_nx, r0:r0 + 8, tc])
                for rr in range(8):
                    d = r0 + rr - par_pv * DH
                    if 0 <= d < DH:
                        qb_s[par_pv, d, :, tc] = jnp.broadcast_to(blk[rr:rr + 1, :], (8, 128))

            ptl = _timeline([(1, lambda anchor, i=i: build_kb(j_nx, par_pv, i, anchor))
                             for i in range(DH)], NU - 3.84, edges)
            qtl = _timeline([(1, lambda anchor, t=t, v=v: prep_q(anchor, t, v))
                             for t in range(S // 128) for v in range(3)],
                            NU - 2.3, edges)
            if h_pv is not None:
                j = h_pv >> 1

            vsteps = []
            for sb in range(NSB):
                for k0 in range(R - rvs[sb], R, PKM):
                    PK = min(PKM, R - k0)
                    PQ = PQM * PKM // PK
                    for qq in range(SB // PQ):
                        st = {}
                        for d0 in range(0, DH, AE):
                            def step(anchor, k0=k0, q0=sb * SB + qq * PQ, d0=d0, st=st, PK=PK, PQ=PQ):
                                for d in range(d0, min(DH, d0 + AE)):
                                    kb = kb_s[par_qk, d, k0:k0 + PK, :]
                                    if d == d0:
                                        w = (d0 // AE) % (PK // 8)
                                        kb = jnp.concatenate(
                                            [anchor(kb[i * 8:(i + 1) * 8]) if i == w
                                             else kb[i * 8:(i + 1) * 8]
                                             for i in range(PK // 8)], axis=0)
                                    qr = qb_s[par_qk, d, :, q0:q0 + PQ]
                                    t = (jnp.concatenate([kb] * (PQ // 128), axis=1)
                                         * jnp.concatenate([qr] * (PK // 8), axis=0))
                                    st["a"] = t if d == 0 else st["a"] + t
                                if d0 + AE >= DH:
                                    s2[par_qk, SM + k0:SM + k0 + PK,
                                       q0:q0 + PQ] = jnp.exp2(st["a"])
                            vsteps.append((min(DH, d0 + AE) - d0, step))
            vtl = _timeline(vsteps, NU - 0.25, edges)

            acc = None
            for sb in range(NSB):
                cols = slice(sb * SB, (sb + 1) * SB)
                for c in range(NC):
                    u = sb * NC + c
                    r0, r1 = bnds[sb][c], bnds[sb][c + 1]
                    kc = pltpu.bitcast(kp_s[jq, r0 // 2:r1 // 2, :], BF16)
                    qt = qh_s[par_qk, jq, :, cols]
                    if par_qk == 1:
                        qt = jnp.concatenate([jnp.zeros((8, SB), U32), qt], axis=0)
                    qt = pltpu.bitcast(qt, BF16)
                    s = jnp.dot(kc[:, 0:qt.shape[0]], qt, preferred_element_type=F32)
                    s2[par_qk, r0:r1, cols] = jnp.exp2(s)
                    ties = s
                    if h_pv is not None:
                        ct, kq = divmod(u, NSB)
                        pc = slice(ct * 128, (ct + 1) * 128)
                        rs = [jnp.dot(vt_s[par_pv, j, :, kq * SB + i * CK:kq * SB + (i + 1) * CK],
                                      s2[par_pv, kq * SB + i * CK:kq * SB + (i + 1) * CK, pc],
                                      preferred_element_type=F32) for i in range(SB // CK)]
                        if kq == 0:
                            z = tie_to(s[0:8, 0:128])(jnp.zeros((8, 128), F32))
                            acc = jnp.concatenate([z] * 3, axis=0)
                        for rr in rs:
                            acc = acc + rr
                        if kq == NSB - 1:
                            ot_s[par_pv, j, :, pc] = acc
                        if u < NU - 1:
                            ties = jnp.concatenate([s, jnp.concatenate(rs, axis=1)], axis=0)
                    ng = ties.shape[0] // 8
                    for col, tl in ((0, vtl.get(u, [])), (1, ptl.get(u, [])), (2, ftl.get(u, [])),
                                    (3, qtl.get(u, []))):
                        for frac, p in tl:
                            gi = min(ng - 1, int(frac * ng))
                            p(tie_to(ties[gi * 8:(gi + 1) * 8, col * 128:(col + 1) * 128]))

        def fast_path():
            def body(i, carry):
                stage(2 * i + 1, 1, 2 * i, freq_steps(i, (2, 3, 4)), RODD)

                @pl.when(i < H // 2 - 1)
                def _():
                    stage(2 * i + 2, 0, 2 * i + 1, freq_steps(i + 1, (0, 1)), REVEN)
                return carry

            jax.lax.fori_loop(0, H // 2, body, 0)

        def slow_path():
            nq = S // SQ

            def block(it_qk, it_pv, wbuf):
                rbuf = 1 - wbuf
                h = it_qk // nq
                c0 = pl.multiple_of((it_qk % nq) * SQ, SQ)
                q32 = qh_s[h & 1, h >> 1, :, pl.ds(c0, SQ)]
                z = jnp.zeros((8, SQ), U32)
                qt = pltpu.bitcast(jnp.where((h & 1) == 1, jnp.concatenate([z, q32], axis=0),
                                             jnp.concatenate([q32, z], axis=0)), BF16)
                hp = it_pv // nq
                cp = pl.multiple_of((it_pv % nq) * SQ, SQ)
                m = jnp.max(m2[rbuf], axis=0, keepdims=True)
                mx = None
                acc = None
                for c in range(S // SK):
                    rows = slice(c * SK, (c + 1) * SK)
                    kc = pltpu.bitcast(kp_s[h >> 1, c * SK // 2:(c + 1) * SK // 2, :], BF16)
                    s = jnp.dot(kc[:, 0:48], qt, preferred_element_type=F32)
                    ss[wbuf, rows, :] = s
                    cm = jnp.max(s.reshape(SK // 8, 8, SQ), axis=0)
                    mx = cm if mx is None else jnp.maximum(mx, cm)
                    p = jnp.exp2(ss[rbuf, rows, :] - m)
                    s2[1, rows, pl.ds(cp, SQ)] = p
                    r = jnp.dot(vt_s[hp & 1, hp >> 1, :, rows], p, preferred_element_type=F32)
                    acc = r if acc is None else acc + r
                m2[wbuf] = mx
                ot_s[hp & 1, hp >> 1, :, pl.ds(cp, SQ)] = acc

            ss[1] = jnp.zeros((S, SQ), F32)
            m2[1] = jnp.zeros((8, SQ), F32)

            def body(it, carry):
                cur = jnp.minimum(it, H * nq - 1)
                prv = jnp.maximum(it - 1, 0)

                @pl.when((it & 1) == 0)
                def _():
                    block(cur, prv, 0)

                @pl.when((it & 1) == 1)
                def _():
                    block(cur, prv, 1)
                return carry

            jax.lax.fori_loop(0, H * nq + 1, body, 0)

            def fbody(i, carry):
                cols = pl.ds(pl.multiple_of((i % NCH) * 128, 128), 128)
                for _, p in freq_steps(i // NCH, (cols,)):
                    p(lambda v: v)
                return carry

            jax.lax.fori_loop(0, NG * NCH, fbody, 0)

        safe = jnp.logical_and(
            kmax * qmax * (1.02 * DH) <= SCORE_BOUND,
            jnp.logical_and(vmax <= 2.0 ** 30, vmax >= 2.0 ** -20))

        stage(0, 0, None, freq_steps(0, (0, 1)), [R0] * NSB)

        jax.lax.cond(safe, fast_path, slow_path)

        cp_inv.wait()
        cp_wo.wait()
        accs = [None] * NSB
        ga = {}

        def pv_last(sb, c):
            cols = slice(sb * SB, (sb + 1) * SB)
            r = jnp.dot(vt_s[1, H // 2 - 1, :, c * CK:(c + 1) * CK],
                        s2[1, c * CK:(c + 1) * CK, cols], preferred_element_type=F32)
            accs[sb] = r if accs[sb] is None else accs[sb] + r

        def inv_block(i):
            rows = slice(i * BLK, (i + 1) * BLK)
            y = jnp.dot(inv_ref[...], zf_s[:, i].reshape(2 * BLK, D), preferred_element_type=F32)
            gx = x_v[rows, :].astype(F32) * jnp.concatenate([g_s[rows, :]] * NCH, axis=1)
            ga[i] = gx * (y + kv_s[rows, :])

        def out_block(i):
            sb, ii = divmod(i, SB // BLK)
            rows = slice(i * BLK, (i + 1) * BLK)
            oe = ot_s[0, :, :, rows]
            oo = jnp.concatenate([ot_s[1, 0:H // 2 - 1, :, rows],
                                  accs[sb][None, :, ii * BLK:(ii + 1) * BLK]], axis=0)
            low = jax.lax.broadcasted_iota(I32, (H // 2, 8, BLK), 1) < 4
            den = jnp.where(low, oo[:, 0:8], oe[:, 16:24])
            inv = pl.reciprocal(den, approx=True)
            inv = inv * (2.0 - den * inv)
            o = jnp.concatenate(
                [oe[:, 0:16] * inv[:, 4:5],
                 jnp.where(low, oe[:, 16:24], oo[:, 0:8]) * pltpu.roll(inv, 4, 1),
                 oo[:, 8:24] * inv[:, 0:1]], axis=1)
            o = o.reshape(D, BLK).T.astype(BF16)
            bb = jnp.dot(o, wo_v[...], preferred_element_type=F32)
            g1 = 1.0 - g_s[rows, :]
            out_v[rows, :] = (ga[i] + jnp.concatenate([g1] * NCH, axis=1) * bb).astype(BF16)
            pltpu.make_async_copy(out_v.at[rows, :], out_hbm.at[0, rows, :],
                                  sems.at[SEM_OUT]).start()

        nb = SB // BLK
        for i in range(nb):
            if i < nb - 1:
                for c in range(i * NC // (nb - 1), (i + 1) * NC // (nb - 1)):
                    pv_last(0, c)
            inv_block(i)
        for i in range(NB):
            out_block(i)
            sb, ii = divmod(i, nb)
            if sb + 1 < NSB:
                for c in range(ii * NC // nb, (ii + 1) * NC // nb):
                    pv_last(sb + 1, c)
                inv_block(i + nb)
        pltpu.make_async_copy(out_v, out_hbm.at[0], sems.at[SEM_OUT]).wait()

    pl.run_scoped(
        post_phase,
        pltpu.VMEM((2, S, S + 128), F32),
        pltpu.VMEM((4, 8, SQ), F32),
        pltpu.VMEM((NG, NB, 16, D), F32),
        pltpu.VMEM((2, H // 2, 24, S), F32),
        pltpu.VMEM((2, S, SQ), F32),
    )


@jax.jit
def pallas_gated_mix__ssm_conv_h3__mha_block__prompt_kernel(
    A_q: jax.Array,
    A_k: jax.Array,
    A_v: jax.Array,
    A_shift_k: jax.Array,
    A_ssm_k: jax.Array,
    A_ssm_D: jax.Array,
    B_x: jax.Array,
    B_wqkv: jax.Array,
    B_wo: jax.Array,
    gate_w: jax.Array,
):
    fwd, inv = _dft_consts()
    fwd = jnp.asarray(fwd, dtype=BF16)
    inv = jnp.asarray(inv, dtype=BF16).astype(F32)
    hbm = pl.BlockSpec(memory_space=pl.ANY)
    scratch = [
        pltpu.VMEM((S, D), BF16),
        pltpu.VMEM((S, D), BF16),
        pltpu.VMEM((D, D), BF16),
        pltpu.VMEM((H // 2, S // 2, 128), U32),
        pltpu.VMEM((2, H // 2, 16, S), U32),
        pltpu.VMEM((2, H // 2, 24, S), F32),
        pltpu.VMEM((S, D), F32),
        pltpu.VMEM((S, 128), F32),
        pltpu.VMEM((NG, NB, 16, D), F32),
        pltpu.VMEM((NG, NB, 16, D), F32),
        pltpu.VMEM((H // 2, RP, 128), F32),
        pltpu.VMEM((2, DH, RP, 128), F32),
        pltpu.VMEM((H // 2, 2 * DH, S), F32),
        pltpu.VMEM((2, DH, 8, S + 128), F32),
        pltpu.VMEM((4, 8, 128), F32),
        pltpu.VMEM((BLK, 2 * BLK), F32),
        pltpu.SMEM((1,), I32),
        pltpu.SemaphoreType.DMA((NSEM,)),
    ]
    return pl.pallas_call(
        _kernel,
        out_shape=jax.ShapeDtypeStruct((1, S, D), BF16),
        in_specs=[hbm] * 11,
        out_specs=hbm,
        scratch_shapes=scratch,
        compiler_params=pltpu.CompilerParams(vmem_limit_bytes=127 * 1024 * 1024),
    )(A_q, A_k, A_v, A_shift_k.T, A_ssm_k, A_ssm_D, B_wqkv, B_wo, gate_w, fwd, inv)
```

```python
import math

import jax
import jax.numpy as jnp
import numpy as np
import jax.experimental.pallas as pl
import jax.experimental.pallas.tpu as pltpu

S = 2048
D = 640
H = 32
DH = 20
KS = 4
NCH = D // 128
BLK = 128
NB = S // BLK
NG = BLK // 8
CK = 128
SB = 512
NC = S // CK
NSB = S // SB
NU = NC * NSB
RB = 256
NRB = S // RB
NPEEL = 3
QB = 512
NQB = S // QB
RODD = (304, 288, 304, 288)
REVEN = (320, 304, 304, 304)
R0 = 256
R = max(RODD + REVEN)
RP = (R + 31) // 32 * 32
SM = S - R
PKM, PQM = 32, 256
AE = 3
FE = 2
MA, MB = 2, 4
WA = 256
SQ = 128
SK = 512
SCORE_BOUND = 80.0
F32 = jnp.float32
BF16 = jnp.bfloat16
U32 = jnp.uint32
I32 = jnp.int32
NT = (((1,), (1,)), ((), ()))

SEM_WK, SEM_WQ, SEM_WV, SEM_WO, SEM_OUT = 0, 1, 2, 3, 4
SEM_GW, SEM_SHK, SEM_SSD, SEM_FWD, SEM_INV = 5, 6, 7, 8, 9
SEM_WK2 = 10
SEM_X = 11
SEM_K = SEM_X + NRB
SEM_V = SEM_K + NQB
SEM_H = SEM_V + NQB
NSEM = SEM_H + NQB


def _dft_consts():
    f = np.concatenate([np.arange(0, BLK, 2), np.arange(1, BLK, 2)]).astype(np.float64)
    n = np.arange(BLK, dtype=np.float64)
    ang = 2.0 * np.pi * (f[:, None] + 0.5) * n[None, :] / (2 * BLK)
    re = np.cos(ang).reshape(NG, 8, BLK)
    im = -np.sin(ang).reshape(NG, 8, BLK)
    fwd = np.concatenate([re, im], axis=1).reshape(2 * BLK, BLK)
    inv = fwd.T / BLK
    return fwd, inv


def _timeline(steps, t1, edges):
    total = sum(w for w, _ in steps)
    out = {}
    acc = 0
    for w, p in steps:
        cyc = t1 * acc / total / NU * edges[-1]
        acc += w
        u = max(i for i in range(NU) if edges[i] <= cyc)
        out.setdefault(u, []).append(((cyc - edges[u]) / (edges[u + 1] - edges[u]), p))
    return out


def _kernel(x_hbm, k_hbm, v_hbm, shk_hbm, h_hbm, ssd_hbm, w_hbm, wo_hbm, gw_hbm,
            fwd_hbm, inv_hbm, out_hbm,
            x_v, k_v, wo_v, kp_s, qh_s, vt_s, kv_s, g_s, uf_s, hf_s,
            kfp, kb_s, qf_s, qb_s, bd_s, inv_ref, fl_s, sems):
    out_v = k_v
    cp_wo = pltpu.make_async_copy(wo_hbm, wo_v, sems.at[SEM_WO])
    cp_inv = pltpu.make_async_copy(inv_hbm, inv_ref, sems.at[SEM_INV])

    def build_kb(j, par, d, anchor=None, lo=0):
        t = jnp.full((8, 128), par * DH + d, I32)
        if anchor is not None:
            t = anchor(t) & 127
        idx = jnp.concatenate([t] * ((R - lo) // 8), axis=0)
        kb_s[par, d, lo:R, :] = jnp.take_along_axis(
            kfp[j, lo:R, :], idx, axis=1, mode="promise_in_bounds")

    def pre_phase(v_v, h_v, w_v, wt_s, kf_s, hp_s, kn_s, fwd_ref, shk_ref, ssd_ref, gw_ref):
        def w_copy(part, sem):
            return pltpu.make_async_copy(w_hbm.at[:, part * D:(part + 1) * D],
                                         w_v.at[:, part * D:(part + 1) * D], sems.at[sem])

        def wk_copy(lo, hi, sem):
            return pltpu.make_async_copy(w_hbm.at[:, D + lo:D + hi],
                                         w_v.at[:, D + lo:D + hi], sems.at[sem])

        def x_copy(i):
            r0 = pl.multiple_of(i * RB, RB)
            return pltpu.make_async_copy(x_hbm.at[0, pl.ds(r0, RB), :],
                                         x_v.at[pl.ds(r0, RB), :], sems.at[SEM_X + i])

        def kvh_copies(i):
            r0 = pl.multiple_of(i * QB, QB)
            return (
                pltpu.make_async_copy(k_hbm.at[0, pl.ds(r0, QB), :],
                                      k_v.at[pl.ds(r0, QB), :], sems.at[SEM_K + i]),
                pltpu.make_async_copy(v_hbm.at[0, pl.ds(r0, QB), :],
                                      v_v.at[pl.ds(r0, QB), :], sems.at[SEM_V + i]),
                pltpu.make_async_copy(h_hbm.at[:, pl.ds(r0, QB)],
                                      h_v.at[:, pl.ds(r0, QB)], sems.at[SEM_H + i]),
            )

        cp_gw = pltpu.make_async_copy(gw_hbm, gw_ref, sems.at[SEM_GW])
        cp_small = (
            pltpu.make_async_copy(shk_hbm, shk_ref, sems.at[SEM_SHK]),
            pltpu.make_async_copy(ssd_hbm, ssd_ref, sems.at[SEM_SSD]),
            pltpu.make_async_copy(fwd_hbm, fwd_ref, sems.at[SEM_FWD]),
        )
        cp_gw.start()
        x_copy(0).start()
        wk_copy(0, WA, SEM_WK).start()
        wk_copy(WA, D, SEM_WK2).start()
        for i in range(1, NRB):
            x_copy(i).start()
        for cp in cp_small:
            cp.start()
        w_copy(0, SEM_WQ).start()
        w_copy(2, SEM_WV).start()
        for i in range(NQB):
            for cp in kvh_copies(i):
                cp.start()
        cp_wo.start()
        cp_inv.start()

        kf_s[0:8, :] = jnp.zeros((8, D), F32)
        hp_s[...] = jnp.zeros((2 * BLK, D), F32)
        bd_s[...] = jnp.zeros((4, 8, 128), F32)

        def track(i, val):
            a = jnp.abs(val)
            a = jnp.max(a.reshape(a.shape[0] // 8, 8, a.shape[1]), axis=0)
            m = bd_s[i]
            for c in range(a.shape[1] // 128):
                m = jnp.maximum(m, a[:, c * 128:(c + 1) * 128])
            bd_s[i] = m

        def split_pairs(val):
            lane = jax.lax.broadcasted_iota(I32, (val.shape[0], 128), 1)
            parts = [val[:, c * 128:(c + 1) * 128] for c in range(NCH)]
            out = []
            for j in range(H // 2):
                c, sh = divmod(2 * DH * j, 128)
                src = parts[c]
                if sh + 2 * DH > 128:
                    src = jnp.where(lane >= 64, src, parts[c + 1])
                out.append(pltpu.roll(src, 128 - sh, 1) if sh else src)
            return out

        def gate(r0):
            gw = gw_ref[...].astype(F32).reshape(1, D)
            xb = x_v[pl.ds(r0, RB), :].astype(F32)
            g = jax.nn.sigmoid(jnp.sum(xb * gw, axis=-1, keepdims=True))
            g_s[pl.ds(r0, RB), :] = jnp.broadcast_to(g, (RB, 128))

        def kproj(rb, head=None):
            r0 = pl.multiple_of(rb * RB, RB)
            xb = x_v[pl.ds(r0, RB), :]
            if head is None:
                kk = jnp.dot(xb, w_v[:, D:2 * D], preferred_element_type=F32)
            else:
                rest = jnp.concatenate(
                    [jnp.dot(xb[i * RB // MB:(i + 1) * RB // MB], w_v[:, D + WA:2 * D],
                             preferred_element_type=F32) for i in range(MB)], axis=0)
                kk = jnp.concatenate([head, rest], axis=1)
            track(0, kk)
            kp = pltpu.bitcast(kk.astype(BF16), U32)
            h0 = pl.multiple_of(rb * (RB // 2), RB // 2)
            kn_s[pl.ds(h0, RB // 2), :] = kp
            if isinstance(rb, int) and (rb + 1) * RB > SM:
                lo = max(SM, rb * RB)
                for j, part in enumerate(split_pairs(kp[(lo - rb * RB) // 2:, :])):
                    kfp[j, lo - SM:(rb + 1) * RB - SM, :] = pltpu.bitcast(part, BF16).astype(F32)
            if head is None:
                gate(r0)

        cp_gw.wait()
        x_copy(0).wait()
        gate(0)
        wk_copy(0, WA, SEM_WK).wait()
        head = jnp.concatenate(
            [jnp.dot(x_v[i * RB // MA:(i + 1) * RB // MA, :], w_v[:, D:D + WA],
                     preferred_element_type=F32) for i in range(MA)], axis=0)
        wk_copy(WA, D, SEM_WK2).wait()
        kproj(0, head)

        def kproj_loop(rb, carry):
            x_copy(rb).wait()
            kproj(rb)
            return carry

        jax.lax.fori_loop(1, NRB - NPEEL, kproj_loop, 0)
        for i in range(NRB - NPEEL, NRB):
            x_copy(i).wait()
        w_copy(0, SEM_WQ).wait()
        w_copy(2, SEM_WV).wait()
        for cp in cp_small:
            cp.wait()
        kproj(NRB - 1)
        wt_s[0:D, :] = w_v[:, 0:D].astype(F32).T.astype(BF16)
        wt_s[D:2 * D, :] = w_v[:, 2 * D:3 * D].astype(F32).T.astype(BF16)
        for i in range(NRB - 2, NRB - NPEEL - 1, -1):
            kproj(i)
        for d in range(DH):
            build_kb(0, 0, d, lo=R - R0)

        qscale = (DH ** -0.5) * math.log2(math.e)

        def fold(cur, prev):
            cur = cur.reshape(NG, 16, D)
            prev = prev.reshape(NG, 16, D)
            hg = NG // 2
            lo = jnp.concatenate(
                [cur[:hg, 0:8] - prev[:hg, 8:16], cur[:hg, 8:16] + prev[:hg, 0:8]], axis=1)
            hi = jnp.concatenate(
                [cur[hg:, 0:8] + prev[hg:, 8:16], cur[hg:, 8:16] - prev[hg:, 0:8]], axis=1)
            return jnp.concatenate([lo, hi], axis=0)

        def qvproj(rb, carry):
            for cp in kvh_copies(rb):
                cp.wait()
            ssd = ssd_ref[...].astype(F32).reshape(1, D)
            shk = shk_ref[...].astype(F32)
            r0 = pl.multiple_of(rb * QB, QB)

            def q_part(rs):
                xb = x_v[pl.ds(rs, RB), :]
                qt = jax.lax.dot_general(wt_s[0:D, :], xb, NT, preferred_element_type=F32)
                qt = qt * qscale
                track(1, qt)
                qf = qt.reshape(H // 2, 2 * DH, RB)
                row = jax.lax.broadcasted_iota(I32, (H // 2, 24, RB), 1)
                zpad = jnp.zeros((H // 2, 8, RB), F32)
                for par, win in ((0, jnp.where(row < DH, qf[:, 0:24], 0.0)),
                                 (1, jnp.where(row >= 4, qf[:, 16:40], 0.0))):
                    win = jnp.concatenate([win, zpad], axis=1).reshape(H // 2 * 32, RB)
                    qh_s[par, :, :, pl.ds(rs, RB)] = pltpu.bitcast(
                        win.astype(BF16), U32).reshape(H // 2, 16, RB)
                qf_s[:, :, pl.ds(rs, RB)] = qf
                for d in range(DH):
                    qb_s[0, d, :, pl.ds(rs, RB)] = jnp.broadcast_to(qf[0, d:d + 1, :], (8, RB))

            def v_part(rs):
                xb = x_v[pl.ds(rs, RB), :]
                vt = jax.lax.dot_general(wt_s[D:2 * D, :], xb, NT, preferred_element_type=F32)
                track(2, vt)
                vt = vt.reshape(H // 2, 2 * DH, RB)
                row = jax.lax.broadcasted_iota(I32, (H // 2, 24, RB), 1)
                vt_s[0, :, :, pl.ds(rs, RB)] = jnp.where(row < DH, vt[:, 0:24, :], 1.0)
                vt_s[1, :, :, pl.ds(rs, RB)] = jnp.where(row >= 4, vt[:, 16:40, :], 1.0)

            def k_split(rs):
                h0 = pl.multiple_of(rs // 2, RB // 2)
                for j, part in enumerate(split_pairs(kn_s[pl.ds(h0, RB // 2), :])):
                    kp_s[j, pl.ds(h0, RB // 2), :] = part

            def u_part(u, ktail):
                ru = pl.multiple_of(r0 + u * BLK, BLK)
                kc = k_v[pl.ds(ru, BLK), :].astype(F32)
                e3 = jnp.concatenate([ktail, kc], axis=0).reshape(BLK // 8 + 1, 8, D)
                sub = jax.lax.broadcasted_iota(I32, (BLK // 8, 8, D), 1)
                ksh = kc * shk[0:1, :]
                for j in range(1, KS):
                    rot = pltpu.roll(e3, j, 1)
                    sh = jnp.where(sub >= j, rot[1:], rot[:-1]).reshape(BLK, D)
                    ksh = ksh + sh * shk[j:j + 1, :]
                kv = ksh * v_v[pl.ds(ru, BLK), :].astype(F32)
                kv_s[pl.ds(ru, BLK), :] = kv * ssd
                uf_s[:, rb * (QB // BLK) + u] = jnp.dot(
                    fwd_ref[...], kv.astype(BF16),
                    preferred_element_type=F32).reshape(NG, 16, D)
                return kc[BLK - 8:, :]

            def h_part(u, prev):
                ru = pl.multiple_of(r0 + u * BLK, BLK)
                raw = jax.lax.dot_general(fwd_ref[...], h_v[:, pl.ds(ru, BLK)], NT,
                                          preferred_element_type=F32)
                hf_s[:, rb * (QB // BLK) + u] = fold(raw, prev)
                return raw

            ktail = kf_s[0:8, :]
            prev = hp_s[...]
            for sub in range(QB // RB):
                rs = pl.multiple_of(r0 + sub * RB, RB)
                k_split(rs)
                q_part(rs)
                ktail = u_part(2 * sub, ktail)
                prev = h_part(2 * sub, prev)
                prev = h_part(2 * sub + 1, prev)
                if sub == QB // RB - 1:
                    hp_s[...] = prev
                v_part(rs)
                ktail = u_part(2 * sub + 1, ktail)
            kf_s[0:8, :] = ktail
            return carry + rb

        fl_s[0] = jax.lax.fori_loop(0, NQB, qvproj, jnp.int32(0))

    pl.run_scoped(
        pre_phase,
        pltpu.VMEM((S, D), BF16),
        pltpu.VMEM((D, S), BF16),
        pltpu.VMEM((D, 3 * D), BF16),
        pltpu.VMEM((2 * D, D), BF16),
        pltpu.VMEM((32, D), F32),
        pltpu.VMEM((2 * BLK, D), F32),
        pltpu.VMEM((S // 2, D), U32),
        pltpu.VMEM((2 * BLK, BLK), BF16),
        pltpu.VMEM((KS, D), BF16),
        pltpu.VMEM((D,), BF16),
        pltpu.VMEM((D,), BF16),
    )

    def post_phase(s2, m2, zf_s, ot_s, ss):
        def freq_steps(g, chunks):
            steps = []
            for c in chunks:
                cols = slice(c * 128, (c + 1) * 128) if isinstance(c, int) else c
                for i in range(NB):
                    st = {}
                    for m0 in range(0, i + 1, FE):
                        ms = list(range(m0, min(i + 1, m0 + FE)))

                        def step(anchor, i=i, cols=cols, ms=ms, st=st):
                            for m in ms:
                                ur = uf_s[g, m, 0:8, cols]
                                ui = uf_s[g, m, 8:16, cols]
                                hr = hf_s[g, i - m, 0:8, cols]
                                hi = hf_s[g, i - m, 8:16, cols]
                                if m == ms[0]:
                                    ur = anchor(ur)
                                tr = ur * hr - ui * hi
                                ti = ur * hi + ui * hr
                                st["r"] = tr if m == 0 else st["r"] + tr
                                st["i"] = ti if m == 0 else st["i"] + ti
                            if ms[-1] == i:
                                zf_s[g, i, 0:8, cols] = st["r"]
                                zf_s[g, i, 8:16, cols] = st["i"]
                        steps.append((len(ms), step))
            return steps

        kmax = jnp.max(bd_s[0])
        qmax = jnp.max(bd_s[1])
        vmax = jnp.max(bd_s[2])
        live = fl_s[0] >= 0

        def tie_to(tie):
            def anchor(v):
                t = tie if tie.dtype == v.dtype else pltpu.bitcast(tie, v.dtype)
                return jnp.where(live, v, t)
            return anchor

        def stage(h_qk, par_qk, h_pv, fsteps, rvs, rn):
            par_pv = 1 - par_qk
            bnds = [[min(S - rv, (((S - rv) * c // NC) + 15) // 16 * 16) for c in range(NC + 1)]
                    for rv in rvs]
            jq = h_qk >> 1
            j_nx = 0 if isinstance(h_qk, int) else jnp.minimum(h_qk + 1, H - 1) >> 1
            edges = [0]
            for u in range(NU):
                edges.append(edges[-1] + bnds[u // NC][u % NC + 1] - bnds[u // NC][u % NC]
                             + (24 if h_pv is not None else 0))
            ftl = _timeline(fsteps, NU - 0.24, edges)

            def prep_q(anchor, t, v):
                tc = slice(t * 128, (t + 1) * 128)
                r0 = par_pv * 16 + v * 8
                blk = anchor(qf_s[j_nx, r0:r0 + 8, tc])
                for rr in range(8):
                    d = r0 + rr - par_pv * DH
                    if 0 <= d < DH:
                        qb_s[par_pv, d, :, tc] = jnp.broadcast_to(blk[rr:rr + 1, :], (8, 128))

            ptl = _timeline([(1, lambda anchor, i=i: build_kb(j_nx, par_pv, i, anchor, R - rn))
                             for i in range(DH)], NU - 3.68, edges)
            qtl = _timeline([(1, lambda anchor, t=t, v=v: prep_q(anchor, t, v))
                             for t in range(S // 128) for v in range(3)],
                            NU - 0.55, edges)
            if h_pv is not None:
                j = h_pv >> 1

            vsteps = []
            for sb in range(NSB):
                for k0 in range(R - rvs[sb], R, PKM):
                    PK = min(PKM, R - k0)
                    PQ = PQM * PKM // PK
                    for qq in range(SB // PQ):
                        st = {}
                        for d0 in range(0, DH, AE):
                            def step(anchor, k0=k0, q0=sb * SB + qq * PQ, d0=d0, st=st, PK=PK, PQ=PQ):
                                for d in range(d0, min(DH, d0 + AE)):
                                    kb = kb_s[par_qk, d, k0:k0 + PK, :]
                                    if d == d0:
                                        w = (d0 // AE + 3) % (PK // 8)
                                        kb = jnp.concatenate(
                                            [anchor(kb[i * 8:(i + 1) * 8]) if i == w
                                             else kb[i * 8:(i + 1) * 8]
                                             for i in range(PK // 8)], axis=0)
                                    qr = qb_s[par_qk, d, :, q0:q0 + PQ]
                                    t = (jnp.concatenate([kb] * (PQ // 128), axis=1)
                                         * jnp.concatenate([qr] * (PK // 8), axis=0))
                                    st["a"] = t if d == 0 else st["a"] + t
                                if d0 + AE >= DH:
                                    s2[par_qk, SM + k0:SM + k0 + PK,
                                       q0:q0 + PQ] = jnp.exp2(st["a"])
                            vsteps.append((min(DH, d0 + AE) - d0, step))
            vtl = _timeline(vsteps, NU - 0.08, edges)

            acc = None
            for sb in range(NSB):
                cols = slice(sb * SB, (sb + 1) * SB)
                for c in range(NC):
                    u = sb * NC + c
                    r0, r1 = bnds[sb][c], bnds[sb][c + 1]
                    kc = pltpu.bitcast(kp_s[jq, r0 // 2:r1 // 2, :], BF16)
                    qt = qh_s[par_qk, jq, :, cols]
                    if par_qk == 1:
                        qt = jnp.concatenate([jnp.zeros((8, SB), U32), qt], axis=0)
                    qt = pltpu.bitcast(qt, BF16)
                    s = jnp.dot(kc[:, 0:qt.shape[0]], qt, preferred_element_type=F32)
                    s2[par_qk, r0:r1, cols] = jnp.exp2(s)
                    ties = s
                    if h_pv is not None:
                        ct, kq = divmod(u, NSB)
                        pc = slice(ct * 128, (ct + 1) * 128)
                        rs = [jnp.dot(vt_s[par_pv, j, :, kq * SB + i * CK:kq * SB + (i + 1) * CK],
                                      s2[par_pv, kq * SB + i * CK:kq * SB + (i + 1) * CK, pc],
                                      preferred_element_type=F32) for i in range(SB // CK)]
                        if kq == 0:
                            acc = None
                        for rr in rs:
                            acc = rr if acc is None else acc + rr
                        if kq == NSB - 1:
                            ot_s[par_pv, j, :, pc] = acc
                        if u < NU - 1:
                            ties = jnp.concatenate([s, jnp.concatenate(rs, axis=1)], axis=0)
                    ng = ties.shape[0] // 8
                    for col, tl in ((2, vtl.get(u, [])), (0, ptl.get(u, [])), (1, ftl.get(u, [])),
                                    (2, qtl.get(u, []))):
                        for frac, p in tl:
                            gi = min(ng - 1, int(frac * ng))
                            p(tie_to(ties[gi * 8:(gi + 1) * 8, col * 128:(col + 1) * 128]))

        def fast_path():
            def body(i, carry):
                stage(2 * i + 1, 1, 2 * i, freq_steps(i, (2, 3, 4)), RODD, max(REVEN))

                @pl.when(i < H // 2 - 1)
                def _():
                    stage(2 * i + 2, 0, 2 * i + 1, freq_steps(i + 1, (0, 1)), REVEN, max(RODD))
                return carry

            jax.lax.fori_loop(0, H // 2, body, 0)

        def slow_path():
            nq = S // SQ

            def block(it_qk, it_pv, wbuf):
                rbuf = 1 - wbuf
                h = it_qk // nq
                c0 = pl.multiple_of((it_qk % nq) * SQ, SQ)
                q32 = qh_s[h & 1, h >> 1, :, pl.ds(c0, SQ)]
                z = jnp.zeros((8, SQ), U32)
                qt = pltpu.bitcast(jnp.where((h & 1) == 1, jnp.concatenate([z, q32], axis=0),
                                             jnp.concatenate([q32, z], axis=0)), BF16)
                hp = it_pv // nq
                cp = pl.multiple_of((it_pv % nq) * SQ, SQ)
                m = jnp.max(m2[rbuf], axis=0, keepdims=True)
                mx = None
                acc = None
                for c in range(S // SK):
                    rows = slice(c * SK, (c + 1) * SK)
                    kc = pltpu.bitcast(kp_s[h >> 1, c * SK // 2:(c + 1) * SK // 2, :], BF16)
                    s = jnp.dot(kc[:, 0:48], qt, preferred_element_type=F32)
                    ss[wbuf, rows, :] = s
                    cm = jnp.max(s.reshape(SK // 8, 8, SQ), axis=0)
                    mx = cm if mx is None else jnp.maximum(mx, cm)
                    p = jnp.exp2(ss[rbuf, rows, :] - m)
                    s2[1, rows, pl.ds(cp, SQ)] = p
                    r = jnp.dot(vt_s[hp & 1, hp >> 1, :, rows], p, preferred_element_type=F32)
                    acc = r if acc is None else acc + r
                m2[wbuf] = mx
                ot_s[hp & 1, hp >> 1, :, pl.ds(cp, SQ)] = acc

            ss[1] = jnp.zeros((S, SQ), F32)
            m2[1] = jnp.zeros((8, SQ), F32)

            def body(it, carry):
                cur = jnp.minimum(it, H * nq - 1)
                prv = jnp.maximum(it - 1, 0)

                @pl.when((it & 1) == 0)
                def _():
                    block(cur, prv, 0)

                @pl.when((it & 1) == 1)
                def _():
                    block(cur, prv, 1)
                return carry

            jax.lax.fori_loop(0, H * nq + 1, body, 0)

            def fbody(i, carry):
                cols = pl.ds(pl.multiple_of((i % NCH) * 128, 128), 128)
                for _, p in freq_steps(i // NCH, (cols,)):
                    p(lambda v: v)
                return carry

            jax.lax.fori_loop(0, NG * NCH, fbody, 0)

        safe = jnp.logical_and(
            kmax * qmax * (1.02 * DH) <= SCORE_BOUND,
            jnp.logical_and(vmax <= 2.0 ** 30, vmax >= 2.0 ** -20))

        stage(0, 0, None, freq_steps(0, (0, 1)), [R0] * NSB, max(RODD))

        jax.lax.cond(safe, fast_path, slow_path)

        cp_inv.wait()
        cp_wo.wait()
        accs = [None] * NSB
        ga = {}

        def pv_last(sb, c):
            cols = slice(sb * SB, (sb + 1) * SB)
            r = jnp.dot(vt_s[1, H // 2 - 1, :, c * CK:(c + 1) * CK],
                        s2[1, c * CK:(c + 1) * CK, cols], preferred_element_type=F32)
            accs[sb] = r if accs[sb] is None else accs[sb] + r

        def inv_block(i):
            rows = slice(i * BLK, (i + 1) * BLK)
            y = jnp.dot(inv_ref[...], zf_s[:, i].reshape(2 * BLK, D), preferred_element_type=F32)
            gx = x_v[rows, :].astype(F32) * jnp.concatenate([g_s[rows, :]] * NCH, axis=1)
            ga[i] = gx * (y + kv_s[rows, :])

        def out_block(i):
            sb, ii = divmod(i, SB // BLK)
            rows = slice(i * BLK, (i + 1) * BLK)
            oe = ot_s[0, :, :, rows]
            oo = jnp.concatenate([ot_s[1, 0:H // 2 - 1, :, rows],
                                  accs[sb][None, :, ii * BLK:(ii + 1) * BLK]], axis=0)
            low = jax.lax.broadcasted_iota(I32, (H // 2, 8, BLK), 1) < 4
            den = jnp.where(low, oo[:, 0:8], oe[:, 16:24])
            inv = pl.reciprocal(den, approx=True)
            inv = inv * (2.0 - den * inv)
            o = jnp.concatenate(
                [oe[:, 0:16] * inv[:, 4:5],
                 jnp.where(low, oe[:, 16:24], oo[:, 0:8]) * pltpu.roll(inv, 4, 1),
                 oo[:, 8:24] * inv[:, 0:1]], axis=1)
            o = o.reshape(D, BLK).T.astype(BF16)
            bb = jnp.dot(o, wo_v[...], preferred_element_type=F32)
            g1 = 1.0 - g_s[rows, :]
            out_v[rows, :] = (ga[i] + jnp.concatenate([g1] * NCH, axis=1) * bb).astype(BF16)
            pltpu.make_async_copy(out_v.at[rows, :], out_hbm.at[0, rows, :],
                                  sems.at[SEM_OUT]).start()

        nb = SB // BLK
        for i in range(nb):
            if i < nb - 1:
                for c in range(i * NC // (nb - 1), (i + 1) * NC // (nb - 1)):
                    pv_last(0, c)
            inv_block(i)
        for i in range(NB):
            out_block(i)
            sb, ii = divmod(i, nb)
            if sb + 1 < NSB:
                for c in range(ii * NC // nb, (ii + 1) * NC // nb):
                    pv_last(sb + 1, c)
                inv_block(i + nb)
        pltpu.make_async_copy(out_v, out_hbm.at[0], sems.at[SEM_OUT]).wait()

    pl.run_scoped(
        post_phase,
        pltpu.VMEM((2, S, S + 128), F32),
        pltpu.VMEM((4, 8, SQ), F32),
        pltpu.VMEM((NG, NB, 16, D), F32),
        pltpu.VMEM((2, H // 2, 24, S), F32),
        pltpu.VMEM((2, S, SQ), F32),
    )


@jax.jit
def pallas_gated_mix__ssm_conv_h3__mha_block__prompt_kernel(
    A_q: jax.Array,
    A_k: jax.Array,
    A_v: jax.Array,
    A_shift_k: jax.Array,
    A_ssm_k: jax.Array,
    A_ssm_D: jax.Array,
    B_x: jax.Array,
    B_wqkv: jax.Array,
    B_wo: jax.Array,
    gate_w: jax.Array,
):
    fwd, inv = _dft_consts()
    fwd = jnp.asarray(fwd, dtype=BF16)
    inv = jnp.asarray(inv, dtype=BF16).astype(F32)
    hbm = pl.BlockSpec(memory_space=pl.ANY)
    scratch = [
        pltpu.VMEM((S, D), BF16),
        pltpu.VMEM((S, D), BF16),
        pltpu.VMEM((D, D), BF16),
        pltpu.VMEM((H // 2, S // 2, 128), U32),
        pltpu.VMEM((2, H // 2, 16, S), U32),
        pltpu.VMEM((2, H // 2, 24, S), F32),
        pltpu.VMEM((S, D), F32),
        pltpu.VMEM((S, 128), F32),
        pltpu.VMEM((NG, NB, 16, D), F32),
        pltpu.VMEM((NG, NB, 16, D), F32),
        pltpu.VMEM((H // 2, RP, 128), F32),
        pltpu.VMEM((2, DH, RP, 128), F32),
        pltpu.VMEM((H // 2, 2 * DH, S), F32),
        pltpu.VMEM((2, DH, 8, S + 128), F32),
        pltpu.VMEM((4, 8, 128), F32),
        pltpu.VMEM((BLK, 2 * BLK), F32),
        pltpu.SMEM((1,), I32),
        pltpu.SemaphoreType.DMA((NSEM,)),
    ]
    return pl.pallas_call(
        _kernel,
        out_shape=jax.ShapeDtypeStruct((1, S, D), BF16),
        in_specs=[hbm] * 11,
        out_specs=hbm,
        scratch_shapes=scratch,
        compiler_params=pltpu.CompilerParams(vmem_limit_bytes=127 * 1024 * 1024),
    )(A_q, A_k, A_v, A_shift_k.T, A_ssm_k, A_ssm_D, B_wqkv, B_wo, gate_w, fwd, inv)
```
